```python
import jax
import jax.numpy as jnp

def _softmax(x, axis=-1):
    return jax.nn.softmax(x, axis=axis)

def _gelu(x):
    return jax.nn.gelu(x, approximate=True)

def _silu(x):
    return jax.nn.silu(x)

def _sigmoid(x):
    return jax.nn.sigmoid(x)

def _layernorm(x, axis=-1, eps=1e-05):
    m = jnp.mean(x, axis=axis, keepdims=True)
    v = jnp.var(x, axis=axis, keepdims=True)
    return (x - m) / jnp.sqrt(v + eps)

def _scatter_add(tgt, idx, src, axis=0):
    return tgt.at[idx].add(src)

def _segment_sum(src, seg, n):
    return jax.ops.segment_sum(src, seg, n)

class _Rng:

    def __init__(self, key):
        self._k = key

    def _next(self):
        self._k, sub = jax.random.split(self._k)
        return sub

    def normal(self, shape):
        return jax.random.normal(self._next(), shape, dtype=jnp.bfloat16)

    def randint(self, lo, hi, shape):
        return jax.random.randint(self._next(), shape, lo, hi, dtype=jnp.int32)

    def uniform(self, shape, lo=0.0, hi=1.0):
        return jax.random.uniform(self._next(), shape, jnp.bfloat16, lo, hi)

    def permutation(self, n):
        return jax.random.permutation(self._next(), n)
kernel_name = 'concat_heads__memory_aug_recurrent_mem_tr__ssm_conv_h3__prompt'

def setup_inputs():
    _rng = _Rng(jax.random.key(int.from_bytes(__import__("os").urandom(4), "little")))
    _w = lambda a: (lambda t: t.astype(jnp.bfloat16) if jnp.issubdtype(t.dtype, jnp.floating) else t)(jnp.asarray(a))

    def _A_setup():
        B, S, Dm = (1, 2048, 1024)
        H, Dh = (32, 128)
        M, seg = (8, 32)
        seg = min(seg, S)
        S = S // seg * seg
        return {'x': _w((lambda *s: _rng.normal(s) * 0.05)(B, S, Dm)), 'mem0': _w((lambda *s: _rng.normal(s) * 0.05)(B, M, Dm)), 'Wq': _w((lambda *s: _rng.normal(s) * 0.05)(Dm, H, Dh) * Dm ** (-0.5)), 'Wk': _w((lambda *s: _rng.normal(s) * 0.05)(Dm, H, Dh) * Dm ** (-0.5)), 'Wv': _w((lambda *s: _rng.normal(s) * 0.05)(Dm, H, Dh) * Dm ** (-0.5)), 'Wo': _w((lambda *s: _rng.normal(s) * 0.05)(H, Dh, Dm) * (H * Dh) ** (-0.5)), 'seg_len': seg}
    _A_in = _A_setup()

    def _B_setup():
        B, S, D = (1, 2048, 1024)
        ks = 4
        return {'q': _w((lambda *s: _rng.normal(s) * 0.05)(B, S, D)), 'k': _w((lambda *s: _rng.normal(s) * 0.05)(B, S, D)), 'v': _w((lambda *s: _rng.normal(s) * 0.05)(B, S, D)), 'shift_k': _w((lambda *s: _rng.normal(s) * 0.05)(D, ks) * 0.5), 'ssm_k': _w((lambda *s: _rng.normal(s) * 0.05)(D, S) * (1.0 / S ** 0.5)), 'ssm_D': _w((lambda *s: _rng.normal(s) * 0.05)(D))}
    _B_in = _B_setup()
    return {'A_x': _A_in['x'], 'A_mem0': _A_in['mem0'], 'A_Wq': _A_in['Wq'], 'A_Wk': _A_in['Wk'], 'A_Wv': _A_in['Wv'], 'A_Wo': _A_in['Wo'], 'A_seg_len': _A_in['seg_len'], 'B_q': _B_in['q'], 'B_k': _B_in['k'], 'B_v': _B_in['v'], 'B_shift_k': _B_in['shift_k'], 'B_ssm_k': _B_in['ssm_k'], 'B_ssm_D': _B_in['ssm_D']}

def reference(A_x, A_mem0, A_Wq, A_Wk, A_Wv, A_Wo, A_seg_len, B_q, B_k, B_v, B_shift_k, B_ssm_k, B_ssm_D):

    def _A_ref(x, mem0, Wq, Wk, Wv, Wo, seg_len):
        B, S, Dm = x.shape
        H, Dh = (Wq.shape[1], Wq.shape[2])
        M = mem0.shape[1]
        scale = Dh ** (-0.5)
        n_seg = S // seg_len
        L = M + seg_len
        idx = jnp.arange(L)
        mask = (idx[:, None] < M) | (idx[:, None] >= idx[None, :])
        mem = mem0
        outs = []
        for s in range(n_seg):
            xs = x[:, s * seg_len:(s + 1) * seg_len, :].copy()
            h = jnp.concatenate([mem, xs], axis=1)
            q = jnp.einsum('btd,dhe->bhte', h, Wq)
            k = jnp.einsum('btd,dhe->bhte', h, Wk)
            v = jnp.einsum('btd,dhe->bhte', h, Wv)
            scores = jnp.einsum('bhqe,bhke->bhqk', q, k) * scale
            scores = jnp.where(mask[None, None], scores, -1000000000.0)
            p = _softmax(scores, axis=-1)
            o = jnp.einsum('bhqk,bhke->bhqe', p, v)
            o = jnp.einsum('bhte,hed->btd', o, Wo)
            mem = o[:, :M, :].copy()
            outs.append(o[:, M:, :])
        return jnp.concatenate(outs, axis=1)

    def _B_ref(q, k, v, shift_k, ssm_k, ssm_D):
        B, S, D = q.shape
        ks = shift_k.shape[-1]
        k_pad = jnp.pad(k, ((0, 0), (ks - 1, 0), (0, 0)))
        k_shift = jnp.zeros_like(k)
        for t in range(ks):
            k_shift = k_shift + k_pad[:, t:t + S, :] * shift_k[:, ks - 1 - t][None, None, :]
        kv = k_shift * v
        L = 2 * S
        kv_pad = jnp.pad(kv, ((0, 0), (0, S), (0, 0)))
        kf_pad = jnp.pad(ssm_k, ((0, 0), (0, S)))
        kv_f = (lambda x, axes=(-2, -1): jnp.fft.rfft2(x.astype(jnp.float32), axes=axes))(kv_pad[:, None, :, :], axes=(1, 2))
        kf_f = (lambda x, axes=(-2, -1): jnp.fft.rfft2(x.astype(jnp.float32), axes=axes))(kf_pad[:, None, :], axes=(1, 2))
        kf_f = (lambda x, *d: x.transpose(*d))(kf_f, 1, 2, 0)
        y_f = kv_f * kf_f[None, :, :, :]
        y = (lambda x, s, axes=(-2, -1): jnp.fft.irfft2(x, s=s, axes=axes).astype(jnp.bfloat16))(y_f, (1, L), axes=(1, 2))[:, 0, :S, :]
        y = y + kv * ssm_D[None, None, :]
        return q * y
    a = _A_ref(A_x, A_mem0, A_Wq, A_Wk, A_Wv, A_Wo, A_seg_len)
    b = _B_ref(B_q, B_k, B_v, B_shift_k, B_ssm_k, B_ssm_D)
    return jnp.concatenate([a, b], axis=-1)
```

```python
import functools
import numpy as np
import jax
import jax.numpy as jnp
import jax.experimental.pallas as pl
import jax.experimental.pallas.tpu as pltpu

S, DM, H, DH, M, D = 2048, 1024, 32, 128, 8, 1024
HD = H * DH
C = 128
NC = S // C
F32, BF16 = jnp.float32, jnp.bfloat16


def _dft_consts():
    th = 2 * np.pi * (np.arange(C)[:, None] + 0.5) / (2 * C)
    n = np.arange(2 * C)[None, :]
    cos, sin = np.cos(th * n), np.sin(th * n)
    fwd = np.concatenate([cos[:, :C], -sin[:, :C]], 0)
    inv = np.concatenate([cos, -sin], 0).T / C
    g = np.concatenate([inv[:C], inv[C:]], 1)
    return fwd.astype(np.float32), g.astype(np.float32)


_FWD, _INV = _dft_consts()


def _nn(a, b):
    return jnp.dot(a, b, preferred_element_type=F32)


def _nt(a, b):
    return jax.lax.dot_general(a, b, (((1,), (1,)), ((), ())), preferred_element_type=F32)


def _kernel(x_ref, mem0_ref, wq_h, wk_h, wv_h, wo_h, bq_h, bk_h, bv_h, sk_ref, ssmk_h, sd_ref,
            fwd_ref, inv_ref, o_ref, wq, wk, wv, wo, mo, wsem, *, seg):
    wcopies = [pltpu.make_async_copy(s_, d_, wsem.at[i])
               for i, (s_, d_) in enumerate(((wk_h, wk), (wv_h, wv), (wq_h, wq), (wo_h, wo)))]

    scale = DH ** -0.5
    nseg = S // seg
    G = 128 // seg

    L = M + seg

    def branch_a(prod):
        for c in wcopies:
            c.wait()
        ri = jax.lax.broadcasted_iota(jnp.int32, (L, L), 0)
        ci = jax.lax.broadcasted_iota(jnp.int32, (L, L), 1)
        mask = (ri < M) | (ri >= ci)

        def step(s, mem):
            rows = pl.ds(pl.multiple_of(s * seg, seg), seg)
            hb = jnp.concatenate([mem, x_ref[rows, :].astype(F32)], 0).astype(BF16)
            q = _nn(hb, wq[...]).astype(BF16)
            k = _nn(hb, wk[...]).astype(BF16)
            v = _nn(hb, wv[...]).astype(BF16)
            for h in range(H):
                cs = slice(h * DH, (h + 1) * DH)
                sc = jnp.where(mask, _nt(q[:, cs], k[:, cs]) * scale, -1e9)
                e = jnp.exp(sc - jnp.max(sc, -1, keepdims=True))
                p = (e / jnp.sum(e, -1, keepdims=True)).astype(BF16)
                mo[:, cs] = _nn(p, v[:, cs])
            prod(s)
            o = _nn(mo[...].astype(BF16), wo[...]).astype(BF16)
            o_ref[rows, 0:DM] = o[M:, :].astype(o_ref.dtype)
            return o[:M, :].astype(F32)
        jax.lax.fori_loop(0, nseg, step, mem0_ref[...].astype(F32))


    def branch_b(bq, bk, bv, sk, kp, kv, xf, kf, yb, sem):
        cps = [pltpu.make_async_copy(s_, d_, sem.at[i])
               for i, (s_, d_) in enumerate(((bk_h, bk), (bv_h, bv), (ssmk_h, sk), (bq_h, bq)))]
        for c in cps:
            c.start()
        for c in wcopies:
            c.start()
        fwd = fwd_ref[...]
        cps[0].wait()
        cps[1].wait()
        for c in range(NC):
            if c == 0:
                kp[0:16, :] = jnp.zeros((16, D), F32)
                kp[16:, :] = bk[0:C, :].astype(F32)
            else:
                kp[...] = bk[c * C - 16:(c + 1) * C, :].astype(F32)
            acc = kp[16:16 + C, :] * sk_ref[0:1, :].astype(F32)
            for d in range(1, 4):
                acc = acc + kp[16 - d:16 - d + C, :] * sk_ref[d:d + 1, :].astype(F32)
            kvc = (acc.astype(BF16).astype(F32) * bv[c * C:(c + 1) * C, :].astype(F32)).astype(BF16)
            kv[c * C:(c + 1) * C, :] = kvc
            xf[c * 2 * C:(c + 1) * 2 * C, :] = _nn(fwd, kvc)
        cps[2].wait()

        def kspec(c, _):
            st = pl.multiple_of(c * C, C)
            kf[pl.ds(pl.multiple_of(c * 2 * C, 2 * C), 2 * C), :] = _nt(fwd, sk[:, pl.ds(st, C)])
            return 0
        jax.lax.fori_loop(0, NC, kspec, 0)

        def prod(t):
            a = t // (D // 128)
            col = pl.ds(pl.multiple_of((t % (D // 128)) * 128, 128), 128)
            ar = ai = None
            for n in range(NC + 1):
                first = n <= a
                i = jnp.where(first, a, NC - 1 - a)
                j = jnp.where(first, n, n - a - 1)
                xo = pl.multiple_of((i - j) * 2 * C, 2 * C)
                ko = pl.multiple_of(j * 2 * C, 2 * C)
                xr, xi = xf[pl.ds(xo, C), col], xf[pl.ds(xo + C, C), col]
                kr, ki = kf[pl.ds(ko, C), col], kf[pl.ds(ko + C, C), col]
                tr, ti = xr * kr - xi * ki, xr * ki + xi * kr
                if n == 0:
                    ar, ai = tr, ti
                else:
                    rs = j == 0
                    ar, ai = jnp.where(rs, 0.0, ar) + tr, jnp.where(rs, 0.0, ai) + ti
                yo = pl.multiple_of(i * 2 * C, 2 * C)
                yb[pl.ds(yo, C), col] = ar.astype(BF16)
                yb[pl.ds(yo + C, C), col] = ai.astype(BF16)
        branch_a(prod)
        cps[3].wait()
        inv = inv_ref[...]
        for c in range(NC):
            y = _nn(inv[:, :2 * C], yb[c * 2 * C:(c + 1) * 2 * C, :])
            if c > 0:
                y = y + _nn(inv[:, 2 * C:], yb[(c - 1) * 2 * C:c * 2 * C, :])
            rows = slice(c * C, (c + 1) * C)
            y = y + kv[rows, :].astype(F32) * sd_ref[...].astype(F32)
            o_ref[rows, DM:DM + D] = (bq[rows, :].astype(F32) * y).astype(o_ref.dtype)

    pl.run_scoped(branch_b, pltpu.VMEM((S, D), BF16), pltpu.VMEM((S, D), BF16), pltpu.VMEM((S, D), BF16),
                  pltpu.VMEM((D, S), BF16), pltpu.VMEM((C + 16, D), F32), pltpu.VMEM((S, D), BF16),
                  pltpu.VMEM((2 * S, D), F32), pltpu.VMEM((2 * S, D), F32), pltpu.VMEM((2 * S, D), BF16), pltpu.SemaphoreType.DMA((4,)))


@functools.partial(jax.jit, static_argnames=("A_seg_len",))
def pallas_concat_heads__memory_aug_recurrent_mem_tr__ssm_conv_h3__prompt_kernel(
        A_x, A_mem0, A_Wq, A_Wk, A_Wv, A_Wo, A_seg_len, B_q, B_k, B_v, B_shift_k, B_ssm_k, B_ssm_D):
    seg = int(A_seg_len)
    vm = pl.BlockSpec(memory_space=pltpu.VMEM)
    hbm = pl.BlockSpec(memory_space=pl.ANY)
    out = pl.pallas_call(
        functools.partial(_kernel, seg=seg),
        in_specs=[vm, vm, hbm, hbm, hbm, hbm, hbm, hbm, hbm, vm, hbm, vm, vm, vm],
        out_specs=vm,
        out_shape=jax.ShapeDtypeStruct((S, DM + D), BF16),
        scratch_shapes=[pltpu.VMEM((DM, HD), BF16)] * 3 + [pltpu.VMEM((HD, DM), BF16), pltpu.VMEM((M + seg, HD), F32),
 pltpu.SemaphoreType.DMA((4,))],
        compiler_params=pltpu.CompilerParams(vmem_limit_bytes=124 * 1024 * 1024),
    )(A_x[0], A_mem0[0], A_Wq.reshape(DM, HD), A_Wk.reshape(DM, HD), A_Wv.reshape(DM, HD),
      A_Wo.reshape(HD, DM), B_q[0], B_k[0], B_v[0], B_shift_k.T, B_ssm_k, B_ssm_D.reshape(1, D),
      jnp.asarray(_FWD).astype(BF16), jnp.asarray(_INV).astype(BF16))
    return out[None]
```

```python
import functools
import numpy as np
import jax
import jax.numpy as jnp
import jax.experimental.pallas as pl
import jax.experimental.pallas.tpu as pltpu

S, DM, H, DH, M, D = 2048, 1024, 32, 128, 8, 1024
HD = H * DH
SEG = 32
NSEG = S // SEG
C = 128
NC = S // C
GH = 2
F32, BF16, U32 = jnp.float32, jnp.bfloat16, jnp.uint32


def _dft_consts():
    th = 2 * np.pi * (np.arange(C)[:, None] + 0.5) / (2 * C)
    n = np.arange(2 * C)[None, :]
    cos, sin = np.cos(th * n), np.sin(th * n)
    fwd = np.concatenate([cos[:, :C], -sin[:, :C]], 0)
    inv = np.concatenate([cos, -sin], 0).T / C
    perm = np.arange(2 * C).reshape(2, C).T.reshape(-1)
    inv = inv[:, perm]
    g = np.concatenate([inv[:C], inv[C:]], 1)
    return fwd.astype(np.float32), g.astype(np.float32)


_FWD, _INV = _dft_consts()


def _nn(a, b):
    return jnp.dot(a, b, preferred_element_type=F32)


def _nt(a, b):
    return jax.lax.dot_general(a, b, (((1,), (1,)), ((), ())), preferred_element_type=F32)


def _b(x):
    return pltpu.bitcast(x, BF16)


def _pk(x):
    return pltpu.bitcast(x.astype(BF16), U32)


def _unpack2(a, b):
    lo = lambda x: pltpu.bitcast(x << 16, F32)
    hi = lambda x: pltpu.bitcast(x & jnp.uint32(0xffff0000), F32)
    ev = _pk(jnp.concatenate([lo(a), lo(b)], 0))
    od = _pk(jnp.concatenate([hi(a), hi(b)], 0))
    return ev, od


def _kernel(x_ref, mem0_ref, wq_h, wk_h, wv_h, wo_h, x_h, bq_h, bk_h, bv_h, sk_ref, ssmk_h, sd_ref,
            fwd_ref, inv_ref, out_h,
            w3, wo, qkv3, kv, xf, kf, ob, osem):
    scale = DH ** -0.5
    w_h = [r.bitcast(U32) for r in (wq_h, wk_h, wv_h)]

    def phase1(slab, x3, bk, sk, kp, wsem, dsem):
        def slab_cp(m, hp):
            return pltpu.make_async_copy(w_h[m].at[:, hp, :], slab.at[hp], wsem.at[hp])
        x3_cp = pltpu.make_async_copy(x_h.reshape(NSEG, SEG, DM).at[:, pl.ds(24, 8), :], x3, dsem.at[0])
        wo_cp = pltpu.make_async_copy(wo_h.bitcast(U32), wo, dsem.at[1])
        bk_cp = pltpu.make_async_copy(bk_h, bk, dsem.at[2])
        bv_cp = pltpu.make_async_copy(bv_h, kv, dsem.at[3])
        sk_cp = pltpu.make_async_copy(ssmk_h, sk, dsem.at[4])
        x3_cp.start()
        for hp in range(16):
            slab_cp(0, hp).start()
        x3_cp.wait()
        x3v = x3.reshape(NSEG * 8, DM)
        for m in range(3):
            def quarter(qi, _):
                for hh in range(4):
                    hp = qi * 4 + hh
                    slab_cp(m, hp).wait()

                    def body(i, _):
                        r = pl.multiple_of(i * 64, 64)
                        for j in range(4):
                            ev, od = _unpack2(slab[hp, pl.ds(r + j * 16, 8), :],
                                              slab[hp, pl.ds(r + j * 16 + 8, 8), :])
                            r2 = pl.ds(pl.multiple_of(i * 32 + j * 8, 8), 8)
                            w3[m, r2, pl.ds(pl.multiple_of(hp * 256, 256), 128)] = ev
                            w3[m, r2, pl.ds(pl.multiple_of(hp * 256 + 128, 128), 128)] = od
                        return 0
                    jax.lax.fori_loop(0, 16, body, 0, unroll=2)
                    if m < 2:
                        slab_cp(m + 1, hp).start()
                cols = pl.ds(pl.multiple_of(qi * 1024, 1024), 1024)
                r = _nn(x3v[...], _b(w3[m, :, cols]))
                qkv3[m, :, cols] = _pk(r)
                return 0
            jax.lax.fori_loop(0, 4, quarter, 0)
            if m == 0:
                bk_cp.start()
                bv_cp.start()
            elif m == 1:
                sk_cp.start()
                wo_cp.start()

        fwd = fwd_ref[...]
        bk_cp.wait()
        bv_cp.wait()
        kp[0:16, :] = jnp.zeros((16, D), F32)

        def bfwd(c, _):
            rows = pl.ds(pl.multiple_of(c * C, C), C)
            kp[16:, :] = bk[rows, :].astype(F32)
            acc = kp[16:16 + C, :] * sk_ref[0:1, :].astype(F32)
            for d in range(1, 4):
                acc = acc + kp[16 - d:16 - d + C, :] * sk_ref[d:d + 1, :].astype(F32)
            kvc = (acc.astype(BF16).astype(F32) * kv[rows, :].astype(F32)).astype(BF16)
            kv[rows, :] = kvc
            xf[pl.ds(pl.multiple_of(c * 2 * C, 2 * C), 2 * C), :] = _nn(fwd, kvc)
            kp[0:16, :] = kp[C:C + 16, :]
            return 0
        jax.lax.fori_loop(0, NC, bfwd, 0)
        sk_cp.wait()

        def kspec(c, _):
            st = pl.multiple_of(c * C, C)
            kf[pl.ds(pl.multiple_of(c * 2 * C, 2 * C), 2 * C), :] = _nt(fwd, sk[:, pl.ds(st, C)])
            return 0
        jax.lax.fori_loop(0, NC, kspec, 0)
        wo_cp.wait()

    pl.run_scoped(phase1, pltpu.VMEM((16, 1024, 128), U32), pltpu.VMEM((NSEG, 8, DM), BF16),
                  pltpu.VMEM((S, D), BF16), pltpu.VMEM((D, S), BF16), pltpu.VMEM((C + 16, D), F32),
                  pltpu.SemaphoreType.DMA((16,)), pltpu.SemaphoreType.DMA((5,)))

    def phase2(yb, bq, o3, dsem):
        bq_cp = pltpu.make_async_copy(bq_h, bq, dsem.at[0])
        bq_cp.start()

        def prod(u, a, tie):
            xf[pl.ds(2 * S, 8), 0:128] = tie
            fr = (u >> 3) * 8
            col = pl.ds(pl.multiple_of((u & 7) * 128, 128), 128)
            for i in (a, NC - 1 - a):
                ar = ai = None
                for j in range(i + 1):
                    xo = pl.multiple_of((i - j) * 2 * C + fr, 8)
                    ko = pl.multiple_of(j * 2 * C + fr, 8)
                    xr, xi = xf[pl.ds(xo, 8), col], xf[pl.ds(xo + C, 8), col]
                    kr, ki = kf[pl.ds(ko, 8), col], kf[pl.ds(ko + C, 8), col]
                    tr, ti = xr * kr - xi * ki, xr * ki + xi * kr
                    ar, ai = (tr, ti) if ar is None else (ar + tr, ai + ti)
                yb[pl.ds(pl.multiple_of(i * C + fr, 8), 8), col] = pltpu.pack_elementwise([ar, ai], packed_dtype=BF16)

        ri = jax.lax.broadcasted_iota(jnp.int32, (48, 48), 0)
        ci = jax.lax.broadcasted_iota(jnp.int32, (48, 48), 1)

        def tok(i):
            return jnp.where(i < 16, i + 8, jnp.where(i < 32, i - 16, 24 + (i & 7)))
        base = (ri < M) | (ci < M) | (tok(ci) <= tok(ri))
        mask0 = base & (ci < 40)
        mask1 = base & ((ci < 32) | (ci >= 40))
        sub = jax.lax.broadcasted_iota(jnp.int32, (8, 128), 0)

        def step(s, mem):
            par = s & 1
            j = s >> 1
            bias = jnp.where(par == 0, jnp.where(mask0, 1.0, 0.0), jnp.where(mask1, 1.0, 0.0)) > 0.5
            keep = jnp.where(par == 0, jnp.where(sub < 4, 1, 0), jnp.where(sub >= 4, 1, 0)) > 0
            r0 = pl.multiple_of(s * SEG, SEG)
            xs0 = x_ref[pl.ds(r0, 16), :]
            xs1 = x_ref[pl.ds(r0 + 16, 8), :].astype(F32)
            hb = jnp.concatenate([jnp.concatenate([mem, xs1], 0).astype(BF16), xs0], 0)
            jr = pl.ds(pl.multiple_of(j * 8, 8), 8)

            def proj(g):
                cs = slice(g * GH * DH, (g + 1) * GH * DH)
                res = [_nn(hb, _b(w3[m, :, cs])) for m in (1, 0, 2)]
                return [t.astype(BF16) for t in res], res[0][0:8, 0:128]

            def attn(g, kqv):
                k, q, v = kqv
                outs = []
                for hh in range(GH):
                    h = g * GH + hh
                    cs = slice(h * DH, (h + 1) * DH)
                    ls = slice(hh * DH, (hh + 1) * DH)
                    qh = jnp.concatenate([q[:, ls], _b(qkv3[0, jr, cs])], 0)
                    kh = jnp.concatenate([k[:, ls], _b(qkv3[1, jr, cs])], 0)
                    vh = jnp.concatenate([v[:, ls], _b(qkv3[2, jr, cs])], 0)
                    sc = jnp.where(bias, _nt(qh, kh) * scale, -1e9)
                    e = jnp.exp(sc - jnp.max(sc, -1, keepdims=True))
                    p = (e / jnp.sum(e, -1, keepdims=True)).astype(BF16)
                    oh = _nn(p, vh)
                    outs.append(oh[:32].astype(BF16))
                    o3[jr, cs] = jnp.where(keep, _pk(oh[32:]), o3[jr, cs])
                return outs
            NG = H // GH
            os_ = []
            prev, tie = proj(0)
            prod(2 * s, 0, tie)
            r = None
            done = 0
            for g in range(1, NG + 1):
                if g < NG:
                    cur, tie = proj(g)
                os_ += attn(g - 1, prev)
                prev = cur
                if g < NG:
                    prod(2 * s + g // 8, g % 8, tie)
                if g in (8, NG):
                    n = len(os_)
                    part = _nn(jnp.concatenate(os_, 1), _b(wo[done * DH // 2:(done + n) * DH // 2, :]))
                    r = part if r is None else r + part
                    os_ = []
                    done += n
            r = r.astype(BF16)
            ob[pl.ds(r0, 16), 0:DM] = r[16:32]
            ob[pl.ds(r0 + 16, 8), 0:DM] = r[8:16]
            return r[0:8].astype(F32)
        o3[...] = jnp.zeros(o3.shape, U32)
        jax.lax.fori_loop(0, NSEG, step, mem0_ref[...].astype(F32))

        ob3 = ob.reshape(NSEG, SEG, DM + D)
        out3 = out_h.reshape(NSEG, SEG, DM + D)
        a_cp = pltpu.make_async_copy(ob3.at[:, pl.ds(0, 24), pl.ds(0, DM)],
                                     out3.at[:, pl.ds(0, 24), pl.ds(0, DM)], osem.at[0])
        a_cp.start()

        bq_cp.wait()
        inv = inv_ref[...]

        def b_cp(c):
            rows = pl.ds(pl.multiple_of(c * C, C), C)
            return pltpu.make_async_copy(ob.at[rows, pl.ds(DM, D)], out_h.at[rows, pl.ds(DM, D)], osem.at[1])

        def binv(c, _):
            rows = pl.ds(pl.multiple_of(c * C, C), C)
            y = _nn(inv[:, :2 * C], _b(yb[pl.ds(pl.multiple_of(c * C, C), C), :]))
            cm = jnp.maximum(c - 1, 0)
            y2 = _nn(inv[:, 2 * C:], _b(yb[pl.ds(pl.multiple_of(cm * C, C), C), :]))
            y = y + jnp.where(c > 0, y2, 0.0)
            y = y + kv[rows, :].astype(F32) * sd_ref[...].astype(F32)
            ob[rows, DM:DM + D] = (bq[rows, :].astype(F32) * y).astype(BF16)
            b_cp(c).start()
            return 0
        jax.lax.fori_loop(0, NC, binv, 0)

        def f_cp(n):
            return pltpu.make_async_copy(ob3.at[pl.ds(n * 16, 16), pl.ds(24, 8), pl.ds(0, DM)],
                                         out3.at[pl.ds(n * 16, 16), pl.ds(24, 8), pl.ds(0, DM)], osem.at[2])

        def fin(n, _):
            rows = pl.ds(pl.multiple_of(n * 64, 64), 64)
            r = _nn(_b(o3[rows, :]), _b(wo[...]))
            for i in range(16):
                ob[pl.ds(pl.multiple_of(n * 512 + i * 32 + 24, 8), 8), 0:DM] = r[i * 8:(i + 1) * 8].astype(BF16)
            f_cp(n).start()
            return 0
        jax.lax.fori_loop(0, 4, fin, 0)
        a_cp.wait()
        for c in range(NC):
            b_cp(c).wait()
        for n in range(4):
            f_cp(n).wait()

    pl.run_scoped(phase2, pltpu.VMEM((S, D), U32), pltpu.VMEM((S, D), BF16), pltpu.VMEM((256, HD), U32),
                  pltpu.SemaphoreType.DMA((1,)))


@functools.partial(jax.jit, static_argnames=("A_seg_len",))
def pallas_concat_heads__memory_aug_recurrent_mem_tr__ssm_conv_h3__prompt_kernel(
        A_x, A_mem0, A_Wq, A_Wk, A_Wv, A_Wo, A_seg_len, B_q, B_k, B_v, B_shift_k, B_ssm_k, B_ssm_D):
    assert int(A_seg_len) == SEG
    vm = pl.BlockSpec(memory_space=pltpu.VMEM)
    hbm = pl.BlockSpec(memory_space=pl.ANY)
    out = pl.pallas_call(
        _kernel,
        in_specs=[vm, vm, hbm, hbm, hbm, hbm, hbm, hbm, hbm, hbm, vm, hbm, vm, vm, vm],
        out_specs=hbm,
        out_shape=jax.ShapeDtypeStruct((S, DM + D), BF16),
        scratch_shapes=[pltpu.VMEM((3, 512, HD), U32), pltpu.VMEM((HD // 2, DM), U32),
                        pltpu.VMEM((3, 256, HD), U32), pltpu.VMEM((S, D), BF16),
                        pltpu.VMEM((2 * S + 8, D), F32), pltpu.VMEM((2 * S, D), F32),
                        pltpu.VMEM((S, DM + D), BF16), pltpu.SemaphoreType.DMA((3,))],
        compiler_params=pltpu.CompilerParams(vmem_limit_bytes=126 * 1024 * 1024),
    )(A_x[0], A_mem0[0], A_Wq, A_Wk, A_Wv, A_Wo.reshape(HD, DM), A_x[0], B_q[0], B_k[0], B_v[0],
      B_shift_k.T, B_ssm_k, B_ssm_D.reshape(1, D),
      jnp.asarray(_FWD).astype(BF16), jnp.asarray(_INV).astype(BF16))
    return out[None]
```

```python
import functools
import numpy as np
import jax
import jax.numpy as jnp
import jax.experimental.pallas as pl
import jax.experimental.pallas.tpu as pltpu

S, DM, H, DH, M, D = 2048, 1024, 32, 128, 8, 1024
HD = H * DH
SEG = 32
NSEG = S // SEG
C = 128
NC = S // C
GH = 2
ORDER = (('q', 0), ('pv', 2), ('qk', 1), ('k', 0), ('v', 0), ('sm', 1))
PARTS = ((16, 0), (28, 16), (32, 0))
F32, BF16, U32 = jnp.float32, jnp.bfloat16, jnp.uint32
LOG2E = 1.4426950408889634


def _dft_consts():
    th = 2 * np.pi * (np.arange(C)[:, None] + 0.5) / (2 * C)
    n = np.arange(2 * C)[None, :]
    cos, sin = np.cos(th * n), np.sin(th * n)
    fwd = np.concatenate([cos[:, :C], -sin[:, :C]], 0)
    inv = np.concatenate([cos, -sin], 0).T / C
    perm = np.arange(2 * C).reshape(2, C).T.reshape(-1)
    inv = inv[:, perm]
    g = np.concatenate([inv[:C], inv[C:]], 1)
    return fwd.astype(np.float32), g.astype(np.float32)


def _attn_masks():
    nat = np.array([-1] * 8 + list(range(16, 24)) + list(range(16)))
    qlab = np.concatenate([nat, np.arange(24, 32)])
    c = np.arange(16)
    inter = c // 2 + 8 * (c % 2)
    klab = np.concatenate([nat[:16][inter], nat[16:][inter], 24 + c // 2])
    out = np.zeros((2, 40, 128), np.float32)
    for par in range(2):
        valid = np.concatenate([np.ones(32, bool), c % 2 == par])
        ok = (qlab[:, None] < 0) | (klab[None, :] < 0) | (klab[None, :] <= qlab[:, None])
        out[par, :, :48] = ok & valid[None, :]
    return out


_FWD, _INV = _dft_consts()
_MASKS = _attn_masks()


def _nn(a, b):
    return jnp.dot(a, b, preferred_element_type=F32)


def _nt(a, b):
    return jax.lax.dot_general(a, b, (((1,), (1,)), ((), ())), preferred_element_type=F32)


def _b(x):
    return pltpu.bitcast(x, BF16)


def _pe(lo, hi):
    return pltpu.pack_elementwise([lo, hi], packed_dtype=BF16)


def _lo(w):
    return pltpu.bitcast(w << 16, F32)


def _hi(w):
    return pltpu.bitcast(w & jnp.uint32(0xffff0000), F32)


def _wo(ref):
    return pltpu.annotate(ref, no_hazard_no_deps=True)


def _kernel(mem0_ref, wq_h, wk_h, wv_h, wo_h, x_h, bq_h, bk_h, bv_h, sk_ref, ssmk_h, sd_ref,
            fwd_ref, inv_ref, mask_ref, out_h,
            w3, wo, xs, qkv3, ob, osem):
    c_exp = DH ** -0.5 * LOG2E
    w_h = [r.bitcast(U32).reshape(DM // 2, 2, H // 2, DH) for r in (wq_h, wk_h, wv_h)]

    def b_cp(c):
        rows = pl.ds(pl.multiple_of(c * C, C), C)
        return pltpu.make_async_copy(ob.at[rows, pl.ds(DM, D)], out_h.at[rows, pl.ds(DM, D)], osem.at[1])

    def phase1(slab, x3, bk, bq, kv, sk, kp, xf, kf, yb, wsem, bsem, dsem):
        def slab_cp(m, hp, par):
            return pltpu.make_async_copy(w_h[m].at[:, par, hp, :], slab.at[hp, par], wsem.at[hp, par])
        x32 = x_h.bitcast(U32).reshape(NSEG // 2, 32, DM)
        x3d = x3.reshape(NSEG // 2, 8, DM)
        x3_cps = [pltpu.make_async_copy(x32.at[:, pl.ds(12 + 16 * p, 4), :], x3d.at[:, pl.ds(4 * p, 4), :],
                                        dsem.at[3 + p]) for p in range(2)]
        wo_cp = pltpu.make_async_copy(wo_h.bitcast(U32), wo, dsem.at[0])
        x_cp = pltpu.make_async_copy(x_h, xs, dsem.at[1])
        bq_cp = pltpu.make_async_copy(bq_h, bq, dsem.at[2])
        QB = NC // 4

        def bin_cps(p):
            rows = pl.ds(p * QB * C, QB * C)
            return [pltpu.make_async_copy(bk_h.at[rows], bk.at[rows], bsem.at[0, p]),
                    pltpu.make_async_copy(bv_h.at[rows], kv.at[rows], bsem.at[1, p]),
                    pltpu.make_async_copy(ssmk_h.at[:, rows], sk.at[:, rows], bsem.at[2, p])]

        def unit_cps(m, qi):
            return [slab_cp(m, qi * 4 + hh, par) for hh in range(4) for par in range(2)]

        def start(cps):
            for cp in cps:
                cp.start()

        start(bin_cps(0))
        start(bin_cps(1))
        kp[0:16, :] = jnp.zeros((16, D), F32)
        CB = 256

        def bfwd(c, _):
            fwd = fwd_ref[...]
            rows = pl.ds(pl.multiple_of(c * C, C), C)
            spec = pl.ds(pl.multiple_of(c * 2 * C, 2 * C), 2 * C)
            kp[16:, :] = bk[rows, :].astype(F32)
            for cb in range(D // CB):
                cols = slice(cb * CB, (cb + 1) * CB)
                acc = kp[16:16 + C, cols] * sk_ref[0:1, cols].astype(F32)
                for d in range(1, 4):
                    acc = acc + kp[16 - d:16 - d + C, cols] * sk_ref[d:d + 1, cols].astype(F32)
                kvc = (acc.astype(BF16).astype(F32) * kv[rows, cols].astype(F32)).astype(BF16)
                _wo(kv)[rows, cols] = kvc
                _wo(kf)[spec, cols] = _nt(fwd, sk[cols, rows])
                _wo(xf)[spec, cols] = _nn(fwd, kvc)
            kp[0:16, :] = kp[C:C + 16, :]
            return 0
        for p in range(4):
            for cp in bin_cps(p):
                cp.wait()
            if p + 2 < 4:
                start(bin_cps(p + 2))
            elif p == 2:
                start(x3_cps)
                start(unit_cps(0, 0))
            else:
                start(unit_cps(0, 1))
                start(unit_cps(0, 2))
            jax.lax.fori_loop(p * QB, (p + 1) * QB, bfwd, 0)

        def products(u):
            fr = pl.multiple_of((u >> 3) * 8, 8)
            col = pl.ds(pl.multiple_of((u & 7) * 128, 128), 128)
            xv = xf.at[pl.ds(fr, 2 * S - C + 8), col]
            kw = kf.at[pl.ds(fr, 2 * S - C + 8), col]
            yv = _wo(yb.at[pl.ds(fr, S - C + 8), col])
            for i in range(NC):
                ar = ai = None
                for j in range(i + 1):
                    xo, ko = (i - j) * 2 * C, j * 2 * C
                    xr, xi = xv[xo:xo + 8, :], xv[xo + C:xo + C + 8, :]
                    kr, ki = kw[ko:ko + 8, :], kw[ko + C:ko + C + 8, :]
                    tr, ti = xr * kr - xi * ki, xr * ki + xi * kr
                    ar, ai = (tr, ti) if ar is None else (ar + tr, ai + ti)
                    if j == i:
                        yv[i * C:i * C + 8, :] = _pe(ar, ai)
                    yield

        for cp in x3_cps:
            cp.wait()
        start(unit_cps(0, 3))
        NST = 11

        def unit(un, _):
            m, qi = un >> 2, un & 3
            wm = w3.at[m]
            for hh in range(4):
                hp = qi * 4 + hh
                for mm in range(3):
                    @pl.when(m == mm)
                    def _():
                        slab_cp(mm, hp, 0).wait()
                        slab_cp(mm, hp, 1).wait()

                def body(i, _):
                    for j in range(16):
                        r = pl.ds(pl.multiple_of(i * 128 + j * 8, 8), 8)
                        a, b = slab[hp, 0, r, :], slab[hp, 1, r, :]
                        wm[r, pl.ds(pl.multiple_of(hp * 256, 256), 128)] = (a & 0xffff) | (b << 16)
                        wm[r, pl.ds(pl.multiple_of(hp * 256 + 128, 128), 128)] = (
                            (a >> 16) | (b & jnp.uint32(0xffff0000)))
                    return 0
                jax.lax.fori_loop(0, 4, body, 0)
                for mm in range(2):
                    @pl.when(m == mm)
                    def _():
                        slab_cp(mm + 1, hp, 0).start()
                        slab_cp(mm + 1, hp, 1).start()

            @pl.when(un == 3)
            def _():
                bq_cp.start()

            @pl.when(un == 7)
            def _():
                wo_cp.start()
                x_cp.start()

            def strips():
                for t in range(NST):
                    yield from products(jnp.minimum(un * NST + t, 127))
            work = strips()
            per_dot = -(-NST * (NC * (NC + 1) // 2) // 32)
            wq = wm.at[:, pl.ds(pl.multiple_of(qi * 1024, 1024), 1024)]
            qo = _wo(qkv3.at[m].at[:, pl.ds(pl.multiple_of(qi * 1024, 1024), 1024)])
            for mb in range(4):
                for n in range(8):
                    cols = slice(n * 128, (n + 1) * 128)
                    r = _nn(_b(x3[mb * 64:(mb + 1) * 64, :]), _b(wq[:, cols]))
                    for j in range(8):
                        qo[mb * 64 + 8 * j:mb * 64 + 8 * j + 8, cols] = _pe(r[16 * j:16 * j + 8],
                                                                            r[16 * j + 8:16 * j + 16])
                    for _ in range(per_dot):
                        next(work, None)
            for _ in work:
                pass
            return 0
        jax.lax.fori_loop(0, 12, unit, 0)

        bq_cp.wait()

        def binv(c, _):
            inv = inv_ref[...]
            rows = pl.ds(pl.multiple_of(c * C, C), C)
            prev = pl.ds(pl.multiple_of(jnp.maximum(c - 1, 0) * C, C), C)
            for cb in range(D // CB):
                cols = slice(cb * CB, (cb + 1) * CB)
                y = _nn(inv[:, :2 * C], _b(yb[rows, cols]))
                y2 = _nn(inv[:, 2 * C:], _b(yb[prev, cols]))
                y = y + jnp.where(c > 0, y2, 0.0)
                y = y + kv[rows, cols].astype(F32) * sd_ref[:, cols].astype(F32)
                _wo(ob)[rows, DM + cb * CB:DM + (cb + 1) * CB] = (bq[rows, cols].astype(F32) * y).astype(BF16)
            b_cp(c).start()
            return 0
        jax.lax.fori_loop(0, NC, binv, 0)
        wo_cp.wait()
        x_cp.wait()

    pl.run_scoped(phase1, pltpu.VMEM((16, 2, 512, 128), U32), pltpu.VMEM((NSEG * 4, DM), U32),
                  pltpu.VMEM((S, D), BF16), pltpu.VMEM((S, D), BF16), pltpu.VMEM((S, D), BF16),
                  pltpu.VMEM((D, S), BF16), pltpu.VMEM((C + 16, D), F32),
                  pltpu.VMEM((2 * S, D), F32), pltpu.VMEM((2 * S, D), F32), pltpu.VMEM((S, D), U32),
                  pltpu.SemaphoreType.DMA((16, 2)), pltpu.SemaphoreType.DMA((3, 4)),
                  pltpu.SemaphoreType.DMA((5,)))

    def phase2(o3):
        NG = H // GH

        def step(s, mem):
            odd = (s & 1) == 1
            allowed = mask_ref[s & 1] > 0.5
            r0 = pl.multiple_of(s * SEG, SEG)
            xs0 = xs[pl.ds(r0, 16), :].astype(F32)
            xs1 = xs[pl.ds(r0 + 16, 8), :].astype(F32)
            hb = jnp.concatenate([mem, xs1, xs0], 0).astype(BF16)
            jr = pl.ds(pl.multiple_of((s >> 1) * 8, 8), 8)
            o3v = _wo(o3.at[pl.ds(pl.multiple_of(s * 8, 8), 8), :])
            st = {}

            def do(op, g):
                if g < 0 or g >= NG:
                    return
                if op in 'qkv':
                    m = 'qkv'.index(op)
                    t = _nn(hb, _b(w3[m, :, g * GH * DH:(g + 1) * GH * DH]))
                for hh in range(GH):
                    h = g * GH + hh
                    hs = slice(h * DH, (h + 1) * DH)
                    ls = slice(hh * DH, (hh + 1) * DH)
                    if op == 'q':
                        q3 = qkv3[0, jr, hs]
                        st['q', h] = jnp.concatenate([t[:, ls], jnp.where(odd, _hi(q3), _lo(q3))], 0).astype(BF16)
                    elif op in 'kv':
                        st[op, h] = jnp.concatenate([_pe(t[0:8, ls], t[8:16, ls]), _pe(t[16:24, ls], t[24:32, ls]),
                                                     qkv3[m, jr, hs]], 0)
                    elif op == 'qk':
                        st['s', h] = _nt(st.pop(('q', h)), _b(st.pop(('k', h))))
                    elif op == 'sm':
                        sc = jnp.where(allowed[:, 0:48], st.pop(('s', h)) * c_exp, -1e9)
                        e = jnp.exp2(sc - jnp.max(sc, -1, keepdims=True))
                        st['p', h] = (e * (1.0 / jnp.sum(e, -1, keepdims=True))).astype(BF16)
                    else:
                        oh = _nn(st.pop(('p', h)), _b(st.pop(('v', h))))
                        st['o', h] = oh[0:32]
                        o3v[:, hs] = oh[32:40]
            r = None
            done = 0
            for g in range(NG + max(d for _, d in ORDER)):
                for op, d in ORDER:
                    do(op, g - d)
                for p, gmin in PARTS:
                    if g >= gmin and done < p and all(('o', h) in st for h in range(done, p)):
                        part = _nn(jnp.concatenate([st.pop(('o', h)) for h in range(done, p)], 1).astype(BF16),
                                   _b(wo[done * DH // 2:p * DH // 2, :]))
                        r = part if r is None else r + part
                        done = p
            rb = r.astype(BF16)
            ob[pl.ds(r0, 16), 0:DM] = rb[16:32]
            ob[pl.ds(r0 + 16, 8), 0:DM] = rb[8:16]
            return rb[0:8].astype(F32)
        jax.lax.fori_loop(0, NSEG, step, mem0_ref[...].astype(F32))

        ob3 = ob.reshape(NSEG, SEG, DM + D)
        out3 = out_h.reshape(NSEG, SEG, DM + D)
        a_cp = pltpu.make_async_copy(ob3.at[:, pl.ds(0, 24), pl.ds(0, DM)],
                                     out3.at[:, pl.ds(0, 24), pl.ds(0, DM)], osem.at[0])
        a_cp.start()

        def f_cp(n):
            return pltpu.make_async_copy(ob3.at[pl.ds(n * 16, 16), pl.ds(24, 8), pl.ds(0, DM)],
                                         out3.at[pl.ds(n * 16, 16), pl.ds(24, 8), pl.ds(0, DM)], osem.at[2])

        def fin(n, _):
            rows = pl.ds(pl.multiple_of(n * 128, 128), 128)
            r = _nn(o3[rows, :].astype(BF16), _b(wo[...]))
            for i in range(16):
                ob[pl.ds(pl.multiple_of(n * 512 + i * 32 + 24, 8), 8), 0:DM] = r[i * 8:(i + 1) * 8].astype(BF16)
            f_cp(n).start()
            return 0
        jax.lax.fori_loop(0, 4, fin, 0)
        a_cp.wait()
        for c in range(NC):
            b_cp(c).wait()
        for n in range(4):
            f_cp(n).wait()

    pl.run_scoped(phase2, pltpu.VMEM((NSEG * 8, HD), F32))


@functools.partial(jax.jit, static_argnames=("A_seg_len",))
def pallas_concat_heads__memory_aug_recurrent_mem_tr__ssm_conv_h3__prompt_kernel(
        A_x, A_mem0, A_Wq, A_Wk, A_Wv, A_Wo, A_seg_len, B_q, B_k, B_v, B_shift_k, B_ssm_k, B_ssm_D):
    assert int(A_seg_len) == SEG
    vm = pl.BlockSpec(memory_space=pltpu.VMEM)
    hbm = pl.BlockSpec(memory_space=pl.ANY)
    out = pl.pallas_call(
        _kernel,
        in_specs=[vm, hbm, hbm, hbm, hbm, hbm, hbm, hbm, hbm, vm, hbm, vm, vm, vm, vm],
        out_specs=hbm,
        out_shape=jax.ShapeDtypeStruct((S, DM + D), BF16),
        scratch_shapes=[pltpu.VMEM((3, 512, HD), U32), pltpu.VMEM((HD // 2, DM), U32),
                        pltpu.VMEM((S, DM), BF16), pltpu.VMEM((3, 256, HD), U32),
                        pltpu.VMEM((S, DM + D), BF16), pltpu.SemaphoreType.DMA((3,))],
        compiler_params=pltpu.CompilerParams(vmem_limit_bytes=126 * 1024 * 1024),
    )(A_mem0[0], A_Wq, A_Wk, A_Wv, A_Wo.reshape(HD, DM), A_x[0], B_q[0], B_k[0], B_v[0],
      B_shift_k.T, B_ssm_k, B_ssm_D.reshape(1, D),
      jnp.asarray(_FWD).astype(BF16), jnp.asarray(_INV).astype(BF16), jnp.asarray(_MASKS))
    return out[None]
```

```python
import functools
import numpy as np
import jax
import jax.numpy as jnp
import jax.experimental.pallas as pl
import jax.experimental.pallas.tpu as pltpu

S, DM, H, DH, M, D = 2048, 1024, 32, 128, 8, 1024
HD = H * DH
SEG = 32
NSEG = S // SEG
C = 128
NC = S // C
CW = C // 2
GH = 2
ORDER = (('q', 0), ('pv', 2), ('qk', 1), ('k', 0), ('v', 0), ('sm', 1))
PARTS = ((16, 0), (28, 16), (32, 0))
UF, UI = 4, 4
F32, BF16, U32 = jnp.float32, jnp.bfloat16, jnp.uint32
LOG2E = 1.4426950408889634


def _dft_consts():
    th = 2 * np.pi * (np.arange(C)[:, None] + 0.5) / (2 * C)
    n = np.arange(2 * C)[None, :]
    cos, sin = np.cos(th * n), np.sin(th * n)
    fwd = np.concatenate([cos[:, :C], -sin[:, :C]], 0)
    inv = np.concatenate([cos, -sin], 0).T / C
    perm = np.arange(2 * C).reshape(2, C).T.reshape(-1)
    inv = inv[:, perm]
    g = np.concatenate([inv[C:], inv[:C]], 1)
    rows = np.arange(C).reshape(C // 16, 8, 2).transpose(0, 2, 1).reshape(-1)
    g = g[rows]
    return fwd.astype(np.float32), g.astype(np.float32)


def _attn_masks():
    nat = np.array([-1] * 8 + list(range(16, 24)) + list(range(16)))
    qlab = np.concatenate([nat, np.arange(24, 32)])
    c = np.arange(16)
    inter = c // 2 + 8 * (c % 2)
    klab = np.concatenate([nat[:16][inter], nat[16:][inter], 24 + c // 2])
    out = np.zeros((2, 40, 128), np.float32)
    for par in range(2):
        valid = np.concatenate([np.ones(32, bool), c % 2 == par])
        ok = (qlab[:, None] < 0) | (klab[None, :] < 0) | (klab[None, :] <= qlab[:, None])
        out[par, :, :48] = ok & valid[None, :]
    return out


_FWD, _INV = _dft_consts()
_MASKS = _attn_masks()


def _nn(a, b):
    return jnp.dot(a, b, preferred_element_type=F32)


def _nt(a, b):
    return jax.lax.dot_general(a, b, (((1,), (1,)), ((), ())), preferred_element_type=F32)


def _b(x):
    return pltpu.bitcast(x, BF16)


def _pe(lo, hi):
    return pltpu.pack_elementwise([lo, hi], packed_dtype=BF16)


def _lo(w):
    return pltpu.bitcast(w << 16, F32)


def _hi(w):
    return pltpu.bitcast(w & jnp.uint32(0xffff0000), F32)


def _wo(ref):
    return pltpu.annotate(ref, no_hazard_no_deps=True)


def _kernel(mem0_ref, wq_h, wk_h, wv_h, wo_h, x_h, bq_h, bk_h, bv_h, sk_ref, ssmk_h, sd_ref,
            fwd_ref, inv_ref, mask_ref, out_h,
            w3, wo, xs, qkv3, ob, obb, osem):
    c_exp = DH ** -0.5 * LOG2E
    w_h = [r.bitcast(U32).reshape(DM // 2, 2, H // 2, DH) for r in (wq_h, wk_h, wv_h)]

    def b_cp(c):
        rows = pl.ds(pl.multiple_of(c * CW, CW), CW)
        return pltpu.make_async_copy(obb.at[rows], out_h.bitcast(U32).at[rows, pl.ds(DM, D)], osem.at[1])

    def phase1(slab, x3, bk, bq, kv, sk, xf, kf, yb, wsem, bsem, dsem):
        def slab_cp(m, hp, par):
            return pltpu.make_async_copy(w_h[m].at[:, par, hp, :], slab.at[hp, par], wsem.at[hp, par])
        x32 = x_h.bitcast(U32).reshape(NSEG // 2, 32, DM)
        x3d = x3.reshape(NSEG // 2, 8, DM)
        x3_cps = [pltpu.make_async_copy(x32.at[:, pl.ds(12 + 16 * p, 4), :], x3d.at[:, pl.ds(4 * p, 4), :],
                                        dsem.at[3 + p]) for p in range(2)]
        wo_cp = pltpu.make_async_copy(wo_h.bitcast(U32), wo, dsem.at[0])
        x_cp = pltpu.make_async_copy(x_h, xs, dsem.at[1])
        bq_cp = pltpu.make_async_copy(bq_h.bitcast(U32), bq, dsem.at[2])
        QB = NC // 4

        bk32, bv32 = bk_h.bitcast(U32), bv_h.bitcast(U32)

        def bin_cps(p):
            rows = pl.ds(p * QB * C, QB * C)
            wr = pl.ds(p * QB * CW, QB * CW)
            return [pltpu.make_async_copy(bk32.at[wr], bk.at[pl.ds(8 + p * QB * CW, QB * CW)], bsem.at[0, p]),
                    pltpu.make_async_copy(bv32.at[wr], kv.at[wr], bsem.at[1, p]),
                    pltpu.make_async_copy(ssmk_h.at[:, rows], sk.at[:, rows], bsem.at[2, p])]

        def unit_cps(m, qi):
            return [slab_cp(m, qi * 4 + hh, par) for hh in range(4) for par in range(2)]

        def start(cps):
            for cp in cps:
                cp.start()

        start(bin_cps(0))
        start(bin_cps(1))
        bk[0:8, :] = jnp.zeros((8, D), U32)
        yb[0:C, :] = jnp.zeros((C, D), U32)
        CB = 512

        def bfwd(cc, _):
          fwd = fwd_ref[...]
          for c in [cc * UF + t for t in range(UF)]:
            rows = pl.ds(pl.multiple_of(c * C, C), C)
            wrows = pl.ds(pl.multiple_of(c * CW, CW), CW)
            spec = pl.ds(pl.multiple_of(c * 2 * C, 2 * C), 2 * C)
            for cb in range(D // CB):
                cols = slice(cb * CB, (cb + 1) * CB)
                _wo(kf)[spec, cols] = _nt(fwd, sk[cols, rows])
                t0, t1, t2, t3 = [sk_ref[d:d + 1, cols].astype(F32) for d in range(4)]
                blk = bk[pl.ds(pl.multiple_of(c * CW, 8), CW + 8), cols]
                w0, w1, w2 = blk[8:], pltpu.roll(blk, 1, 0)[8:], pltpu.roll(blk, 2, 0)[8:]
                e0, o0, e1, o1, o2 = _lo(w0), _hi(w0), _lo(w1), _hi(w1), _hi(w2)
                v = kv[wrows, cols]
                kvw = _pe((e0 * t0 + o1 * t1 + e1 * t2 + o2 * t3) * _lo(v),
                          (o0 * t0 + e0 * t1 + o1 * t2 + e1 * t3) * _hi(v))
                _wo(kv)[wrows, cols] = kvw
                _wo(xf)[spec, cols] = _nn(fwd, _b(kvw))
          return 0
        for p in range(4):
            for cp in bin_cps(p):
                cp.wait()
            if p + 2 < 4:
                start(bin_cps(p + 2))
            elif p == 2:
                start(x3_cps)
                start(unit_cps(0, 0))
            else:
                start(unit_cps(0, 1))
                start(unit_cps(0, 2))
            jax.lax.fori_loop(p * QB // UF, (p + 1) * QB // UF, bfwd, 0)

        def products(u):
            fr = pl.multiple_of((u >> 3) * 8, 8)
            col = pl.ds(pl.multiple_of((u & 7) * 128, 128), 128)
            xv = xf.at[pl.ds(fr, 2 * S - C + 8), col]
            kw = kf.at[pl.ds(fr, 2 * S - C + 8), col]
            yv = _wo(yb.at[pl.ds(C + fr, S - C + 8), col])
            for i in range(NC):
                ar = ai = None
                for j in range(i + 1):
                    xo, ko = (i - j) * 2 * C, j * 2 * C
                    xr, xi = xv[xo:xo + 8, :], xv[xo + C:xo + C + 8, :]
                    kr, ki = kw[ko:ko + 8, :], kw[ko + C:ko + C + 8, :]
                    tr, ti = xr * kr - xi * ki, xr * ki + xi * kr
                    ar, ai = (tr, ti) if ar is None else (ar + tr, ai + ti)
                    if j == i:
                        yv[i * C:i * C + 8, :] = _pe(ar, ai)
                    yield

        for cp in x3_cps:
            cp.wait()
        start(unit_cps(0, 3))
        NST = 11

        def unit(un, _):
            m, qi = un >> 2, un & 3
            wm = w3.at[m]
            with jax.named_scope('z_wait'):
                for mm in range(3):
                    @pl.when(m == mm)
                    def _():
                        for hh in range(4):
                            slab_cp(mm, qi * 4 + hh, 0).wait()
                            slab_cp(mm, qi * 4 + hh, 1).wait()
            with jax.named_scope('z_relay'):
                sl = slab.at[pl.ds(qi * 4, 4)]
                wv = _wo(wm.at[:, pl.ds(pl.multiple_of(qi * 1024, 1024), 1024)])

                def body(i, _):
                    r = pl.ds(pl.multiple_of(i * 8, 8), 8)
                    for hh in range(4):
                        a, b = sl[hh, 0, r, :], sl[hh, 1, r, :]
                        wv[r, hh * 256:hh * 256 + 128] = (a & 0xffff) | (b << 16)
                        wv[r, hh * 256 + 128:hh * 256 + 256] = (a >> 16) | (b & jnp.uint32(0xffff0000))
                    return 0
                jax.lax.fori_loop(0, 64, body, 0, unroll=4)
            with jax.named_scope('z_start'):
                for mm in range(2):
                    @pl.when(m == mm)
                    def _():
                        for hh in range(4):
                            slab_cp(mm + 1, qi * 4 + hh, 0).start()
                            slab_cp(mm + 1, qi * 4 + hh, 1).start()

            @pl.when(un == 3)
            def _():
                bq_cp.start()

            @pl.when(un == 7)
            def _():
                wo_cp.start()
                x_cp.start()

            def strips():
                for t in range(NST):
                    yield from products(jnp.minimum(un * NST + t, 127))
            work = strips()
            per_dot = -(-NST * (NC * (NC + 1) // 2) // 32)
            wq = wm.at[:, pl.ds(pl.multiple_of(qi * 1024, 1024), 1024)]
            qo = _wo(qkv3.at[m].at[:, pl.ds(pl.multiple_of(qi * 1024, 1024), 1024)])
            def adv(k):
                for _ in range(k):
                    next(work, None)
            for mb in range(8):
                for n in range(8):
                    cols = slice(n * 128, (n + 1) * 128)
                    r = _nn(_b(x3[mb * 32:(mb + 1) * 32, :]), _b(wq[:, cols]))
                    for j in range(4):
                        qo[mb * 32 + 8 * j:mb * 32 + 8 * j + 8, cols] = _pe(r[16 * j:16 * j + 8],
                                                                            r[16 * j + 8:16 * j + 16])
                    adv(-(-per_dot // 2))
            for _ in work:
                pass
            return 0
        jax.lax.fori_loop(0, 12, unit, 0)

        bq_cp.wait()

        CB = 1024

        def binv(cc, _):
          inv = inv_ref[...]
          for c in [cc * UI + t for t in range(UI)]:
            wrows = pl.ds(pl.multiple_of(c * CW, CW), CW)
            for cb in range(D // CB):
                cols = slice(cb * CB, (cb + 1) * CB)
                y = _nn(inv, _b(yb[pl.ds(pl.multiple_of(c * C, C), 2 * C), cols]))
                dd = sd_ref[:, cols].astype(F32)
                kvw, qw = kv[wrows, cols], bq[wrows, cols]
                out = []
                for i in range(C // 16):
                    wr = slice(8 * i, 8 * i + 8)
                    ye = y[16 * i:16 * i + 8] + _lo(kvw[wr]) * dd
                    yo = y[16 * i + 8:16 * i + 16] + _hi(kvw[wr]) * dd
                    out.append(_pe(ye * _lo(qw[wr]), yo * _hi(qw[wr])))
                _wo(obb)[wrows, cols] = jnp.concatenate(out, 0)
          for t in range(UI):
              b_cp(cc * UI + t).start()
          return 0
        jax.lax.fori_loop(0, NC // UI, binv, 0)
        wo_cp.wait()
        x_cp.wait()

    pl.run_scoped(phase1, pltpu.VMEM((16, 2, 512, 128), U32), pltpu.VMEM((NSEG * 4, DM), U32),
                  pltpu.VMEM((S // 2 + 8, D), U32), pltpu.VMEM((S // 2, D), U32), pltpu.VMEM((S // 2, D), U32),
                  pltpu.VMEM((D, S), BF16),
                  pltpu.VMEM((2 * S, D), F32), pltpu.VMEM((2 * S, D), F32), pltpu.VMEM((S + C, D), U32),
                  pltpu.SemaphoreType.DMA((16, 2)), pltpu.SemaphoreType.DMA((3, 4)),
                  pltpu.SemaphoreType.DMA((5,)))

    def phase2(o3):
        NG = H // GH

        def step(s, mem):
            odd = (s & 1) == 1
            allowed = mask_ref[s & 1] > 0.5
            r0 = pl.multiple_of(s * SEG, SEG)
            xs0 = xs[pl.ds(r0, 16), :].astype(F32)
            xs1 = xs[pl.ds(r0 + 16, 8), :].astype(F32)
            hb = jnp.concatenate([mem, xs1, xs0], 0).astype(BF16)
            jr = pl.ds(pl.multiple_of((s >> 1) * 8, 8), 8)
            o3v = _wo(o3.at[pl.ds(pl.multiple_of(s * 8, 8), 8), :])
            st = {}

            def do(op, g):
                if g < 0 or g >= NG:
                    return
                if op in 'qkv':
                    m = 'qkv'.index(op)
                    t = _nn(hb, _b(w3[m, :, g * GH * DH:(g + 1) * GH * DH]))
                for hh in range(GH):
                    h = g * GH + hh
                    hs = slice(h * DH, (h + 1) * DH)
                    ls = slice(hh * DH, (hh + 1) * DH)
                    if op == 'q':
                        q3 = qkv3[0, jr, hs]
                        st['q', h] = jnp.concatenate([t[:, ls], jnp.where(odd, _hi(q3), _lo(q3))], 0).astype(BF16)
                    elif op in 'kv':
                        st[op, h] = jnp.concatenate([_pe(t[0:8, ls], t[8:16, ls]), _pe(t[16:24, ls], t[24:32, ls]),
                                                     qkv3[m, jr, hs]], 0)
                    elif op == 'qk':
                        st['s', h] = _nt(st.pop(('q', h)), _b(st.pop(('k', h))))
                    elif op == 'sm':
                        sc = jnp.where(allowed[:, 0:48], st.pop(('s', h)) * c_exp, -1e9)
                        e = jnp.exp2(sc - jnp.max(sc, -1, keepdims=True))
                        st['p', h] = (e * (1.0 / jnp.sum(e, -1, keepdims=True))).astype(BF16)
                    else:
                        oh = _nn(st.pop(('p', h)), _b(st.pop(('v', h))))
                        st['o', h] = oh[0:32]
                        o3v[:, hs] = oh[32:40]
            r = None
            done = 0
            for g in range(NG + max(d for _, d in ORDER)):
                for op, d in ORDER:
                    do(op, g - d)
                for p, gmin in PARTS:
                    if g >= gmin and done < p and all(('o', h) in st for h in range(done, p)):
                        part = _nn(jnp.concatenate([st.pop(('o', h)) for h in range(done, p)], 1).astype(BF16),
                                   _b(wo[done * DH // 2:p * DH // 2, :]))
                        r = part if r is None else r + part
                        done = p
            rb = r.astype(BF16)
            ob[pl.ds(r0, 16), :] = rb[16:32]
            ob[pl.ds(r0 + 16, 8), :] = rb[8:16]
            return rb[0:8].astype(F32)
        jax.lax.fori_loop(0, NSEG, step, mem0_ref[...].astype(F32))

        ob3 = ob.reshape(NSEG, SEG, DM)
        out3 = out_h.reshape(NSEG, SEG, DM + D)
        a_cp = pltpu.make_async_copy(ob3.at[:, pl.ds(0, 24), :],
                                     out3.at[:, pl.ds(0, 24), pl.ds(0, DM)], osem.at[0])
        a_cp.start()

        def f_cp(n):
            return pltpu.make_async_copy(ob3.at[pl.ds(n * 16, 16), pl.ds(24, 8), :],
                                         out3.at[pl.ds(n * 16, 16), pl.ds(24, 8), pl.ds(0, DM)], osem.at[2])

        def fin(n, _):
            rows = pl.ds(pl.multiple_of(n * 128, 128), 128)
            r = _nn(o3[rows, :].astype(BF16), _b(wo[...]))
            for i in range(16):
                ob[pl.ds(pl.multiple_of(n * 512 + i * 32 + 24, 8), 8), :] = r[i * 8:(i + 1) * 8].astype(BF16)
            f_cp(n).start()
            return 0
        jax.lax.fori_loop(0, 4, fin, 0)
        a_cp.wait()
        for c in range(NC):
            b_cp(c).wait()
        for n in range(4):
            f_cp(n).wait()

    pl.run_scoped(phase2, pltpu.VMEM((NSEG * 8, HD), F32))


@functools.partial(jax.jit, static_argnames=("A_seg_len",))
def pallas_concat_heads__memory_aug_recurrent_mem_tr__ssm_conv_h3__prompt_kernel(
        A_x, A_mem0, A_Wq, A_Wk, A_Wv, A_Wo, A_seg_len, B_q, B_k, B_v, B_shift_k, B_ssm_k, B_ssm_D):
    assert int(A_seg_len) == SEG
    vm = pl.BlockSpec(memory_space=pltpu.VMEM)
    hbm = pl.BlockSpec(memory_space=pl.ANY)
    out = pl.pallas_call(
        _kernel,
        in_specs=[vm, hbm, hbm, hbm, hbm, hbm, hbm, hbm, hbm, vm, hbm, vm, vm, vm, vm],
        out_specs=hbm,
        out_shape=jax.ShapeDtypeStruct((S, DM + D), BF16),
        scratch_shapes=[pltpu.VMEM((3, 512, HD), U32), pltpu.VMEM((HD // 2, DM), U32),
                        pltpu.VMEM((S, DM), BF16), pltpu.VMEM((3, 256, HD), U32),
                        pltpu.VMEM((S, DM), BF16), pltpu.VMEM((S // 2, D), U32), pltpu.SemaphoreType.DMA((3,))],
        compiler_params=pltpu.CompilerParams(vmem_limit_bytes=126 * 1024 * 1024),
    )(A_mem0[0], A_Wq, A_Wk, A_Wv, A_Wo.reshape(HD, DM), A_x[0], B_q[0], B_k[0], B_v[0],
      B_shift_k.T, B_ssm_k, B_ssm_D.reshape(1, D),
      jnp.asarray(_FWD).astype(BF16), jnp.asarray(_INV).astype(BF16), jnp.asarray(_MASKS))
    return out[None]
```

```python
import functools
import numpy as np
import jax
import jax.numpy as jnp
import jax.experimental.pallas as pl
import jax.experimental.pallas.tpu as pltpu

S, DM, H, DH, M, D = 2048, 1024, 32, 128, 8, 1024
HD = H * DH
SEG = 32
NSEG = S // SEG
C = 128
NC = S // C
CW = C // 2
GH = 2
ORDER = (('q', 0), ('pv', 2), ('qk', 1), ('k', 0), ('v', 0), ('sm', 1))
PARTS = ((16, 0), (28, 16), (32, 0))
UF, UI = 4, 4
F32, BF16, U32 = jnp.float32, jnp.bfloat16, jnp.uint32
LOG2E = 1.4426950408889634


def _dft_consts():
    th = 2 * np.pi * (np.arange(C)[:, None] + 0.5) / (2 * C)
    n = np.arange(2 * C)[None, :]
    cos, sin = np.cos(th * n), np.sin(th * n)
    fwd = np.concatenate([cos[:, :C], -sin[:, :C]], 0)
    inv = np.concatenate([cos, -sin], 0).T / C
    perm = np.arange(2 * C).reshape(2, C).T.reshape(-1)
    inv = inv[:, perm]
    g = np.concatenate([inv[C:], inv[:C]], 1)
    rows = np.arange(C).reshape(C // 16, 8, 2).transpose(0, 2, 1).reshape(-1)
    g = g[rows]
    return fwd.astype(np.float32), g.astype(np.float32)


def _attn_masks():
    nat = np.array([-1] * 8 + list(range(16, 24)) + list(range(16)))
    qlab = np.concatenate([nat, np.arange(24, 32)])
    c = np.arange(16)
    inter = c // 2 + 8 * (c % 2)
    klab = np.concatenate([nat[:16][inter], nat[16:][inter], 24 + c // 2])
    out = np.zeros((2, 40, 128), np.float32)
    for par in range(2):
        valid = np.concatenate([np.ones(32, bool), c % 2 == par])
        ok = (qlab[:, None] < 0) | (klab[None, :] < 0) | (klab[None, :] <= qlab[:, None])
        out[par, :, :48] = ok & valid[None, :]
    return out


_FWD, _INV = _dft_consts()
_MASKS = _attn_masks()


def _nn(a, b):
    return jnp.dot(a, b, preferred_element_type=F32)


def _nt(a, b):
    return jax.lax.dot_general(a, b, (((1,), (1,)), ((), ())), preferred_element_type=F32)


def _b(x):
    return pltpu.bitcast(x, BF16)


def _pe(lo, hi):
    return pltpu.pack_elementwise([lo, hi], packed_dtype=BF16)


def _lo(w):
    return pltpu.bitcast(w << 16, F32)


def _hi(w):
    return pltpu.bitcast(w & jnp.uint32(0xffff0000), F32)


def _wo(ref):
    return pltpu.annotate(ref, no_hazard_no_deps=True)


def _kernel(mem0_ref, wq_h, wk_h, wv_h, wo_h, x_h, bq_h, bk_h, bv_h, sk_ref, ssmk_h, sd_ref,
            fwd_ref, inv_ref, mask_ref, out_h,
            w3, wo, xs, qkv3, ob, obb, bq, kv, yb, osem):
    c_exp = DH ** -0.5 * LOG2E
    w_h = [r.bitcast(U32).reshape(DM // 2, 2, H // 2, DH) for r in (wq_h, wk_h, wv_h)]

    def b_cp(c):
        rows = pl.ds(pl.multiple_of(c * CW, CW), CW)
        return pltpu.make_async_copy(obb.at[rows], out_h.bitcast(U32).at[rows, pl.ds(DM, D)], osem.at[1])

    def phase1(slab, x3, bk, sk, xf, kf, wsem, bsem, dsem):
        def slab_cp(m, hp, par):
            return pltpu.make_async_copy(w_h[m].at[:, par, hp, :], slab.at[hp, par], wsem.at[hp, par])
        x32 = x_h.bitcast(U32).reshape(NSEG // 2, 32, DM)
        x3d = x3.reshape(NSEG // 2, 8, DM)
        x3_cps = [pltpu.make_async_copy(x32.at[:, pl.ds(12 + 16 * p, 4), :], x3d.at[:, pl.ds(4 * p, 4), :],
                                        dsem.at[3 + p]) for p in range(2)]
        wo_cp = pltpu.make_async_copy(wo_h.bitcast(U32), wo, dsem.at[0])
        x_cp = pltpu.make_async_copy(x_h, xs, dsem.at[1])
        bq_cp = pltpu.make_async_copy(bq_h.bitcast(U32), bq, dsem.at[2])
        QB = NC // 4

        bk32, bv32 = bk_h.bitcast(U32), bv_h.bitcast(U32)

        def bin_cps(p):
            rows = pl.ds(p * QB * C, QB * C)
            wr = pl.ds(p * QB * CW, QB * CW)
            return [pltpu.make_async_copy(bk32.at[wr], bk.at[pl.ds(8 + p * QB * CW, QB * CW)], bsem.at[0, p]),
                    pltpu.make_async_copy(bv32.at[wr], kv.at[wr], bsem.at[1, p]),
                    pltpu.make_async_copy(ssmk_h.at[:, rows], sk.at[:, rows], bsem.at[2, p])]

        def unit_cps(m, qi):
            return [slab_cp(m, qi * 4 + hh, par) for hh in range(4) for par in range(2)]

        def start(cps):
            for cp in cps:
                cp.start()

        start(x3_cps)
        start(unit_cps(0, 0))
        bk[0:8, :] = jnp.zeros((8, D), U32)
        yb[0:C, :] = jnp.zeros((C, D), U32)
        CB = 512

        def bfwd(cc, _):
          fwd = fwd_ref[...]
          for c in [cc * UF + t for t in range(UF)]:
            rows = pl.ds(pl.multiple_of(c * C, C), C)
            wrows = pl.ds(pl.multiple_of(c * CW, CW), CW)
            spec = pl.ds(pl.multiple_of(c * 2 * C, 2 * C), 2 * C)
            for cb in range(D // CB):
                cols = slice(cb * CB, (cb + 1) * CB)
                _wo(kf)[spec, cols] = _nt(fwd, sk[cols, rows])
                t0, t1, t2, t3 = [sk_ref[d:d + 1, cols].astype(F32) for d in range(4)]
                blk = bk[pl.ds(pl.multiple_of(c * CW, 8), CW + 8), cols]
                w0, w1, w2 = blk[8:], pltpu.roll(blk, 1, 0)[8:], pltpu.roll(blk, 2, 0)[8:]
                e0, o0, e1, o1, o2 = _lo(w0), _hi(w0), _lo(w1), _hi(w1), _hi(w2)
                v = kv[wrows, cols]
                kvw = _pe((e0 * t0 + o1 * t1 + e1 * t2 + o2 * t3) * _lo(v),
                          (o0 * t0 + e0 * t1 + o1 * t2 + e1 * t3) * _hi(v))
                _wo(kv)[wrows, cols] = kvw
                _wo(xf)[spec, cols] = _nn(fwd, _b(kvw))
          return 0
        def products(u):
            fr = pl.multiple_of((u >> 3) * 8, 8)
            col = pl.ds(pl.multiple_of((u & 7) * 128, 128), 128)
            xv = xf.at[pl.ds(fr, 2 * S - C + 8), col]
            kw = kf.at[pl.ds(fr, 2 * S - C + 8), col]
            yv = _wo(yb.at[pl.ds(C + fr, S - C + 8), col])
            for i in range(NC):
                ar = ai = None
                for j in range(i + 1):
                    xo, ko = (i - j) * 2 * C, j * 2 * C
                    xr, xi = xv[xo:xo + 8, :], xv[xo + C:xo + C + 8, :]
                    kr, ki = kw[ko:ko + 8, :], kw[ko + C:ko + C + 8, :]
                    tr, ti = xr * kr - xi * ki, xr * ki + xi * kr
                    ar, ai = (tr, ti) if ar is None else (ar + tr, ai + ti)
                    if j == i:
                        yv[i * C:i * C + 8, :] = _pe(ar, ai)
                    yield

        NPRE = 2
        NST = -(-128 // (12 - NPRE))

        def unit(un, _, with_products):
            m, qi = un >> 2, un & 3
            wm = w3.at[m]
            for mm in range(3 if with_products else 1):
                @pl.when(m == mm)
                def _():
                    for cp in unit_cps(mm, qi):
                        cp.wait()
            sl = slab.at[pl.ds(qi * 4, 4)]
            wv = _wo(wm.at[:, pl.ds(pl.multiple_of(qi * 1024, 1024), 1024)])

            def body(i, _):
                r = pl.ds(pl.multiple_of(i * 8, 8), 8)
                for hh in range(4):
                    a, b = sl[hh, 0, r, :], sl[hh, 1, r, :]
                    wv[r, hh * 256:hh * 256 + 128] = (a & 0xffff) | (b << 16)
                    wv[r, hh * 256 + 128:hh * 256 + 256] = (a >> 16) | (b & jnp.uint32(0xffff0000))
                return 0
            jax.lax.fori_loop(0, 64, body, 0, unroll=4)
            if with_products:
                for mm in range(2):
                    @pl.when(m == mm)
                    def _():
                        start(unit_cps(mm + 1, qi))

                @pl.when(un == 5)
                def _():
                    bq_cp.start()

                @pl.when(un == 8)
                def _():
                    wo_cp.start()
                    x_cp.start()
            else:
                @pl.when(un == 0)
                def _():
                    start(unit_cps(0, 1))
                    start(bin_cps(0))

                @pl.when(un == 1)
                def _():
                    start(bin_cps(1))
                    start(bin_cps(2))

            def strips():
                for t in range(NST if with_products else 0):
                    yield from products(jnp.minimum((un - NPRE) * NST + t, 127))
            work = strips()
            per_dot = -(-NST * (NC * (NC + 1) // 2) // 64)
            wq = wm.at[:, pl.ds(pl.multiple_of(qi * 1024, 1024), 1024)]
            qo = _wo(qkv3.at[m].at[:, pl.ds(pl.multiple_of(qi * 1024, 1024), 1024)])
            for mb in range(8):
                for n in range(8):
                    cols = slice(n * 128, (n + 1) * 128)
                    r = _nn(_b(x3[mb * 32:(mb + 1) * 32, :]), _b(wq[:, cols]))
                    for j in range(4):
                        qo[mb * 32 + 8 * j:mb * 32 + 8 * j + 8, cols] = _pe(r[16 * j:16 * j + 8],
                                                                            r[16 * j + 8:16 * j + 16])
                    for _ in range(per_dot):
                        next(work, None)
            for _ in work:
                pass
            return 0

        for cp in x3_cps:
            cp.wait()
        jax.lax.fori_loop(0, NPRE, functools.partial(unit, with_products=False), 0)
        for p in range(4):
            for cp in bin_cps(p):
                cp.wait()
            if p == 0:
                start(bin_cps(3))
            elif p == 1:
                start(unit_cps(0, 2))
                start(unit_cps(0, 3))
            elif p == 2:
                start(unit_cps(1, 0))
                start(unit_cps(1, 1))
            jax.lax.fori_loop(p * QB // UF, (p + 1) * QB // UF, bfwd, 0)
        jax.lax.fori_loop(NPRE, 12, functools.partial(unit, with_products=True), 0)

        bq_cp.wait()
        wo_cp.wait()
        x_cp.wait()

    pl.run_scoped(phase1, pltpu.VMEM((16, 2, 512, 128), U32), pltpu.VMEM((NSEG * 4, DM), U32),
                  pltpu.VMEM((S // 2 + 8, D), U32), pltpu.VMEM((D, S), BF16),
                  pltpu.VMEM((2 * S, D), F32), pltpu.VMEM((2 * S, D), F32),
                  pltpu.SemaphoreType.DMA((16, 2)), pltpu.SemaphoreType.DMA((3, 4)),
                  pltpu.SemaphoreType.DMA((5,)))

    def phase2(o3):
        NG = H // GH

        def step(s, mem, si):
            odd = si & 1 == 1
            allowed = mask_ref[si & 1] > 0.5
            r0 = pl.multiple_of(s * SEG, SEG)
            xs0 = xs[pl.ds(r0, 16), :].astype(F32)
            xs1 = xs[pl.ds(r0 + 16, 8), :].astype(F32)
            hb = jnp.concatenate([mem, xs1, xs0], 0).astype(BF16)
            jr = pl.ds(pl.multiple_of((s >> 1) * 8, 8), 8)
            o3v = _wo(o3.at[pl.ds(pl.multiple_of(s * 8, 8), 8), :])
            st = {}

            def do(op, g):
                if g < 0 or g >= NG:
                    return
                if op in 'qkv':
                    m = 'qkv'.index(op)
                    t = _nn(hb, _b(w3[m, :, g * GH * DH:(g + 1) * GH * DH]))
                for hh in range(GH):
                    h = g * GH + hh
                    hs = slice(h * DH, (h + 1) * DH)
                    ls = slice(hh * DH, (hh + 1) * DH)
                    if op == 'q':
                        q3 = qkv3[0, jr, hs]
                        st['q', h] = jnp.concatenate([t[:, ls], (_hi(q3) if odd else _lo(q3))], 0).astype(BF16)
                    elif op in 'kv':
                        st[op, h] = jnp.concatenate([_pe(t[0:8, ls], t[8:16, ls]), _pe(t[16:24, ls], t[24:32, ls]),
                                                     qkv3[m, jr, hs]], 0)
                    elif op == 'qk':
                        st['s', h] = _nt(st.pop(('q', h)), _b(st.pop(('k', h))))
                    elif op == 'sm':
                        sc = jnp.where(allowed[:, 0:48], st.pop(('s', h)) * c_exp, -1e9)
                        e = jnp.exp2(sc - jnp.max(sc, -1, keepdims=True))
                        st['p', h] = (e * (1.0 / jnp.sum(e, -1, keepdims=True))).astype(BF16)
                    else:
                        oh = _nn(st.pop(('p', h)), _b(st.pop(('v', h))))
                        st['o', h] = oh[0:32]
                        o3v[:, hs] = oh[32:40]
            r = None
            done = 0
            for g in range(NG + max(d for _, d in ORDER)):
                for op, d in ORDER:
                    do(op, g - d)
                for p, gmin in PARTS:
                    if g >= gmin and done < p and all(('o', h) in st for h in range(done, p)):
                        part = _nn(jnp.concatenate([st.pop(('o', h)) for h in range(done, p)], 1).astype(BF16),
                                   _b(wo[done * DH // 2:p * DH // 2, :]))
                        r = part if r is None else r + part
                        done = p
            c = s >> 2
            cols = pl.ds(pl.multiple_of((s & 3) * 256, 256), 256)
            wrows = pl.ds(pl.multiple_of(c * CW, CW), CW)
            y = _nn(inv_ref[...], _b(yb[pl.ds(pl.multiple_of(c * C, C), 2 * C), cols]))
            dd = sd_ref[:, cols].astype(F32)
            kvw, qw = kv[wrows, cols], bq[wrows, cols]
            out = []
            for i in range(C // 16):
                wr = slice(8 * i, 8 * i + 8)
                ye = y[16 * i:16 * i + 8] + _lo(kvw[wr]) * dd
                yo = y[16 * i + 8:16 * i + 16] + _hi(kvw[wr]) * dd
                out.append(_pe(ye * _lo(qw[wr]), yo * _hi(qw[wr])))
            _wo(obb)[wrows, cols] = jnp.concatenate(out, 0)
            rb = r.astype(BF16)
            ob[pl.ds(r0, 16), :] = rb[16:32]
            ob[pl.ds(r0 + 16, 8), :] = rb[8:16]

            if si == 1:
                @pl.when((s & 3) == 3)
                def _():
                    b_cp(c).start()
            return rb[0:8].astype(F32)
        def steps(t, mem):
            for i in range(2):
                mem = step(t * 2 + i, mem, i)
            return mem
        jax.lax.fori_loop(0, NSEG // 2, steps, mem0_ref[...].astype(F32))

        ob3 = ob.reshape(NSEG, SEG, DM)
        out3 = out_h.reshape(NSEG, SEG, DM + D)
        a_cp = pltpu.make_async_copy(ob3.at[:, pl.ds(0, 24), :],
                                     out3.at[:, pl.ds(0, 24), pl.ds(0, DM)], osem.at[0])
        a_cp.start()

        def f_cp(n):
            return pltpu.make_async_copy(ob3.at[pl.ds(n * 16, 16), pl.ds(24, 8), :],
                                         out3.at[pl.ds(n * 16, 16), pl.ds(24, 8), pl.ds(0, DM)], osem.at[2])

        def fin(n, _):
            rows = pl.ds(pl.multiple_of(n * 128, 128), 128)
            r = _nn(o3[rows, :].astype(BF16), _b(wo[...]))
            for i in range(16):
                ob[pl.ds(pl.multiple_of(n * 512 + i * 32 + 24, 8), 8), :] = r[i * 8:(i + 1) * 8].astype(BF16)
            f_cp(n).start()
            return 0
        jax.lax.fori_loop(0, 4, fin, 0)
        a_cp.wait()
        for c in range(NC):
            b_cp(c).wait()
        for n in range(4):
            f_cp(n).wait()

    pl.run_scoped(phase2, pltpu.VMEM((NSEG * 8, HD), F32))


@functools.partial(jax.jit, static_argnames=("A_seg_len",))
def pallas_concat_heads__memory_aug_recurrent_mem_tr__ssm_conv_h3__prompt_kernel(
        A_x, A_mem0, A_Wq, A_Wk, A_Wv, A_Wo, A_seg_len, B_q, B_k, B_v, B_shift_k, B_ssm_k, B_ssm_D):
    assert int(A_seg_len) == SEG
    vm = pl.BlockSpec(memory_space=pltpu.VMEM)
    hbm = pl.BlockSpec(memory_space=pl.ANY)
    out = pl.pallas_call(
        _kernel,
        in_specs=[vm, hbm, hbm, hbm, hbm, hbm, hbm, hbm, hbm, vm, hbm, vm, vm, vm, vm],
        out_specs=hbm,
        out_shape=jax.ShapeDtypeStruct((S, DM + D), BF16),
        scratch_shapes=[pltpu.VMEM((3, 512, HD), U32), pltpu.VMEM((HD // 2, DM), U32),
                        pltpu.VMEM((S, DM), BF16), pltpu.VMEM((3, 256, HD), U32),
                        pltpu.VMEM((S, DM), BF16), pltpu.VMEM((S // 2, D), U32),
                        pltpu.VMEM((S // 2, D), U32), pltpu.VMEM((S // 2, D), U32), pltpu.VMEM((S + C, D), U32),
                        pltpu.SemaphoreType.DMA((3,))],
        compiler_params=pltpu.CompilerParams(vmem_limit_bytes=126 * 1024 * 1024),
    )(A_mem0[0], A_Wq, A_Wk, A_Wv, A_Wo.reshape(HD, DM), A_x[0], B_q[0], B_k[0], B_v[0],
      B_shift_k.T, B_ssm_k, B_ssm_D.reshape(1, D),
      jnp.asarray(_FWD).astype(BF16), jnp.asarray(_INV).astype(BF16), jnp.asarray(_MASKS))
    return out[None]
```

```python
import functools
import numpy as np
import jax
import jax.numpy as jnp
import jax.experimental.pallas as pl
import jax.experimental.pallas.tpu as pltpu

S, DM, H, DH, M, D = 2048, 1024, 32, 128, 8, 1024
HD = H * DH
SEG = 32
NSEG = S // SEG
C = 128
NC = S // C
CW = C // 2
GH = 2
ORDER = (('q',0),('qk',1),('k',0),('pv',2),('v',0),('sm',1))
PARTS = ((16, 0), (28, 16), (32, 0))
UF, UI = 4, 4
F32, BF16, U32 = jnp.float32, jnp.bfloat16, jnp.uint32
LOG2E = 1.4426950408889634


def _dft_consts():
    th = 2 * np.pi * (np.arange(C)[:, None] + 0.5) / (2 * C)
    n = np.arange(2 * C)[None, :]
    cos, sin = np.cos(th * n), np.sin(th * n)
    fwd = np.concatenate([cos[:, :C], -sin[:, :C]], 0)
    inv = np.concatenate([cos, -sin], 0).T / C
    perm = np.arange(2 * C).reshape(2, C).T.reshape(-1)
    inv = inv[:, perm]
    g = inv[:C]
    rows = np.arange(C).reshape(C // 16, 8, 2).transpose(0, 2, 1).reshape(-1)
    g = g[rows]
    return fwd.astype(np.float32), g.astype(np.float32)


def _attn_masks():
    nat = np.array([-1] * 8 + list(range(16, 24)) + list(range(16)))
    qlab = np.concatenate([nat, np.arange(24, 32)])
    c = np.arange(16)
    inter = c // 2 + 8 * (c % 2)
    klab = np.concatenate([nat[:16][inter], nat[16:][inter], 24 + c // 2])
    out = np.zeros((2, 40, 128), np.float32)
    for par in range(2):
        valid = np.concatenate([np.ones(32, bool), c % 2 == par])
        ok = (qlab[:, None] < 0) | (klab[None, :] < 0) | (klab[None, :] <= qlab[:, None])
        out[par, :, :48] = ok & valid[None, :]
    return out


_FWD, _INV = _dft_consts()
_MASKS = _attn_masks()


def _nn(a, b):
    return jnp.dot(a, b, preferred_element_type=F32)


def _nt(a, b):
    return jax.lax.dot_general(a, b, (((1,), (1,)), ((), ())), preferred_element_type=F32)


def _b(x):
    return pltpu.bitcast(x, BF16)


def _pe(lo, hi):
    return pltpu.pack_elementwise([lo, hi], packed_dtype=BF16)


def _lo(w):
    return pltpu.bitcast(w << 16, F32)


def _hi(w):
    return pltpu.bitcast(w & jnp.uint32(0xffff0000), F32)


def _wo(ref):
    return pltpu.annotate(ref, no_hazard_no_deps=True)


def _kernel(mem0_ref, wq_h, wk_h, wv_h, wo_h, x_h, bq_h, bk_h, bv_h, sk_ref, ssmk_h, sd_ref,
            fwd_ref, inv_ref, mask_ref, out_h,
            w3, wo, xs, qkv3, ob, obb, bq, kv, yb, osem):
    c_exp = DH ** -0.5 * LOG2E
    w_h = [r.bitcast(U32).reshape(DM // 2, 2, H // 2, DH) for r in (wq_h, wk_h, wv_h)]

    def b_cp(c):
        rows = pl.ds(pl.multiple_of(c * CW, CW), CW)
        return pltpu.make_async_copy(obb.at[rows], out_h.bitcast(U32).at[rows, pl.ds(DM, D)], osem.at[1])

    def phase1(slab, x3, bk, sk, xf, kf, wsem, bsem, dsem):
        def slab_cp(m, hp, par):
            return pltpu.make_async_copy(w_h[m].at[:, par, hp, :], slab.at[hp, par], wsem.at[hp, par])
        x32 = x_h.bitcast(U32).reshape(NSEG // 2, 32, DM)
        x3d = x3.reshape(NSEG // 2, 8, DM)
        x3_cps = [pltpu.make_async_copy(x32.at[:, pl.ds(12 + 16 * p, 4), :], x3d.at[:, pl.ds(4 * p, 4), :],
                                        dsem.at[3 + p]) for p in range(2)]
        wo_cp = pltpu.make_async_copy(wo_h.bitcast(U32), wo, dsem.at[0])
        x_cp = pltpu.make_async_copy(x_h, xs, dsem.at[1])
        bq_cp = pltpu.make_async_copy(bq_h.bitcast(U32), bq, dsem.at[2])
        QB = NC // 4

        bk32, bv32 = bk_h.bitcast(U32), bv_h.bitcast(U32)

        def bin_cps(p):
            rows = pl.ds(p * QB * C, QB * C)
            wr = pl.ds(p * QB * CW, QB * CW)
            return [pltpu.make_async_copy(bk32.at[wr], bk.at[pl.ds(8 + p * QB * CW, QB * CW)], bsem.at[0, p]),
                    pltpu.make_async_copy(bv32.at[wr], kv.at[wr], bsem.at[1, p]),
                    pltpu.make_async_copy(ssmk_h.at[:, rows], sk.at[:, rows], bsem.at[2, p])]

        def unit_cps(m, qi):
            return [slab_cp(m, qi * 4 + hh, par) for hh in range(4) for par in range(2)]

        def start(cps):
            for cp in cps:
                cp.start()

        start(x3_cps)
        start(unit_cps(0, 0))
        bk[0:8, :] = jnp.zeros((8, D), U32)
        CB = 512

        def bfwd(cc, _):
          fwd = fwd_ref[...]
          for c in [cc * UF + t for t in range(UF)]:
            rows = pl.ds(pl.multiple_of(c * C, C), C)
            wrows = pl.ds(pl.multiple_of(c * CW, CW), CW)
            spec = pl.ds(pl.multiple_of(c * 2 * C, 2 * C), 2 * C)
            for cb in range(D // CB):
                cols = slice(cb * CB, (cb + 1) * CB)
                _wo(kf)[spec, cols] = _nt(fwd, sk[cols, rows])
                t0, t1, t2, t3 = [sk_ref[d:d + 1, cols].astype(F32) for d in range(4)]
                blk = bk[pl.ds(pl.multiple_of(c * CW, 8), CW + 8), cols]
                w0, w1, w2 = blk[8:], pltpu.roll(blk, 1, 0)[8:], pltpu.roll(blk, 2, 0)[8:]
                e0, o0, e1, o1, o2 = _lo(w0), _hi(w0), _lo(w1), _hi(w1), _hi(w2)
                v = kv[wrows, cols]
                kvw = _pe((e0 * t0 + o1 * t1 + e1 * t2 + o2 * t3) * _lo(v),
                          (o0 * t0 + e0 * t1 + o1 * t2 + e1 * t3) * _hi(v))
                _wo(kv)[wrows, cols] = kvw
                _wo(xf)[spec, cols] = _nn(fwd, _b(kvw))
          return 0
        def products(u):
            fr = pl.multiple_of((u >> 3) * 8, 8)
            col = pl.ds(pl.multiple_of((u & 7) * 128, 128), 128)
            xv = xf.at[pl.ds(fr, 2 * S - C + 8), col]
            kw = kf.at[pl.ds(fr, 2 * S - C + 8), col]
            yv = _wo(yb.at[pl.ds(fr, S - C + 8), col])
            sign = jax.lax.broadcasted_iota(U32, (8, 128), 0) << 31

            def flip(t):
                return pltpu.bitcast(pltpu.bitcast(t, U32) ^ sign, F32)
            prev = None
            for i in range(NC):
                ar = ai = None
                for j in range(i + 1):
                    xo, ko = (i - j) * 2 * C, j * 2 * C
                    xr, xi = xv[xo:xo + 8, :], xv[xo + C:xo + C + 8, :]
                    kr, ki = kw[ko:ko + 8, :], kw[ko + C:ko + C + 8, :]
                    tr, ti = xr * kr - xi * ki, xr * ki + xi * kr
                    ar, ai = (tr, ti) if ar is None else (ar + tr, ai + ti)
                    if j == i:
                        zr, zi = (ar, ai) if prev is None else (ar - flip(prev[1]), ai + flip(prev[0]))
                        yv[i * C:i * C + 8, :] = _pe(zr, zi)
                        prev = (ar, ai)
                    yield

        NPRE = 2
        NST = -(-128 // (12 - NPRE))

        def unit(un, _, with_products):
            m, qi = un >> 2, un & 3
            wm = w3.at[m]
            for mm in range(3 if with_products else 1):
                @pl.when(m == mm)
                def _():
                    for cp in unit_cps(mm, qi):
                        cp.wait()
            sl = slab.at[pl.ds(qi * 4, 4)]
            wv = _wo(wm.at[:, pl.ds(pl.multiple_of(qi * 1024, 1024), 1024)])

            def body(i, _):
                r = pl.ds(pl.multiple_of(i * 8, 8), 8)
                for hh in range(4):
                    a, b = sl[hh, 0, r, :], sl[hh, 1, r, :]
                    wv[r, hh * 256:hh * 256 + 128] = (a & 0xffff) | (b << 16)
                    wv[r, hh * 256 + 128:hh * 256 + 256] = (a >> 16) | (b & jnp.uint32(0xffff0000))
                return 0
            jax.lax.fori_loop(0, 64, body, 0, unroll=4)
            if with_products:
                for mm in range(2):
                    @pl.when(m == mm)
                    def _():
                        start(unit_cps(mm + 1, qi))

                @pl.when(un == 5)
                def _():
                    bq_cp.start()

                @pl.when(un == 8)
                def _():
                    wo_cp.start()
                    x_cp.start()
            else:
                @pl.when(un == 0)
                def _():
                    start(unit_cps(0, 1))
                    start(bin_cps(0))

                @pl.when(un == 1)
                def _():
                    start(bin_cps(1))
                    start(bin_cps(2))

            def strips():
                for t in range(NST if with_products else 0):
                    yield from products(jnp.minimum((un - NPRE) * NST + t, 127))
            work = strips()
            per_dot = -(-NST * (NC * (NC + 1) // 2) // 64)
            wq = wm.at[:, pl.ds(pl.multiple_of(qi * 1024, 1024), 1024)]
            qo = _wo(qkv3.at[m].at[:, pl.ds(pl.multiple_of(qi * 1024, 1024), 1024)])
            for mb in range(8):
                for n in range(8):
                    cols = slice(n * 128, (n + 1) * 128)
                    r = _nn(_b(x3[mb * 32:(mb + 1) * 32, :]), _b(wq[:, cols]))
                    for j in range(4):
                        qo[mb * 32 + 8 * j:mb * 32 + 8 * j + 8, cols] = _pe(r[16 * j:16 * j + 8],
                                                                            r[16 * j + 8:16 * j + 16])
                    for _ in range(per_dot):
                        next(work, None)
            for _ in work:
                pass
            return 0

        for cp in x3_cps:
            cp.wait()
        jax.lax.fori_loop(0, NPRE, functools.partial(unit, with_products=False), 0)
        for p in range(4):
            for cp in bin_cps(p):
                cp.wait()
            if p == 0:
                start(bin_cps(3))
            elif p == 1:
                start(unit_cps(0, 2))
                start(unit_cps(0, 3))
            elif p == 2:
                start(unit_cps(1, 0))
                start(unit_cps(1, 1))
            jax.lax.fori_loop(p * QB // UF, (p + 1) * QB // UF, bfwd, 0)
        jax.lax.fori_loop(NPRE, 12, functools.partial(unit, with_products=True), 0)

        bq_cp.wait()
        wo_cp.wait()
        x_cp.wait()

    pl.run_scoped(phase1, pltpu.VMEM((16, 2, 512, 128), U32), pltpu.VMEM((NSEG * 4, DM), U32),
                  pltpu.VMEM((S // 2 + 8, D), U32), pltpu.VMEM((D, S), BF16),
                  pltpu.VMEM((2 * S, D), F32), pltpu.VMEM((2 * S, D), F32),
                  pltpu.SemaphoreType.DMA((16, 2)), pltpu.SemaphoreType.DMA((3, 4)),
                  pltpu.SemaphoreType.DMA((5,)))

    def phase2(o3):
        NG = H // GH

        def step(s, mem, si):
            odd = si & 1 == 1
            allowed = mask_ref[si & 1] > 0.5
            r0 = pl.multiple_of(s * SEG, SEG)
            xs0 = xs[pl.ds(r0, 16), :].astype(F32)
            xs1 = xs[pl.ds(r0 + 16, 8), :].astype(F32)
            hb = jnp.concatenate([mem, xs1, xs0], 0).astype(BF16)
            jr = pl.ds(pl.multiple_of((s >> 1) * 8, 8), 8)
            o3v = _wo(o3.at[pl.ds(pl.multiple_of(s * 8, 8), 8), :])
            st = {}

            def do(op, g):
                if g < 0 or g >= NG:
                    return
                if op in 'qkv':
                    m = 'qkv'.index(op)
                    t = _nn(hb, _b(w3[m, :, g * GH * DH:(g + 1) * GH * DH]))
                for hh in range(GH):
                    h = g * GH + hh
                    hs = slice(h * DH, (h + 1) * DH)
                    ls = slice(hh * DH, (hh + 1) * DH)
                    if op == 'q':
                        q3 = qkv3[0, jr, hs]
                        st['q', h] = jnp.concatenate([t[:, ls], (_hi(q3) if odd else _lo(q3))], 0).astype(BF16)
                    elif op in 'kv':
                        st[op, h] = jnp.concatenate([_pe(t[0:8, ls], t[8:16, ls]), _pe(t[16:24, ls], t[24:32, ls]),
                                                     qkv3[m, jr, hs]], 0)
                    elif op == 'qk':
                        st['s', h] = _nt(st.pop(('q', h)), _b(st.pop(('k', h))))
                    elif op == 'sm':
                        sc = jnp.where(allowed[:, 0:48], st.pop(('s', h)) * c_exp, -1e9)
                        e = jnp.exp2(sc - jnp.max(sc, -1, keepdims=True))
                        st['p', h] = (e * (1.0 / jnp.sum(e, -1, keepdims=True))).astype(BF16)
                    else:
                        oh = _nn(st.pop(('p', h)), _b(st.pop(('v', h))))
                        st['o', h] = oh[0:32]
                        o3v[:, hs] = oh[32:40]
            r = None
            done = 0
            for g in range(NG + max(d for _, d in ORDER)):
                for op, d in ORDER:
                    do(op, g - d)
                for p, gmin in PARTS:
                    if g >= gmin and done < p and all(('o', h) in st for h in range(done, p)):
                        part = _nn(jnp.concatenate([st.pop(('o', h)) for h in range(done, p)], 1).astype(BF16),
                                   _b(wo[done * DH // 2:p * DH // 2, :]))
                        r = part if r is None else r + part
                        done = p
            c = s >> 2
            cols = pl.ds(pl.multiple_of((s & 3) * 256, 256), 256)
            wrows = pl.ds(pl.multiple_of(c * CW, CW), CW)
            y = _nn(inv_ref[...], _b(yb[pl.ds(pl.multiple_of(c * C, C), C), cols]))
            dd = sd_ref[:, cols].astype(F32)
            kvw, qw = kv[wrows, cols], bq[wrows, cols]
            out = []
            for i in range(C // 16):
                wr = slice(8 * i, 8 * i + 8)
                ye = y[16 * i:16 * i + 8] + _lo(kvw[wr]) * dd
                yo = y[16 * i + 8:16 * i + 16] + _hi(kvw[wr]) * dd
                out.append(_pe(ye * _lo(qw[wr]), yo * _hi(qw[wr])))
            _wo(obb)[wrows, cols] = jnp.concatenate(out, 0)
            rb = r.astype(BF16)
            ob[pl.ds(r0, 16), :] = rb[16:32]
            ob[pl.ds(r0 + 16, 8), :] = rb[8:16]

            if si == 1:
                @pl.when((s & 3) == 3)
                def _():
                    b_cp(c).start()
            return rb[0:8].astype(F32)
        def steps(t, mem):
            for i in range(2):
                mem = step(t * 2 + i, mem, i)
            return mem
        jax.lax.fori_loop(0, NSEG // 2, steps, mem0_ref[...].astype(F32))

        ob3 = ob.reshape(NSEG, SEG, DM)
        out3 = out_h.reshape(NSEG, SEG, DM + D)
        a_cp = pltpu.make_async_copy(ob3.at[:, pl.ds(0, 24), :],
                                     out3.at[:, pl.ds(0, 24), pl.ds(0, DM)], osem.at[0])
        a_cp.start()

        def f_cp(n):
            return pltpu.make_async_copy(ob3.at[pl.ds(n * 16, 16), pl.ds(24, 8), :],
                                         out3.at[pl.ds(n * 16, 16), pl.ds(24, 8), pl.ds(0, DM)], osem.at[2])

        def fin(n, _):
            rows = pl.ds(pl.multiple_of(n * 128, 128), 128)
            r = _nn(o3[rows, :].astype(BF16), _b(wo[...]))
            for i in range(16):
                ob[pl.ds(pl.multiple_of(n * 512 + i * 32 + 24, 8), 8), :] = r[i * 8:(i + 1) * 8].astype(BF16)
            f_cp(n).start()
            return 0
        jax.lax.fori_loop(0, 4, fin, 0)
        a_cp.wait()
        for c in range(NC):
            b_cp(c).wait()
        for n in range(4):
            f_cp(n).wait()

    pl.run_scoped(phase2, pltpu.VMEM((NSEG * 8, HD), F32))


@functools.partial(jax.jit, static_argnames=("A_seg_len",))
def pallas_concat_heads__memory_aug_recurrent_mem_tr__ssm_conv_h3__prompt_kernel(
        A_x, A_mem0, A_Wq, A_Wk, A_Wv, A_Wo, A_seg_len, B_q, B_k, B_v, B_shift_k, B_ssm_k, B_ssm_D):
    assert int(A_seg_len) == SEG
    vm = pl.BlockSpec(memory_space=pltpu.VMEM)
    hbm = pl.BlockSpec(memory_space=pl.ANY)
    out = pl.pallas_call(
        _kernel,
        in_specs=[vm, hbm, hbm, hbm, hbm, hbm, hbm, hbm, hbm, vm, hbm, vm, vm, vm, vm],
        out_specs=hbm,
        out_shape=jax.ShapeDtypeStruct((S, DM + D), BF16),
        scratch_shapes=[pltpu.VMEM((3, 512, HD), U32), pltpu.VMEM((HD // 2, DM), U32),
                        pltpu.VMEM((S, DM), BF16), pltpu.VMEM((3, 256, HD), U32),
                        pltpu.VMEM((S, DM), BF16), pltpu.VMEM((S // 2, D), U32),
                        pltpu.VMEM((S // 2, D), U32), pltpu.VMEM((S // 2, D), U32), pltpu.VMEM((S, D), U32),
                        pltpu.SemaphoreType.DMA((3,))],
        compiler_params=pltpu.CompilerParams(vmem_limit_bytes=126 * 1024 * 1024),
    )(A_mem0[0], A_Wq, A_Wk, A_Wv, A_Wo.reshape(HD, DM), A_x[0], B_q[0], B_k[0], B_v[0],
      B_shift_k.T, B_ssm_k, B_ssm_D.reshape(1, D),
      jnp.asarray(_FWD).astype(BF16), jnp.asarray(_INV).astype(BF16), jnp.asarray(_MASKS))
    return out[None]
```

```python
import functools
import numpy as np
import jax
import jax.numpy as jnp
import jax.experimental.pallas as pl
import jax.experimental.pallas.tpu as pltpu

S, DM, H, DH, M, D = 2048, 1024, 32, 128, 8, 1024
HD = H * DH
SEG = 32
NSEG = S // SEG
C = 128
NC = S // C
CW = C // 2
GH = 2
ORDER = (('qk',1),('pv',2),('k',0),('pv3',3),('q',0),('v',0),('sm3',2),('qk3',1),('sm',1))
PARTS = ((16,0),(22,16),(30,17),(32,0))
UF, UI = 4, 4
F32, BF16, U32 = jnp.float32, jnp.bfloat16, jnp.uint32
LOG2E = 1.4426950408889634


def _dft_consts():
    th = 2 * np.pi * (np.arange(C)[:, None] + 0.5) / (2 * C)
    n = np.arange(2 * C)[None, :]
    cos, sin = np.cos(th * n), np.sin(th * n)
    fwd = np.concatenate([cos[:, :C], -sin[:, :C]], 0)
    inv = np.concatenate([cos, -sin], 0).T / C
    perm = np.arange(2 * C).reshape(2, C).T.reshape(-1)
    inv = inv[:, perm]
    g = inv[:C]
    rows = np.arange(C).reshape(C // 16, 8, 2).transpose(0, 2, 1).reshape(-1)
    g = g[rows]
    return fwd.astype(np.float32), g.astype(np.float32)


def _attn_masks():
    nat = np.array([-1] * 8 + list(range(16, 24)) + list(range(16)))
    c = np.arange(16)
    inter = c // 2 + 8 * (c % 2)
    klab = np.concatenate([nat[:16][inter], nat[16:][inter], 24 + c // 2])
    out = np.zeros((80, 128), np.float32)
    for par in range(2):
        valid = np.concatenate([np.ones(32, bool), c % 2 == par])
        ok = (nat[:, None] < 0) | (klab[None, :] < 0) | (klab[None, :] <= nat[:, None])
        out[32 * par:32 * par + 32, :48] = ok & valid[None, :]
    for r in range(16):
        par, i = r % 2, r // 2
        out[64 + r, 32 * par:32 * par + 32] = 1
        out[64 + r, 64:80] = (c % 2 == par) & (c // 2 <= i)
    return out


_FWD, _INV = _dft_consts()
_MASKS = _attn_masks()


def _nn(a, b):
    return jnp.dot(a, b, preferred_element_type=F32)


def _nt(a, b):
    return jax.lax.dot_general(a, b, (((1,), (1,)), ((), ())), preferred_element_type=F32)


def _b(x):
    return pltpu.bitcast(x, BF16)


def _pe(lo, hi):
    return pltpu.pack_elementwise([lo, hi], packed_dtype=BF16)


def _lo(w):
    return pltpu.bitcast(w << 16, F32)


def _hi(w):
    return pltpu.bitcast(w & jnp.uint32(0xffff0000), F32)


def _wo(ref):
    return pltpu.annotate(ref, no_hazard_no_deps=True)


def _kernel(mem0_ref, wq_h, wk_h, wv_h, wo_h, x_h, bq_h, bk_h, bv_h, sk_ref, ssmk_h, sd_ref,
            fwd_ref, inv_ref, mask_ref, out_h,
            w3, wo, xs, qkv3, ob, obb, bq, kv, yb, osem):
    c_exp = DH ** -0.5 * LOG2E
    w_h = [r.bitcast(U32).reshape(DM // 2, 2, H // 2, DH) for r in (wq_h, wk_h, wv_h)]

    def b_cp(c):
        rows = pl.ds(pl.multiple_of(c * CW, CW), CW)
        return pltpu.make_async_copy(obb.at[rows], out_h.bitcast(U32).at[rows, pl.ds(DM, D)], osem.at[1])

    def phase1(slab, x3, bk, sk, xf, kf, wsem, bsem, dsem):
        def slab_cp(m, hp, par):
            return pltpu.make_async_copy(w_h[m].at[:, par, hp, :], slab.at[hp, par], wsem.at[hp, par])
        x32 = x_h.bitcast(U32).reshape(NSEG // 2, 32, DM)
        x3d = x3.reshape(NSEG // 2, 8, DM)
        x3_cps = [pltpu.make_async_copy(x32.at[:, pl.ds(12 + 16 * p, 4), :], x3d.at[:, pl.ds(4 * p, 4), :],
                                        dsem.at[3 + p]) for p in range(2)]
        wo_cp = pltpu.make_async_copy(wo_h.bitcast(U32), wo, dsem.at[0])
        x_cp = pltpu.make_async_copy(x_h, xs, dsem.at[1])
        bq_cp = pltpu.make_async_copy(bq_h.bitcast(U32), bq, dsem.at[2])
        QB = NC // 4

        bk32, bv32 = bk_h.bitcast(U32), bv_h.bitcast(U32)

        def bin_cps(p):
            rows = pl.ds(p * QB * C, QB * C)
            wr = pl.ds(p * QB * CW, QB * CW)
            return [pltpu.make_async_copy(bk32.at[wr], bk.at[pl.ds(8 + p * QB * CW, QB * CW)], bsem.at[0, p]),
                    pltpu.make_async_copy(bv32.at[wr], kv.at[wr], bsem.at[1, p]),
                    pltpu.make_async_copy(ssmk_h.at[:, rows], sk.at[:, rows], bsem.at[2, p])]

        def unit_cps(m, qi):
            return [slab_cp(m, qi * 4 + hh, par) for hh in range(4) for par in range(2)]

        def start(cps):
            for cp in cps:
                cp.start()

        start(x3_cps)
        start(unit_cps(0, 0))
        bk[0:8, :] = jnp.zeros((8, D), U32)
        CB = 512

        def bfwd(cc, _):
          fwd = fwd_ref[...]
          for c in [cc * UF + t for t in range(UF)]:
            rows = pl.ds(pl.multiple_of(c * C, C), C)
            wrows = pl.ds(pl.multiple_of(c * CW, CW), CW)
            spec = pl.ds(pl.multiple_of(c * 2 * C, 2 * C), 2 * C)
            for cb in range(D // CB):
                cols = slice(cb * CB, (cb + 1) * CB)
                _wo(kf)[spec, cols] = _nt(fwd, sk[cols, rows])
                t0, t1, t2, t3 = [sk_ref[d:d + 1, cols].astype(F32) for d in range(4)]
                blk = bk[pl.ds(pl.multiple_of(c * CW, 8), CW + 8), cols]
                w0, w1, w2 = blk[8:], pltpu.roll(blk, 1, 0)[8:], pltpu.roll(blk, 2, 0)[8:]
                e0, o0, e1, o1, o2 = _lo(w0), _hi(w0), _lo(w1), _hi(w1), _hi(w2)
                v = kv[wrows, cols]
                kvw = _pe((e0 * t0 + o1 * t1 + e1 * t2 + o2 * t3) * _lo(v),
                          (o0 * t0 + e0 * t1 + o1 * t2 + e1 * t3) * _hi(v))
                _wo(kv)[wrows, cols] = kvw
                _wo(xf)[spec, cols] = _nn(fwd, _b(kvw))
          return 0
        def products(u):
            fr = pl.multiple_of((u >> 3) * 8, 8)
            col = pl.ds(pl.multiple_of((u & 7) * 128, 128), 128)
            xv = xf.at[pl.ds(fr, 2 * S - C + 8), col]
            kw = kf.at[pl.ds(fr, 2 * S - C + 8), col]
            yv = _wo(yb.at[pl.ds(fr, S - C + 8), col])
            sign = jax.lax.broadcasted_iota(U32, (8, 128), 0) << 31

            def flip(t):
                return pltpu.bitcast(pltpu.bitcast(t, U32) ^ sign, F32)
            prev = None
            for i in range(NC):
                ar = ai = None
                for j in range(i + 1):
                    xo, ko = (i - j) * 2 * C, j * 2 * C
                    xr, xi = xv[xo:xo + 8, :], xv[xo + C:xo + C + 8, :]
                    kr, ki = kw[ko:ko + 8, :], kw[ko + C:ko + C + 8, :]
                    tr, ti = xr * kr - xi * ki, xr * ki + xi * kr
                    ar, ai = (tr, ti) if ar is None else (ar + tr, ai + ti)
                    if j == i:
                        zr, zi = (ar, ai) if prev is None else (ar - flip(prev[1]), ai + flip(prev[0]))
                        yv[i * C:i * C + 8, :] = _pe(zr, zi)
                        prev = (ar, ai)
                    yield

        NPRE = 2
        NST = -(-128 // (12 - NPRE))

        def unit(un, _, with_products):
            m, qi = un >> 2, un & 3
            wm = w3.at[m]
            for mm in range(3 if with_products else 1):
                @pl.when(m == mm)
                def _():
                    for cp in unit_cps(mm, qi):
                        cp.wait()
            sl = slab.at[pl.ds(qi * 4, 4)]
            wv = _wo(wm.at[:, pl.ds(pl.multiple_of(qi * 1024, 1024), 1024)])

            def body(i, _):
                r = pl.ds(pl.multiple_of(i * 8, 8), 8)
                for hh in range(4):
                    a, b = sl[hh, 0, r, :], sl[hh, 1, r, :]
                    wv[r, hh * 256:hh * 256 + 128] = (a & 0xffff) | (b << 16)
                    wv[r, hh * 256 + 128:hh * 256 + 256] = (a >> 16) | (b & jnp.uint32(0xffff0000))
                return 0
            jax.lax.fori_loop(0, 64, body, 0, unroll=4)
            if with_products:
                for mm in range(2):
                    @pl.when(m == mm)
                    def _():
                        start(unit_cps(mm + 1, qi))

                @pl.when(un == 5)
                def _():
                    bq_cp.start()

                @pl.when(un == 8)
                def _():
                    wo_cp.start()
                    x_cp.start()
            else:
                @pl.when(un == 0)
                def _():
                    start(unit_cps(0, 1))
                    start(bin_cps(0))

                @pl.when(un == 1)
                def _():
                    start(bin_cps(1))
                    start(bin_cps(2))

            def strips():
                for t in range(NST if with_products else 0):
                    yield from products(jnp.minimum((un - NPRE) * NST + t, 127))
            work = strips()
            per_dot = -(-NST * (NC * (NC + 1) // 2) // 64)
            wq = wm.at[:, pl.ds(pl.multiple_of(qi * 1024, 1024), 1024)]
            qo = _wo(qkv3.at[m].at[:, pl.ds(pl.multiple_of(qi * 1024, 1024), 1024)])
            for mb in range(8):
                for n in range(8):
                    cols = slice(n * 128, (n + 1) * 128)
                    r = _nn(_b(x3[mb * 32:(mb + 1) * 32, :]), _b(wq[:, cols]))
                    for j in range(4):
                        qo[mb * 32 + 8 * j:mb * 32 + 8 * j + 8, cols] = _pe(r[16 * j:16 * j + 8],
                                                                            r[16 * j + 8:16 * j + 16])
                    for _ in range(per_dot):
                        next(work, None)
            for _ in work:
                pass
            return 0

        for cp in x3_cps:
            cp.wait()
        jax.lax.fori_loop(0, NPRE, functools.partial(unit, with_products=False), 0)
        for p in range(4):
            for cp in bin_cps(p):
                cp.wait()
            if p == 0:
                start(bin_cps(3))
            elif p == 1:
                start(unit_cps(0, 2))
                start(unit_cps(0, 3))
            elif p == 2:
                start(unit_cps(1, 0))
                start(unit_cps(1, 1))
            jax.lax.fori_loop(p * QB // UF, (p + 1) * QB // UF, bfwd, 0)
        jax.lax.fori_loop(NPRE, 12, functools.partial(unit, with_products=True), 0)

        bq_cp.wait()
        wo_cp.wait()
        x_cp.wait()

    pl.run_scoped(phase1, pltpu.VMEM((16, 2, 512, 128), U32), pltpu.VMEM((NSEG * 4, DM), U32),
                  pltpu.VMEM((S // 2 + 8, D), U32), pltpu.VMEM((D, S), BF16),
                  pltpu.VMEM((2 * S, D), F32), pltpu.VMEM((2 * S, D), F32),
                  pltpu.SemaphoreType.DMA((16, 2)), pltpu.SemaphoreType.DMA((3, 4)),
                  pltpu.SemaphoreType.DMA((5,)))

    def phase2(o3):
        NG = H // GH

        def softmax(sc, allowed):
            sc = jnp.where(allowed, sc * c_exp, -1e9)
            e = jnp.exp2(sc - jnp.max(sc, -1, keepdims=True))
            return (e * (1.0 / jnp.sum(e, -1, keepdims=True))).astype(BF16)

        def step(s, mem, si, keep):
            allowed = mask_ref[32 * si:32 * si + 32, 0:48] > 0.5
            allowed3 = mask_ref[64:80, 0:80] > 0.5
            r0 = pl.multiple_of(s * SEG, SEG)
            xs0 = xs[pl.ds(r0, 16), :].astype(F32)
            xs1 = xs[pl.ds(r0 + 16, 8), :].astype(F32)
            hb = jnp.concatenate([mem, xs1, xs0], 0).astype(BF16)
            jr = pl.ds(pl.multiple_of((s >> 1) * 8, 8), 8)
            o3v = _wo(o3.at[pl.ds(pl.multiple_of((s >> 1) * 16, 16), 16), :])
            st = {}

            def do(op, g):
                if g < 0 or g >= NG or (op[-1] == '3' and si == 0):
                    return
                if op in 'qkv':
                    m = 'qkv'.index(op)
                    t = _nn(hb, _b(w3[m, :, g * GH * DH:(g + 1) * GH * DH]))
                for hh in range(GH):
                    h = g * GH + hh
                    hs = slice(h * DH, (h + 1) * DH)
                    ls = slice(hh * DH, (hh + 1) * DH)
                    if op == 'q':
                        st['q', h] = t[:, ls].astype(BF16)
                    elif op in 'kv':
                        two = [_pe(t[0:8, ls], t[8:16, ls]), _pe(t[16:24, ls], t[24:32, ls])]
                        st[op, h] = jnp.concatenate(two + [qkv3[m, jr, hs]], 0)
                        if si == 0:
                            keep[op, h] = two
                        else:
                            st[op + '3', h] = jnp.concatenate(keep.pop((op, h)) + two + [qkv3[m, jr, hs]], 0)
                    elif op == 'qk':
                        st['s', h] = _nt(st.pop(('q', h)), _b(st.pop(('k', h))))
                    elif op == 'sm':
                        st['p', h] = softmax(st.pop(('s', h)), allowed)
                    elif op == 'pv':
                        st['o', h] = _nn(st.pop(('p', h)), _b(st.pop(('v', h))))
                    elif op == 'qk3':
                        st['s3', h] = _nt(_b(qkv3[0, jr, hs]), _b(st.pop(('k3', h))))
                    elif op == 'sm3':
                        st['p3', h] = softmax(st.pop(('s3', h)), allowed3)
                    else:
                        o3v[:, hs] = _nn(st.pop(('p3', h)), _b(st.pop(('v3', h))))
            r = None
            done = 0
            order = ORDER
            for g in range(NG + max(d for _, d in order)):
                for op, d in order:
                    do(op, g - d)
                for p, gmin in PARTS:
                    if g >= gmin and done < p and all(('o', h) in st for h in range(done, p)):
                        part = _nn(jnp.concatenate([st.pop(('o', h)) for h in range(done, p)], 1).astype(BF16),
                                   _b(wo[done * DH // 2:p * DH // 2, :]))
                        r = part if r is None else r + part
                        done = p
            c = s >> 2
            cols = pl.ds(pl.multiple_of((s & 3) * 256, 256), 256)
            wrows = pl.ds(pl.multiple_of(c * CW, CW), CW)
            y = _nn(inv_ref[...], _b(yb[pl.ds(pl.multiple_of(c * C, C), C), cols]))
            dd = sd_ref[:, cols].astype(F32)
            kvw, qw = kv[wrows, cols], bq[wrows, cols]
            out = []
            for i in range(C // 16):
                wr = slice(8 * i, 8 * i + 8)
                ye = y[16 * i:16 * i + 8] + _lo(kvw[wr]) * dd
                yo = y[16 * i + 8:16 * i + 16] + _hi(kvw[wr]) * dd
                out.append(_pe(ye * _lo(qw[wr]), yo * _hi(qw[wr])))
            _wo(obb)[wrows, cols] = jnp.concatenate(out, 0)
            rb = r.astype(BF16)
            ob[pl.ds(r0, 16), :] = rb[16:32]
            ob[pl.ds(r0 + 16, 8), :] = rb[8:16]

            if si == 1:
                @pl.when((s & 3) == 3)
                def _():
                    b_cp(c).start()
            return rb[0:8].astype(F32)
        def steps(t, mem):
            keep = {}
            for i in range(2):
                mem = step(t * 2 + i, mem, i, keep)
            return mem
        jax.lax.fori_loop(0, NSEG // 2, steps, mem0_ref[...].astype(F32))

        ob3 = ob.reshape(NSEG, SEG, DM)
        out3 = out_h.reshape(NSEG, SEG, DM + D)
        a_cp = pltpu.make_async_copy(ob3.at[:, pl.ds(0, 24), :],
                                     out3.at[:, pl.ds(0, 24), pl.ds(0, DM)], osem.at[0])
        a_cp.start()

        def f_cp(n):
            return pltpu.make_async_copy(ob3.at[pl.ds(n * 16, 16), pl.ds(24, 8), :],
                                         out3.at[pl.ds(n * 16, 16), pl.ds(24, 8), pl.ds(0, DM)], osem.at[2])

        def fin(n, _):
            rows = pl.ds(pl.multiple_of(n * 128, 128), 128)
            r = _nn(o3[rows, :].astype(BF16), _b(wo[...]))
            w = pltpu.bitcast(r.astype(BF16), U32)
            for i in range(8):
                wi = w[i * 8:(i + 1) * 8]
                for half, val in ((0, _lo(wi)), (1, _hi(wi))):
                    ob[pl.ds(pl.multiple_of(n * 512 + i * 64 + half * 32 + 24, 8), 8), :] = val.astype(BF16)
            f_cp(n).start()
            return 0
        jax.lax.fori_loop(0, 4, fin, 0)
        a_cp.wait()
        for c in range(NC):
            b_cp(c).wait()
        for n in range(4):
            f_cp(n).wait()

    pl.run_scoped(phase2, pltpu.VMEM((NSEG * 8, HD), F32))


@functools.partial(jax.jit, static_argnames=("A_seg_len",))
def pallas_concat_heads__memory_aug_recurrent_mem_tr__ssm_conv_h3__prompt_kernel(
        A_x, A_mem0, A_Wq, A_Wk, A_Wv, A_Wo, A_seg_len, B_q, B_k, B_v, B_shift_k, B_ssm_k, B_ssm_D):
    assert int(A_seg_len) == SEG
    vm = pl.BlockSpec(memory_space=pltpu.VMEM)
    hbm = pl.BlockSpec(memory_space=pl.ANY)
    out = pl.pallas_call(
        _kernel,
        in_specs=[vm, hbm, hbm, hbm, hbm, hbm, hbm, hbm, hbm, vm, hbm, vm, vm, vm, vm],
        out_specs=hbm,
        out_shape=jax.ShapeDtypeStruct((S, DM + D), BF16),
        scratch_shapes=[pltpu.VMEM((3, 512, HD), U32), pltpu.VMEM((HD // 2, DM), U32),
                        pltpu.VMEM((S, DM), BF16), pltpu.VMEM((3, 256, HD), U32),
                        pltpu.VMEM((S, DM), BF16), pltpu.VMEM((S // 2, D), U32),
                        pltpu.VMEM((S // 2, D), U32), pltpu.VMEM((S // 2, D), U32), pltpu.VMEM((S, D), U32),
                        pltpu.SemaphoreType.DMA((3,))],
        compiler_params=pltpu.CompilerParams(vmem_limit_bytes=126 * 1024 * 1024),
    )(A_mem0[0], A_Wq, A_Wk, A_Wv, A_Wo.reshape(HD, DM), A_x[0], B_q[0], B_k[0], B_v[0],
      B_shift_k.T, B_ssm_k, B_ssm_D.reshape(1, D),
      jnp.asarray(_FWD).astype(BF16), jnp.asarray(_INV).astype(BF16), jnp.asarray(_MASKS))
    return out[None]
```

```python
import functools
import numpy as np
import jax
import jax.numpy as jnp
import jax.experimental.pallas as pl
import jax.experimental.pallas.tpu as pltpu

S, DM, H, DH, M, D = 2048, 1024, 32, 128, 8, 1024
HD = H * DH
SEG = 32
NSEG = S // SEG
C = 128
NC = S // C
CW = C // 2
GH = 2
ORDER = (('qk',1),('pv',2),('k',0),('pv3',3),('q',0),('v',0),('sm3',2),('qk3',1),('sm',1))
PARTS = ((16,0),(22,16),(30,17),(32,0))
UF, UI = 4, 4
FILL = ((0, 100, 0), (1, 100, 1))
F32, BF16, U32 = jnp.float32, jnp.bfloat16, jnp.uint32
LOG2E = 1.4426950408889634


def _dft_consts():
    th = 2 * np.pi * (np.arange(C)[:, None] + 0.5) / (2 * C)
    n = np.arange(2 * C)[None, :]
    cos, sin = np.cos(th * n), np.sin(th * n)
    fwd = np.concatenate([cos[:, :C], -sin[:, :C]], 0)
    inv = np.concatenate([cos, -sin], 0).T / C
    perm = np.arange(2 * C).reshape(2, C).T.reshape(-1)
    inv = inv[:, perm]
    g = inv[:C]
    rows = np.arange(C).reshape(C // 16, 8, 2).transpose(0, 2, 1).reshape(-1)
    g = g[rows]
    return fwd.astype(np.float32), g.astype(np.float32)


def _attn_masks():
    nat = np.array([-1] * 8 + list(range(16, 24)) + list(range(16)))
    c = np.arange(16)
    inter = c // 2 + 8 * (c % 2)
    klab = np.concatenate([nat[:16][inter], nat[16:][inter], 24 + c // 2])
    out = np.zeros((80, 128), np.float32)
    for par in range(2):
        valid = np.concatenate([np.ones(32, bool), c % 2 == par])
        ok = (nat[:, None] < 0) | (klab[None, :] < 0) | (klab[None, :] <= nat[:, None])
        out[32 * par:32 * par + 32, :48] = ok & valid[None, :]
    for r in range(16):
        par, i = r % 2, r // 2
        out[64 + r, 32 * par:32 * par + 32] = 1
        out[64 + r, 64:80] = (c % 2 == par) & (c // 2 <= i)
    return out


_FWD, _INV = _dft_consts()
_MASKS = _attn_masks()


def _nn(a, b):
    return jnp.dot(a, b, preferred_element_type=F32)


def _nt(a, b):
    return jax.lax.dot_general(a, b, (((1,), (1,)), ((), ())), preferred_element_type=F32)


def _b(x):
    return pltpu.bitcast(x, BF16)


def _pe(lo, hi):
    rnd = lambda t: pltpu.bitcast(t.astype(BF16).astype(F32), U32)
    return (rnd(lo) >> 16) | rnd(hi)


def _lo(w):
    return pltpu.bitcast(w << 16, F32)


def _hi(w):
    return pltpu.bitcast(w & jnp.uint32(0xffff0000), F32)


def _kernel(mem0_ref, wq_h, wk_h, wv_h, wo_h, x_h, bq_h, bk_h, bv_h, sk_ref, ssmk_h, sd_ref,
            fwd_ref, inv_ref, mask_ref, out_h,
            w3, wo, xs, qkv3, ob, obb, bq, kv, yb, osem):
    c_exp = DH ** -0.5 * LOG2E
    w_h = [r.bitcast(U32) for r in (wq_h, wk_h, wv_h)]

    def b_cp(c):
        segs = pl.ds(c * (C // SEG), C // SEG)
        return pltpu.make_async_copy(obb.at[segs], out_h.bitcast(U32).at[segs, :, pl.ds(DM, D)], osem.at[1])

    def phase1(slab, x3, bk, sk, xf, kf, wsem, bsem, dsem):
        def slab_cp(m, hp, par):
            return pltpu.make_async_copy(w_h[m].at[:, par, hp, :], slab.at[hp, par], wsem.at[hp, par])
        x32 = x_h.bitcast(U32)
        x3_cps = [pltpu.make_async_copy(x32.at[:, pl.ds(12 + 16 * p, 4), :], x3.at[:, pl.ds(4 * p, 4), :],
                                        dsem.at[3 + p]) for p in range(2)]
        wo_cp = pltpu.make_async_copy(wo_h.bitcast(U32), wo, dsem.at[0])
        x_cp = pltpu.make_async_copy(x_h, xs, dsem.at[1])
        bq_cp = pltpu.make_async_copy(bq_h.bitcast(U32), bq, dsem.at[2])
        QB = NC // 4

        bk32, bv32 = bk_h.bitcast(U32), bv_h.bitcast(U32)

        def bin_cps(p):
            rows = pl.ds(p * QB * C, QB * C)
            wr = pl.ds(p * QB * CW, QB * CW)
            return [pltpu.make_async_copy(bk32.at[wr], bk.at[pl.ds(8 + p * QB * CW, QB * CW)], bsem.at[0, p]),
                    pltpu.make_async_copy(bv32.at[wr], kv.at[wr], bsem.at[1, p]),
                    pltpu.make_async_copy(ssmk_h.at[:, rows], sk.at[:, rows], bsem.at[2, p])]

        def unit_cps(m, qi):
            return [slab_cp(m, qi * 4 + hh, par) for hh in range(4) for par in range(2)]

        def start(cps):
            for cp in cps:
                cp.start()

        start(x3_cps)
        start(unit_cps(0, 0))
        bk[0:8, :] = jnp.zeros((8, D), U32)
        CB = 512

        def bfwd(cc, _):
          fwd = fwd_ref[...]
          for c in [cc * UF + t for t in range(UF)]:
            rows = pl.ds(pl.multiple_of(c * C, C), C)
            wrows = pl.ds(pl.multiple_of(c * CW, CW), CW)
            spec = pl.ds(pl.multiple_of(c * 2 * C, 2 * C), 2 * C)
            for cb in range(D // CB):
                cols = slice(cb * CB, (cb + 1) * CB)
                kf[spec, cols] = _nt(fwd, sk[cols, rows])
                t0, t1, t2, t3 = [sk_ref[d:d + 1, cols].astype(F32) for d in range(4)]
                blk = bk[pl.ds(pl.multiple_of(c * CW, 8), CW + 8), cols]
                w0, w1, w2 = blk[8:], pltpu.roll(blk, 1, 0)[8:], pltpu.roll(blk, 2, 0)[8:]
                e0, o0, e1, o1, o2 = _lo(w0), _hi(w0), _lo(w1), _hi(w1), _hi(w2)
                v = kv[wrows, cols]
                kvw = _pe((e0 * t0 + o1 * t1 + e1 * t2 + o2 * t3) * _lo(v),
                          (o0 * t0 + e0 * t1 + o1 * t2 + e1 * t3) * _hi(v))
                kv[wrows, cols] = kvw
                xf[spec, cols] = _nn(fwd, _b(kvw))
          return 0
        def products(u):
            fr = pl.multiple_of((u >> 3) * 8, 8)
            col = pl.ds(pl.multiple_of((u & 7) * 128, 128), 128)
            xv = xf.at[pl.ds(fr, 2 * S - C + 8), col]
            kw = kf.at[pl.ds(fr, 2 * S - C + 8), col]
            yv = yb.at[pl.ds(fr, S - C + 8), col]
            sign = jax.lax.broadcasted_iota(U32, (8, 128), 0) << 31

            def flip(t):
                return pltpu.bitcast(pltpu.bitcast(t, U32) ^ sign, F32)
            prev = None
            for i in range(NC):
                ar = ai = None
                for j in range(i + 1):
                    xo, ko = (i - j) * 2 * C, j * 2 * C
                    xr, xi = xv[xo:xo + 8, :], xv[xo + C:xo + C + 8, :]
                    kr, ki = kw[ko:ko + 8, :], kw[ko + C:ko + C + 8, :]
                    tr, ti = xr * kr - xi * ki, xr * ki + xi * kr
                    ar, ai = (tr, ti) if ar is None else (ar + tr, ai + ti)
                    if j == i:
                        zr, zi = (ar, ai) if prev is None else (ar - flip(prev[1]), ai + flip(prev[0]))
                        yv[i * C:i * C + 8, :] = _pe(zr, zi)
                        prev = (ar, ai)
                    yield

        NPRE = 2
        NST = -(-128 // (12 - NPRE))

        def unit(un, _, with_products):
            m, qi = un >> 2, un & 3
            wm = w3.at[m]
            for mm in range(3 if with_products else 1):
                @pl.when(m == mm)
                def _():
                    for cp in unit_cps(mm, qi):
                        cp.wait()
            sl = slab.at[pl.ds(qi * 4, 4)]
            wv = wm.at[:, pl.ds(pl.multiple_of(qi * 1024, 1024), 1024)]

            def body(i, _):
                r = pl.ds(pl.multiple_of(i * 8, 8), 8)
                for hh in range(4):
                    a, b = sl[hh, 0, r, :], sl[hh, 1, r, :]
                    wv[r, hh * 256:hh * 256 + 128] = (a & 0xffff) | (b << 16)
                    wv[r, hh * 256 + 128:hh * 256 + 256] = (a >> 16) | (b & jnp.uint32(0xffff0000))
                return 0
            jax.lax.fori_loop(0, 64, body, 0, unroll=4)
            if with_products:
                for mm in range(2):
                    @pl.when(m == mm)
                    def _():
                        start(unit_cps(mm + 1, qi))

                @pl.when(un == 5)
                def _():
                    bq_cp.start()

                @pl.when(un == 8)
                def _():
                    wo_cp.start()
                    x_cp.start()
            else:
                @pl.when(un == 0)
                def _():
                    start(unit_cps(0, 1))
                    start(bin_cps(0))

                @pl.when(un == 1)
                def _():
                    start(bin_cps(1))
                    start(bin_cps(2))

            def strips():
                for t in range(NST if with_products else 0):
                    yield from products(jnp.minimum((un - NPRE) * NST + t, 127))
            work = strips()
            per_dot = -(-NST * (NC * (NC + 1) // 2) // 64)
            wq = wm.at[:, pl.ds(pl.multiple_of(qi * 1024, 1024), 1024)]
            qo = qkv3.at[m].at[:, pl.ds(pl.multiple_of(qi * 1024, 1024), 1024)]
            for mb in range(8):
                for n in range(8):
                    cols = slice(n * 128, (n + 1) * 128)
                    r = _nn(_b(x3[mb * 4:(mb + 1) * 4].reshape(32, DM)), _b(wq[:, cols]))
                    for j in range(4):
                        qo[mb * 32 + 8 * j:mb * 32 + 8 * j + 8, cols] = _pe(r[16 * j:16 * j + 8],
                                                                            r[16 * j + 8:16 * j + 16])
                    for _ in range(per_dot):
                        next(work, None)
            for _ in work:
                pass
            return 0

        for cp in x3_cps:
            cp.wait()
        jax.lax.fori_loop(0, NPRE, functools.partial(unit, with_products=False), 0)
        for p in range(4):
            for cp in bin_cps(p):
                cp.wait()
            if p == 0:
                start(bin_cps(3))
            elif p == 1:
                start(unit_cps(0, 2))
                start(unit_cps(0, 3))
            elif p == 2:
                start(unit_cps(1, 0))
                start(unit_cps(1, 1))
            jax.lax.fori_loop(p * QB // UF, (p + 1) * QB // UF, bfwd, 0)
        jax.lax.fori_loop(NPRE, 12, functools.partial(unit, with_products=True), 0)

        bq_cp.wait()
        wo_cp.wait()
        x_cp.wait()

    pl.run_scoped(phase1, pltpu.VMEM((16, 2, 512, 128), U32), pltpu.VMEM((NSEG // 2, 8, DM), U32),
                  pltpu.VMEM((S // 2 + 8, D), U32), pltpu.VMEM((D, S), BF16),
                  pltpu.VMEM((2 * S, D), F32), pltpu.VMEM((2 * S, D), F32),
                  pltpu.SemaphoreType.DMA((16, 2)), pltpu.SemaphoreType.DMA((3, 4)),
                  pltpu.SemaphoreType.DMA((5,)))

    def phase2(o3):
        NG = H // GH

        def softmax(sc, allowed):
            sc = jnp.where(allowed, sc * c_exp, -1e9)
            e = jnp.exp2(sc - jnp.max(sc, -1, keepdims=True))
            return (e * (1.0 / jnp.sum(e, -1, keepdims=True))).astype(BF16)

        def step(s, mem, si, keep):
            allowed = mask_ref[32 * si:32 * si + 32, 0:48] > 0.5
            allowed3 = mask_ref[64:80, 0:80] > 0.5
            xs0 = xs[s >> 1, 32 * si:32 * si + 16, :].astype(F32)
            xs1 = xs[s >> 1, 32 * si + 16:32 * si + 24, :].astype(F32)
            hb = jnp.concatenate([mem, xs1, xs0], 0).astype(BF16)
            jr = pl.ds(pl.multiple_of((s >> 1) * 8, 8), 8)
            o3v = o3.at[pl.ds(pl.multiple_of((s >> 1) * 16, 16), 16), :]
            st = {}

            def do(op, g):
                if g < 0 or g >= NG or (op[-1] == '3' and si == 0):
                    return
                if op in 'qkv':
                    m = 'qkv'.index(op)
                    t = _nn(hb, _b(w3[m, :, g * GH * DH:(g + 1) * GH * DH]))
                for hh in range(GH):
                    h = g * GH + hh
                    hs = slice(h * DH, (h + 1) * DH)
                    ls = slice(hh * DH, (hh + 1) * DH)
                    if op == 'q':
                        st['q', h] = t[:, ls].astype(BF16)
                    elif op in 'kv':
                        two = [_pe(t[0:8, ls], t[8:16, ls]), _pe(t[16:24, ls], t[24:32, ls])]
                        st[op, h] = jnp.concatenate(two + [qkv3[m, jr, hs]], 0)
                        if si == 0:
                            keep[op, h] = two
                        else:
                            st[op + '3', h] = jnp.concatenate(keep.pop((op, h)) + two + [qkv3[m, jr, hs]], 0)
                    elif op == 'qk':
                        st['s', h] = _nt(st.pop(('q', h)), _b(st.pop(('k', h))))
                    elif op == 'sm':
                        st['p', h] = softmax(st.pop(('s', h)), allowed)
                    elif op == 'pv':
                        st['o', h] = _nn(st.pop(('p', h)), _b(st.pop(('v', h))))
                    elif op == 'qk3':
                        st['s3', h] = _nt(_b(qkv3[0, jr, hs]), _b(st.pop(('k3', h))))
                    elif op == 'sm3':
                        st['p3', h] = softmax(st.pop(('s3', h)), allowed3)
                    else:
                        o3v[:, hs] = _nn(st.pop(('p3', h)), _b(st.pop(('v3', h))))
            def fill(cb):
                c = s >> 2
                cols = pl.ds(pl.multiple_of(cb * 256, 256), 256)
                wrows = pl.ds(pl.multiple_of(c * CW, CW), CW)
                y = _nn(inv_ref[...], _b(yb[pl.ds(pl.multiple_of(c * C, C), C), cols]))
                dd = sd_ref[:, cols].astype(F32)
                kvw, qw = kv[wrows, cols], bq[wrows, cols]
                out = []
                for i in range(C // 16):
                    wr = slice(8 * i, 8 * i + 8)
                    ye = y[16 * i:16 * i + 8] + _lo(kvw[wr]) * dd
                    yo = y[16 * i + 8:16 * i + 16] + _hi(kvw[wr]) * dd
                    out.append(_pe(ye * _lo(qw[wr]), yo * _hi(qw[wr])))
                obb[pl.ds(c * (C // SEG), C // SEG), :, cols] = jnp.concatenate(out, 0).reshape(C // SEG, SEG // 2, 256)

            def fills(pos):
                for fsi, fpos, k in FILL:
                    if fsi == si and fpos == pos:
                        fill((s & 2) + k)
            r = None
            done = 0
            order = ORDER
            for g in range(NG + max(d for _, d in order)):
                fills(100 + g)
                for op, d in order:
                    do(op, g - d)
                for p, gmin in PARTS:
                    if g >= gmin and done < p and all(('o', h) in st for h in range(done, p)):
                        fills(p)
                        part = _nn(jnp.concatenate([st.pop(('o', h)) for h in range(done, p)], 1).astype(BF16),
                                   _b(wo[done * DH // 2:p * DH // 2, :]))
                        r = part if r is None else r + part
                        done = p
            fills(99)
            rb = r.astype(BF16)
            ob[s, 0:16, :] = rb[16:32]
            ob[s, 16:24, :] = rb[8:16]

            if si == 1:
                @pl.when((s & 3) == 3)
                def _():
                    b_cp(s >> 2).start()
            return rb[0:8].astype(F32)
        def steps(t, mem):
            keep = {}
            for i in range(2):
                mem = step(t * 2 + i, mem, i, keep)
            return mem
        jax.lax.fori_loop(0, NSEG // 2, steps, mem0_ref[...].astype(F32))

        a_cp = pltpu.make_async_copy(ob.at[:, pl.ds(0, 24), :], out_h.at[:, pl.ds(0, 24), pl.ds(0, DM)],
                                     osem.at[0])
        a_cp.start()

        def f_cp(n):
            return pltpu.make_async_copy(ob.at[pl.ds(n * 16, 16), pl.ds(24, 8), :],
                                         out_h.at[pl.ds(n * 16, 16), pl.ds(24, 8), pl.ds(0, DM)], osem.at[2])

        def fin(n, _):
            rows = pl.ds(pl.multiple_of(n * 128, 128), 128)
            r = _nn(o3[rows, :].astype(BF16), _b(wo[...]))
            w = pltpu.bitcast(r.astype(BF16), U32)
            for i in range(8):
                wi = w[i * 8:(i + 1) * 8]
                for half, val in ((0, _lo(wi)), (1, _hi(wi))):
                    ob[n * 16 + 2 * i + half, 24:32, :] = val.astype(BF16)
            f_cp(n).start()
            return 0
        jax.lax.fori_loop(0, 4, fin, 0)
        a_cp.wait()
        for c in range(NC):
            b_cp(c).wait()
        for n in range(4):
            f_cp(n).wait()

    pl.run_scoped(phase2, pltpu.VMEM((NSEG * 8, HD), F32))


@functools.partial(jax.jit, static_argnames=("A_seg_len",))
def pallas_concat_heads__memory_aug_recurrent_mem_tr__ssm_conv_h3__prompt_kernel(
        A_x, A_mem0, A_Wq, A_Wk, A_Wv, A_Wo, A_seg_len, B_q, B_k, B_v, B_shift_k, B_ssm_k, B_ssm_D):
    assert int(A_seg_len) == SEG
    vm = pl.BlockSpec(memory_space=pltpu.VMEM)
    hbm = pl.BlockSpec(memory_space=pl.ANY)
    out = pl.pallas_call(
        _kernel,
        in_specs=[vm, hbm, hbm, hbm, hbm, hbm, hbm, hbm, hbm, vm, hbm, vm, vm, vm, vm],
        out_specs=hbm,
        out_shape=jax.ShapeDtypeStruct((NSEG, SEG, DM + D), BF16),
        scratch_shapes=[pltpu.VMEM((3, 512, HD), U32), pltpu.VMEM((HD // 2, DM), U32),
                        pltpu.VMEM((NSEG // 2, 2 * SEG, DM), BF16), pltpu.VMEM((3, 256, HD), U32),
                        pltpu.VMEM((NSEG, SEG, DM), BF16), pltpu.VMEM((NSEG, SEG // 2, D), U32),
                        pltpu.VMEM((S // 2, D), U32), pltpu.VMEM((S // 2, D), U32), pltpu.VMEM((S, D), U32),
                        pltpu.SemaphoreType.DMA((3,))],
        compiler_params=pltpu.CompilerParams(vmem_limit_bytes=126 * 1024 * 1024),
    )(A_mem0[0], *[w.reshape(DM // 2, 2, H, DH) for w in (A_Wq, A_Wk, A_Wv)], A_Wo.reshape(HD, DM),
      A_x.reshape(NSEG // 2, 2 * SEG, DM), B_q[0], B_k[0], B_v[0],
      B_shift_k.T, B_ssm_k, B_ssm_D.reshape(1, D),
      jnp.asarray(_FWD).astype(BF16), jnp.asarray(_INV).astype(BF16), jnp.asarray(_MASKS))
    return out.reshape(1, S, DM + D)
```

```python
import functools
import numpy as np
import jax
import jax.numpy as jnp
import jax.experimental.pallas as pl
import jax.experimental.pallas.tpu as pltpu

S, DM, H, DH, M, D = 2048, 1024, 32, 128, 8, 1024
HD = H * DH
SEG = 32
NSEG = S // SEG
C = 128
NC = S // C
CW = C // 2
GH = 2
ORDER = (('qk',1),('pv',2),('k',0),('pv3',3),('q',0),('v',0),('sm3',2),('qk3',1),('sm',1))
PARTS = ((16,0),(22,16),(30,17),(32,0))
FILL = ((0, 100, 0), (1, 100, 1))
FINM, FINW = 64, 1024
F32, BF16, U32 = jnp.float32, jnp.bfloat16, jnp.uint32
LOG2E = 1.4426950408889634


def _dft_consts():
    th = 2 * np.pi * (np.arange(C)[:, None] + 0.5) / (2 * C)
    n = np.arange(2 * C)[None, :]
    cos, sin = np.cos(th * n), np.sin(th * n)
    fwd = np.concatenate([cos[:, :C], -sin[:, :C]], 0)
    inv = np.concatenate([cos, -sin], 0).T / C
    perm = np.arange(2 * C).reshape(2, C).T.reshape(-1)
    inv = inv[:, perm]
    g = inv[:C]
    rows = np.arange(C).reshape(C // 16, 8, 2).transpose(0, 2, 1).reshape(-1)
    g = g[rows]
    return fwd.astype(np.float32), g.astype(np.float32)


def _attn_masks():
    nat = np.array([-1] * 8 + list(range(16, 24)) + list(range(16)))
    c = np.arange(16)
    inter = c // 2 + 8 * (c % 2)
    klab = np.concatenate([nat[:16][inter], nat[16:][inter], 24 + c // 2])
    out = np.zeros((80, 128), np.float32)
    for par in range(2):
        valid = np.concatenate([np.ones(32, bool), c % 2 == par])
        ok = (nat[:, None] < 0) | (klab[None, :] < 0) | (klab[None, :] <= nat[:, None])
        out[32 * par:32 * par + 32, :48] = ok & valid[None, :]
    for r in range(16):
        par, i = r % 2, r // 2
        out[64 + r, 32 * par:32 * par + 32] = 1
        out[64 + r, 64:80] = (c % 2 == par) & (c // 2 <= i)
    return out


_FWD, _INV = _dft_consts()
_MASKS = _attn_masks()


def _nn(a, b):
    return jnp.dot(a, b, preferred_element_type=F32)


def _nt(a, b):
    return jax.lax.dot_general(a, b, (((1,), (1,)), ((), ())), preferred_element_type=F32)


def _b(x):
    return pltpu.bitcast(x, BF16)


def _pe(lo, hi):
    rnd = lambda t: pltpu.bitcast(t.astype(BF16).astype(F32), U32)
    return (rnd(lo) >> 16) | rnd(hi)


def _lo(w):
    return pltpu.bitcast(w << 16, F32)


def _hi(w):
    return pltpu.bitcast(w & jnp.uint32(0xffff0000), F32)


def _kernel(mem0_h, wq_h, wk_h, wv_h, wo_h, x_h, bq_h, bk_h, bv_h, sk_h, ssmk_h, sd_h,
            fwd_h, inv_h, mask_h, out_h,
            w3, wo, xs, qkv3, ob, obb, bq, kv, yb, osem,
            mem0_ref, sk_ref, sd_ref, fwd_ref, inv_ref, mask_ref, csem):
    c_exp = DH ** -0.5 * LOG2E
    small = [pltpu.make_async_copy(src, dst, csem.at[i]) for i, (src, dst) in enumerate(
        ((sk_h, sk_ref), (fwd_h, fwd_ref), (mem0_h, mem0_ref), (sd_h, sd_ref), (inv_h, inv_ref), (mask_h, mask_ref)))]
    w_h = [r.bitcast(U32) for r in (wq_h, wk_h, wv_h)]

    def b_cp(c):
        segs = pl.ds(c * (C // SEG), C // SEG)
        return pltpu.make_async_copy(obb.at[segs], out_h.bitcast(U32).at[segs, :, pl.ds(DM, D)], osem.at[1])

    def phase1(slab, x3, bk, sk, xf, kf, wsem, bsem, dsem):
        def slab_cp(m, hp, par):
            return pltpu.make_async_copy(w_h[m].at[:, par, hp, :], slab.at[hp, par], wsem.at[hp, par])
        x32 = x_h.bitcast(U32)
        x3_cps = [pltpu.make_async_copy(x32.at[:, pl.ds(12 + 16 * p, 4), :], x3.at[:, pl.ds(4 * p, 4), :],
                                        dsem.at[3 + p]) for p in range(2)]
        wo_cp = pltpu.make_async_copy(wo_h.bitcast(U32), wo, dsem.at[0])
        x_cp = pltpu.make_async_copy(x_h, xs, dsem.at[1])
        bq_cp = pltpu.make_async_copy(bq_h.bitcast(U32), bq, dsem.at[2])
        QB = NC // 4

        bk32, bv32 = bk_h.bitcast(U32), bv_h.bitcast(U32)

        def bin_cps(p):
            rows = pl.ds(p * QB * C, QB * C)
            wr = pl.ds(p * QB * CW, QB * CW)
            return [pltpu.make_async_copy(bk32.at[wr], bk.at[pl.ds(8 + p * QB * CW, QB * CW)], bsem.at[0, p]),
                    pltpu.make_async_copy(bv32.at[wr], kv.at[wr], bsem.at[1, p]),
                    pltpu.make_async_copy(ssmk_h.at[:, rows], sk.at[:, rows], bsem.at[2, p])]

        def unit_cps(m, qi):
            return [slab_cp(m, qi * 4 + hh, par) for hh in range(4) for par in range(2)]

        def start(cps):
            for cp in cps:
                cp.start()

        start(x3_cps)
        start(unit_cps(0, 0))
        start(small)
        bk[0:8, :] = jnp.zeros((8, D), U32)
        CB = 512

        def bfwd(p):
            fwd = fwd_ref[...]
            for c in range(p * QB, (p + 1) * QB):
                rows, wrows, spec = pl.ds(c * C, C), pl.ds(c * CW, CW), pl.ds(c * 2 * C, 2 * C)
                for cb in range(D // CB):
                    cols = slice(cb * CB, (cb + 1) * CB)
                    kf[spec, cols] = _nt(fwd, sk[cols, rows])
                    t0, t1, t2, t3 = [sk_ref[d:d + 1, cols].astype(F32) for d in range(4)]
                    blk = bk[pl.ds(c * CW, CW + 8), cols]
                    w0, w1, w2 = blk[8:], pltpu.roll(blk, 1, 0)[8:], pltpu.roll(blk, 2, 0)[8:]
                    e0, o0, e1, o1, o2 = _lo(w0), _hi(w0), _lo(w1), _hi(w1), _hi(w2)
                    v = kv[wrows, cols]
                    kvw = _pe((e0 * t0 + o1 * t1 + e1 * t2 + o2 * t3) * _lo(v),
                              (o0 * t0 + e0 * t1 + o1 * t2 + e1 * t3) * _hi(v))
                    kv[wrows, cols] = kvw
                    xf[spec, cols] = _nn(fwd, _b(kvw))

        def products(u):
            fr = pl.multiple_of((u >> 3) * 8, 8)
            col = pl.ds(pl.multiple_of((u & 7) * 128, 128), 128)
            xv = xf.at[pl.ds(fr, 2 * S - C + 8), col]
            kw = kf.at[pl.ds(fr, 2 * S - C + 8), col]
            yv = yb.at[pl.ds(fr, S - C + 8), col]
            sign = jax.lax.broadcasted_iota(U32, (8, 128), 0) << 31

            def flip(t):
                return pltpu.bitcast(pltpu.bitcast(t, U32) ^ sign, F32)
            prev = None
            for i in range(NC):
                ar = ai = None
                for j in range(i + 1):
                    xo, ko = (i - j) * 2 * C, j * 2 * C
                    xr, xi = xv[xo:xo + 8, :], xv[xo + C:xo + C + 8, :]
                    kr, ki = kw[ko:ko + 8, :], kw[ko + C:ko + C + 8, :]
                    tr, ti = xr * kr - xi * ki, xr * ki + xi * kr
                    ar, ai = (tr, ti) if ar is None else (ar + tr, ai + ti)
                    if j == i:
                        zr, zi = (ar, ai) if prev is None else (ar - flip(prev[1]), ai + flip(prev[0]))
                        yv[i * C:i * C + 8, :] = _pe(zr, zi)
                        prev = (ar, ai)
                    yield

        NPRE = 2
        NST = -(-128 // (12 - NPRE))

        def unit(un, _, with_products):
            m, qi = un >> 2, un & 3
            wm = w3.at[m]
            for mm in range(3 if with_products else 1):
                @pl.when(m == mm)
                def _():
                    for cp in unit_cps(mm, qi):
                        cp.wait()
            sl = slab.at[pl.ds(qi * 4, 4)]
            wv = wm.at[:, pl.ds(pl.multiple_of(qi * 1024, 1024), 1024)]

            def body(i, _):
                r = pl.ds(pl.multiple_of(i * 8, 8), 8)
                for hh in range(4):
                    a, b = sl[hh, 0, r, :], sl[hh, 1, r, :]
                    wv[r, hh * 256:hh * 256 + 128] = (a & 0xffff) | (b << 16)
                    wv[r, hh * 256 + 128:hh * 256 + 256] = (a >> 16) | (b & jnp.uint32(0xffff0000))
                return 0
            jax.lax.fori_loop(0, 64, body, 0, unroll=4)
            if with_products:
                for mm in range(2):
                    @pl.when(m == mm)
                    def _():
                        start(unit_cps(mm + 1, qi))

                @pl.when(un == 5)
                def _():
                    bq_cp.start()

                @pl.when(un == 8)
                def _():
                    wo_cp.start()
                    x_cp.start()
            else:
                @pl.when(un == 0)
                def _():
                    start(unit_cps(0, 1))
                    start(bin_cps(0))

                @pl.when(un == 1)
                def _():
                    start(bin_cps(1))
                    start(bin_cps(2))

            def strips():
                for t in range(NST if with_products else 0):
                    yield from products(jnp.minimum((un - NPRE) * NST + t, 127))
            work = strips()
            per_dot = -(-NST * (NC * (NC + 1) // 2) // 64)
            wq = wm.at[:, pl.ds(pl.multiple_of(qi * 1024, 1024), 1024)]
            qo = qkv3.at[m].at[:, pl.ds(pl.multiple_of(qi * 1024, 1024), 1024)]
            for mb in range(8):
                for n in range(8):
                    cols = slice(n * 128, (n + 1) * 128)
                    r = _nn(_b(x3[mb * 4:(mb + 1) * 4].reshape(32, DM)), _b(wq[:, cols]))
                    for j in range(4):
                        qo[mb * 32 + 8 * j:mb * 32 + 8 * j + 8, cols] = _pe(r[16 * j:16 * j + 8],
                                                                            r[16 * j + 8:16 * j + 16])
                    for _ in range(per_dot):
                        next(work, None)
            for _ in work:
                pass
            return 0

        for cp in x3_cps:
            cp.wait()
        jax.lax.fori_loop(0, NPRE, functools.partial(unit, with_products=False), 0)
        for cp in small:
            cp.wait()
        for p in range(4):
            for cp in bin_cps(p):
                cp.wait()
            if p == 0:
                start(bin_cps(3))
            elif p == 1:
                start(unit_cps(0, 2))
                start(unit_cps(0, 3))
            elif p == 2:
                start(unit_cps(1, 0))
                start(unit_cps(1, 1))
            bfwd(p)
        jax.lax.fori_loop(NPRE, 12, functools.partial(unit, with_products=True), 0)

        bq_cp.wait()
        wo_cp.wait()
        x_cp.wait()

    pl.run_scoped(phase1, pltpu.VMEM((16, 2, 512, 128), U32), pltpu.VMEM((NSEG // 2, 8, DM), U32),
                  pltpu.VMEM((S // 2 + 8, D), U32), pltpu.VMEM((D, S), BF16),
                  pltpu.VMEM((2 * S, D), F32), pltpu.VMEM((2 * S, D), F32),
                  pltpu.SemaphoreType.DMA((16, 2)), pltpu.SemaphoreType.DMA((3, 4)),
                  pltpu.SemaphoreType.DMA((5,)))

    def phase2(o3):
        NG = H // GH

        def softmax(sc, allowed):
            sc = jnp.where(allowed, sc * c_exp, -1e9)
            e = jnp.exp2(sc - jnp.max(sc, -1, keepdims=True))
            return (e * (1.0 / jnp.sum(e, -1, keepdims=True))).astype(BF16)

        def step(s, mem, si, keep):
            allowed = mask_ref[32 * si:32 * si + 32, 0:48] > 0.5
            allowed3 = mask_ref[64:80, 0:80] > 0.5
            xs0 = xs[s >> 1, 32 * si:32 * si + 16, :].astype(F32)
            xs1 = xs[s >> 1, 32 * si + 16:32 * si + 24, :].astype(F32)
            hb = jnp.concatenate([mem, xs1, xs0], 0).astype(BF16)
            jr = pl.ds(pl.multiple_of((s >> 1) * 8, 8), 8)
            o3v = o3.at[pl.ds(pl.multiple_of((s >> 1) * 16, 16), 16), :]
            st = {}

            def do(op, g):
                if g < 0 or g >= NG or (op[-1] == '3' and si == 0):
                    return
                if op in 'qkv':
                    m = 'qkv'.index(op)
                    t = _nn(hb, _b(w3[m, :, g * GH * DH:(g + 1) * GH * DH]))
                for hh in range(GH):
                    h = g * GH + hh
                    hs = slice(h * DH, (h + 1) * DH)
                    ls = slice(hh * DH, (hh + 1) * DH)
                    if op == 'q':
                        st['q', h] = t[:, ls].astype(BF16)
                    elif op in 'kv':
                        two = [_pe(t[0:8, ls], t[8:16, ls]), _pe(t[16:24, ls], t[24:32, ls])]
                        st[op, h] = jnp.concatenate(two + [qkv3[m, jr, hs]], 0)
                        if si == 0:
                            keep[op, h] = two
                        else:
                            st[op + '3', h] = jnp.concatenate(keep.pop((op, h)) + two + [qkv3[m, jr, hs]], 0)
                    elif op == 'qk':
                        st['s', h] = _nt(st.pop(('q', h)), _b(st.pop(('k', h))))
                    elif op == 'sm':
                        st['p', h] = softmax(st.pop(('s', h)), allowed)
                    elif op == 'pv':
                        st['o', h] = _nn(st.pop(('p', h)), _b(st.pop(('v', h))))
                    elif op == 'qk3':
                        st['s3', h] = _nt(_b(qkv3[0, jr, hs]), _b(st.pop(('k3', h))))
                    elif op == 'sm3':
                        st['p3', h] = softmax(st.pop(('s3', h)), allowed3)
                    else:
                        o3v[:, hs] = _nn(st.pop(('p3', h)), _b(st.pop(('v3', h))))
            def fill(cb):
                c = s >> 2
                cols = pl.ds(pl.multiple_of(cb * 256, 256), 256)
                wrows = pl.ds(pl.multiple_of(c * CW, CW), CW)
                y = _nn(inv_ref[...], _b(yb[pl.ds(pl.multiple_of(c * C, C), C), cols]))
                dd = sd_ref[:, cols].astype(F32)
                kvw, qw = kv[wrows, cols], bq[wrows, cols]
                out = []
                for i in range(C // 16):
                    wr = slice(8 * i, 8 * i + 8)
                    ye = y[16 * i:16 * i + 8] + _lo(kvw[wr]) * dd
                    yo = y[16 * i + 8:16 * i + 16] + _hi(kvw[wr]) * dd
                    out.append(_pe(ye * _lo(qw[wr]), yo * _hi(qw[wr])))
                obb[pl.ds(c * (C // SEG), C // SEG), :, cols] = jnp.concatenate(out, 0).reshape(C // SEG, SEG // 2, 256)

            def fills(pos):
                for fsi, fpos, k in FILL:
                    if fsi == si and fpos == pos:
                        fill((s & 2) + k)
            r = None
            done = 0
            order = ORDER
            for g in range(NG + max(d for _, d in order)):
                fills(100 + g)
                for op, d in order:
                    do(op, g - d)
                for p, gmin in PARTS:
                    if g >= gmin and done < p and all(('o', h) in st for h in range(done, p)):
                        fills(p)
                        part = _nn(jnp.concatenate([st.pop(('o', h)) for h in range(done, p)], 1).astype(BF16),
                                   _b(wo[done * DH // 2:p * DH // 2, :]))
                        r = part if r is None else r + part
                        done = p
            fills(99)
            rb = r.astype(BF16)
            ob[s, 0:16, :] = rb[16:32]
            ob[s, 16:24, :] = rb[8:16]

            if si == 1:
                @pl.when((s & 3) == 3)
                def _():
                    b_cp(s >> 2).start()
            return rb[0:8].astype(F32)
        def steps(t, mem):
            keep = {}
            for i in range(2):
                mem = step(t * 2 + i, mem, i, keep)
            return mem
        jax.lax.fori_loop(0, NSEG // 2, steps, mem0_ref[...].astype(F32))

        a_cp = pltpu.make_async_copy(ob.at[:, pl.ds(0, 24), :], out_h.at[:, pl.ds(0, 24), pl.ds(0, DM)],
                                     osem.at[0])
        a_cp.start()

        FS = FINM // 8

        def f_cp(n):
            return pltpu.make_async_copy(ob.at[pl.ds(n * FS, FS), pl.ds(24, 8), :],
                                         out_h.at[pl.ds(n * FS, FS), pl.ds(24, 8), pl.ds(0, DM)], osem.at[2])

        def fin(n, _):
            rows = pl.ds(pl.multiple_of(n * FINM, FINM), FINM)
            lhs = o3[rows, :].astype(BF16)
            for cb in range(DM // FINW):
                cols = slice(cb * FINW, (cb + 1) * FINW)
                w = pltpu.bitcast(_nn(lhs, _b(wo[:, cols])).astype(BF16), U32)
                for i in range(FINM // 16):
                    wi = w[i * 8:(i + 1) * 8]
                    for half, val in ((0, _lo(wi)), (1, _hi(wi))):
                        ob[n * FS + 2 * i + half, 24:32, cols] = val.astype(BF16)
            f_cp(n).start()
            return 0
        jax.lax.fori_loop(0, 512 // FINM, fin, 0)
        a_cp.wait()
        for c in range(NC):
            b_cp(c).wait()
        for n in range(512 // FINM):
            f_cp(n).wait()

    pl.run_scoped(phase2, pltpu.VMEM((NSEG * 8, HD), F32))


@functools.partial(jax.jit, static_argnames=("A_seg_len",))
def pallas_concat_heads__memory_aug_recurrent_mem_tr__ssm_conv_h3__prompt_kernel(
        A_x, A_mem0, A_Wq, A_Wk, A_Wv, A_Wo, A_seg_len, B_q, B_k, B_v, B_shift_k, B_ssm_k, B_ssm_D):
    assert int(A_seg_len) == SEG
    vm = pl.BlockSpec(memory_space=pltpu.VMEM)
    hbm = pl.BlockSpec(memory_space=pl.ANY)
    out = pl.pallas_call(
        _kernel,
        in_specs=[hbm] * 15,
        out_specs=hbm,
        out_shape=jax.ShapeDtypeStruct((NSEG, SEG, DM + D), BF16),
        scratch_shapes=[pltpu.VMEM((3, 512, HD), U32), pltpu.VMEM((HD // 2, DM), U32),
                        pltpu.VMEM((NSEG // 2, 2 * SEG, DM), BF16), pltpu.VMEM((3, 256, HD), U32),
                        pltpu.VMEM((NSEG, SEG, DM), BF16), pltpu.VMEM((NSEG, SEG // 2, D), U32),
                        pltpu.VMEM((S // 2, D), U32), pltpu.VMEM((S // 2, D), U32), pltpu.VMEM((S, D), U32),
                        pltpu.SemaphoreType.DMA((3,)),
                        pltpu.VMEM((M, DM), BF16), pltpu.VMEM((4, D), BF16), pltpu.VMEM((1, D), BF16),
                        pltpu.VMEM((2 * C, C), BF16), pltpu.VMEM((C, 2 * C), BF16), pltpu.VMEM((80, 128), F32),
                        pltpu.SemaphoreType.DMA((6,))],
        compiler_params=pltpu.CompilerParams(vmem_limit_bytes=126 * 1024 * 1024),
    )(A_mem0[0], *[w.reshape(DM // 2, 2, H, DH) for w in (A_Wq, A_Wk, A_Wv)], A_Wo.reshape(HD, DM),
      A_x.reshape(NSEG // 2, 2 * SEG, DM), B_q[0], B_k[0], B_v[0],
      B_shift_k.T, B_ssm_k, B_ssm_D.reshape(1, D),
      jnp.asarray(_FWD).astype(BF16), jnp.asarray(_INV).astype(BF16), jnp.asarray(_MASKS))
    return out.reshape(1, S, DM + D)
```

```python
import functools
import numpy as np
import jax
import jax.numpy as jnp
import jax.experimental.pallas as pl
import jax.experimental.pallas.tpu as pltpu

S, DM, H, DH, M, D = 2048, 1024, 32, 128, 8, 1024
HD = H * DH
SEG = 32
NSEG = S // SEG
C = 128
NC = S // C
CW = C // 2
GH = 2
ORDER = (('qk',1),('pv',2),('k',0),('pv3',3),('q',0),('v',0),('sm3',2),('qk3',1),('sm',1))
PARTS = ((16,0),(22,16),(30,17),(32,0))
FILL = ((0, 100, 0), (1, 100, 1))
FINM, FINW = 64, 1024
OB = 4
MR, NW = 64, 128
NMAJ = 0
PRE = 0
NPRE = 2
RU = 32
BSCHED = ((0,), (1, 2))
BSCHED2 = ((3,), (), (), ())
USCHED = ((), (2, 3), (4,), ())
F32, BF16, U32 = jnp.float32, jnp.bfloat16, jnp.uint32
LOG2E = 1.4426950408889634


def _dft_consts():
    th = 2 * np.pi * (np.arange(C)[:, None] + 0.5) / (2 * C)
    n = np.arange(2 * C)[None, :]
    cos, sin = np.cos(th * n), np.sin(th * n)
    fwd = np.concatenate([cos[:, :C], -sin[:, :C]], 0)
    inv = np.concatenate([cos, -sin], 0).T / C
    perm = np.arange(2 * C).reshape(2, C).T.reshape(-1)
    inv = inv[:, perm]
    g = inv[:C]
    rows = np.arange(C).reshape(C // 16, 8, 2).transpose(0, 2, 1).reshape(-1)
    g = g[rows]
    return fwd.astype(np.float32), g.astype(np.float32)


def _attn_masks():
    nat = np.array([-1] * 8 + list(range(16, 24)) + list(range(16)))
    c = np.arange(16)
    inter = c // 2 + 8 * (c % 2)
    klab = np.concatenate([nat[:16][inter], nat[16:][inter], 24 + c // 2])
    out = np.zeros((80, 128), np.float32)
    for par in range(2):
        valid = np.concatenate([np.ones(32, bool), c % 2 == par])
        ok = (nat[:, None] < 0) | (klab[None, :] < 0) | (klab[None, :] <= nat[:, None])
        out[32 * par:32 * par + 32, :48] = ok & valid[None, :]
    for r in range(16):
        par, i = r % 2, r // 2
        out[64 + r, 32 * par:32 * par + 32] = 1
        out[64 + r, 64:80] = (c % 2 == par) & (c // 2 <= i)
    return out


_FWD, _INV = _dft_consts()
_MASKS = _attn_masks()


def _nn(a, b):
    return jnp.dot(a, b, preferred_element_type=F32)


def _nt(a, b):
    return jax.lax.dot_general(a, b, (((1,), (1,)), ((), ())), preferred_element_type=F32)


def _b(x):
    return pltpu.bitcast(x, BF16)


def _pe(lo, hi):
    rnd = lambda t: pltpu.bitcast(t.astype(BF16).astype(F32), U32)
    return (rnd(lo) >> 16) | rnd(hi)


def _lo(w):
    return pltpu.bitcast(w << 16, F32)


def _hi(w):
    return pltpu.bitcast(w & jnp.uint32(0xffff0000), F32)


def _kernel(mem0_h, wq_h, wk_h, wv_h, wo_h, x_h, bq_h, bk_h, bv_h, sk_h, ssmk_h, sd_h,
            fwd_h, inv_h, mask_h, out_h,
            w3, wo, xs, qkv3, ob, obb, bq, kv, yb, osem,
            mem0_ref, sk_ref, sd_ref, fwd_ref, inv_ref, mask_ref, csem):
    c_exp = DH ** -0.5 * LOG2E
    small = [pltpu.make_async_copy(src, dst, csem.at[i]) for i, (src, dst) in enumerate(
        ((sk_h, sk_ref), (fwd_h, fwd_ref), (mem0_h, mem0_ref), (sd_h, sd_ref), (inv_h, inv_ref), (mask_h, mask_ref)))]
    w_h = [r.bitcast(U32) for r in (wq_h, wk_h, wv_h)]

    def b_cp(c):
        segs = pl.ds(c * (C // SEG), C // SEG)
        return pltpu.make_async_copy(obb.at[segs], out_h.bitcast(U32).at[segs, :, pl.ds(DM, D)], osem.at[1])

    def phase1(slab, x3, bk, sk, xf, kf, wsem, bsem, dsem):
        def slab_cp(m, hp, par):
            return pltpu.make_async_copy(w_h[m].at[:, par, hp, :], slab.at[hp, par], wsem.at[hp, par])
        x32 = x_h.bitcast(U32)
        x3_cps = [pltpu.make_async_copy(x32.at[:, pl.ds(12 + 16 * p, 4), :], x3.at[:, pl.ds(4 * p, 4), :],
                                        dsem.at[3 + p]) for p in range(2)]
        wo_cp = pltpu.make_async_copy(wo_h.bitcast(U32), wo, dsem.at[0])
        x_cp = pltpu.make_async_copy(x_h, xs, dsem.at[1])
        bq_cp = pltpu.make_async_copy(bq_h.bitcast(U32), bq, dsem.at[2])
        QB = NC // 4

        bk32, bv32 = bk_h.bitcast(U32), bv_h.bitcast(U32)

        def bin_cps(p):
            rows = pl.ds(p * QB * C, QB * C)
            wr = pl.ds(p * QB * CW, QB * CW)
            return [pltpu.make_async_copy(bk32.at[wr], bk.at[pl.ds(8 + p * QB * CW, QB * CW)], bsem.at[0, p]),
                    pltpu.make_async_copy(bv32.at[wr], kv.at[wr], bsem.at[1, p]),
                    pltpu.make_async_copy(ssmk_h.at[:, rows], sk.at[:, rows], bsem.at[2, p])]

        def unit_cps(m, qi):
            return [slab_cp(m, qi * 4 + hh, par) for hh in range(4) for par in range(2)]

        def start(cps):
            for cp in cps:
                cp.start()

        start(x3_cps)
        start(unit_cps(0, 0))
        start(small)
        bk[0:8, :] = jnp.zeros((8, D), U32)
        CB = 512

        def bfwd(p):
            fwd = fwd_ref[...]
            for c in range(p * QB, (p + 1) * QB):
                rows, wrows, spec = pl.ds(c * C, C), pl.ds(c * CW, CW), pl.ds(c * 2 * C, 2 * C)
                for cb in range(D // CB):
                    cols = slice(cb * CB, (cb + 1) * CB)
                    kf[spec, cols] = _nt(fwd, sk[cols, rows])
                    t0, t1, t2, t3 = [sk_ref[d:d + 1, cols].astype(F32) for d in range(4)]
                    blk = bk[pl.ds(c * CW, CW + 8), cols]
                    w0, w1, w2 = blk[8:], pltpu.roll(blk, 1, 0)[8:], pltpu.roll(blk, 2, 0)[8:]
                    e0, o0, e1, o1, o2 = _lo(w0), _hi(w0), _lo(w1), _hi(w1), _hi(w2)
                    v = kv[wrows, cols]
                    kvw = _pe((e0 * t0 + o1 * t1 + e1 * t2 + o2 * t3) * _lo(v),
                              (o0 * t0 + e0 * t1 + o1 * t2 + e1 * t3) * _hi(v))
                    kv[wrows, cols] = kvw
                    xf[spec, cols] = _nn(fwd, _b(kvw))

        def products(u):
            fr = pl.multiple_of((u >> 3) * 8, 8)
            col = pl.ds(pl.multiple_of((u & 7) * 128, 128), 128)
            xv = xf.at[pl.ds(fr, 2 * S - C + 8), col]
            kw = kf.at[pl.ds(fr, 2 * S - C + 8), col]
            yv = yb.at[pl.ds(fr, S - C + 8), col]
            sign = jax.lax.broadcasted_iota(U32, (8, 128), 0) << 31

            def flip(t):
                return pltpu.bitcast(pltpu.bitcast(t, U32) ^ sign, F32)
            prev = None
            for i0 in range(0, NC, OB):
                acc = [None] * OB
                xs_ = {}
                for j in range(i0 + OB):
                    kr, ki = kw[j * 2 * C:j * 2 * C + 8, :], kw[j * 2 * C + C:j * 2 * C + C + 8, :]
                    for o in range(OB):
                        n = i0 + o - j
                        if n < 0:
                            continue
                        if n not in xs_:
                            xs_[n] = (xv[n * 2 * C:n * 2 * C + 8, :], xv[n * 2 * C + C:n * 2 * C + C + 8, :])
                        xr, xi = xs_[n]
                        tr, ti = xr * kr - xi * ki, xr * ki + xi * kr
                        acc[o] = (tr, ti) if acc[o] is None else (acc[o][0] + tr, acc[o][1] + ti)
                        if n == 0:
                            ar, ai = acc[o]
                            zr, zi = (ar, ai) if prev is None else (ar - flip(prev[1]), ai + flip(prev[0]))
                            yv[(i0 + o) * C:(i0 + o) * C + 8, :] = _pe(zr, zi)
                            prev = (ar, ai)
                        yield
                    xs_.pop(i0 + OB - 1 - j, None)

        NST = -(-128 // (12 - NPRE))

        def unit(un, _, with_products):
            m, qi = un >> 2, un & 3
            wm = w3.at[m]
            for mm in range(3 if with_products else 1):
                @pl.when(m == mm)
                def _():
                    for cp in unit_cps(mm, qi):
                        cp.wait()
            if with_products:
                nx = un + 3
                for mm in range(1, 3):
                    @pl.when((nx >> 2) == mm)
                    def _():
                        start(unit_cps(mm, nx & 3))

                @pl.when(un == 5)
                def _():
                    bq_cp.start()

                @pl.when(un == 8)
                def _():
                    wo_cp.start()
                    x_cp.start()
            else:
                for u0 in range(NPRE):
                    @pl.when(un == u0)
                    def _():
                        if u0 + 1 < NPRE:
                            start(unit_cps(0, u0 + 1))
                        for pp in BSCHED[u0]:
                            start(bin_cps(pp))
            sl = slab.at[pl.ds(qi * 4, 4)]
            wv = wm.at[:, pl.ds(pl.multiple_of(qi * 1024, 1024), 1024)]

            for i in range(64):
                r = slice(i * 8, i * 8 + 8)
                for hh in range(4):
                    a, b = sl[hh, 0, r, :], sl[hh, 1, r, :]
                    wv[r, hh * 256:hh * 256 + 128] = (a & 0xffff) | (b << 16)
                    wv[r, hh * 256 + 128:hh * 256 + 256] = (a >> 16) | (b & jnp.uint32(0xffff0000))
            def strips():
                for t in range(NST if with_products else 0):
                    yield from products(jnp.minimum((un - NPRE) * NST + t, 127))
            work = strips()
            per_dot = -(-NST * (NC * (NC + 1) // 2) // ((512 // MR) * (1024 // NW)))
            wq = wm.at[:, pl.ds(pl.multiple_of(qi * 1024, 1024), 1024)]
            qo = qkv3.at[m].at[:, pl.ds(pl.multiple_of(qi * 1024, 1024), 1024)]
            tiles = [(mb, n) for mb in range(512 // MR) for n in range(1024 // NW)]
            if NMAJ:
                tiles = [(mb, n) for n in range(1024 // NW) for mb in range(512 // MR)]
            for mb, n in tiles:
                cols = slice(n * NW, (n + 1) * NW)
                r = _nn(_b(x3[mb * MR // 16:(mb + 1) * MR // 16].reshape(MR // 2, DM)), _b(wq[:, cols]))
                for _ in range(PRE):
                    next(work, None)
                for j in range(MR // 16):
                    qo[mb * MR // 2 + 8 * j:mb * MR // 2 + 8 * j + 8, cols] = _pe(
                        r[16 * j:16 * j + 8], r[16 * j + 8:16 * j + 16])
                for _ in range(per_dot - PRE):
                    next(work, None)
            for _ in work:
                pass
            return 0

        for cp in x3_cps:
            cp.wait()
        jax.lax.fori_loop(0, NPRE, functools.partial(unit, with_products=False), 0)
        for cp in small:
            cp.wait()
        for p in range(4):
            for cp in bin_cps(p):
                cp.wait()
            for pp in BSCHED2[p]:
                start(bin_cps(pp))
            for uu in USCHED[p]:
                start(unit_cps(uu >> 2, uu & 3))
            bfwd(p)
        jax.lax.fori_loop(NPRE, 12, functools.partial(unit, with_products=True), 0)

        bq_cp.wait()
        wo_cp.wait()
        x_cp.wait()

    pl.run_scoped(phase1, pltpu.VMEM((16, 2, 512, 128), U32), pltpu.VMEM((NSEG // 2, 8, DM), U32),
                  pltpu.VMEM((S // 2 + 8, D), U32), pltpu.VMEM((D, S), BF16),
                  pltpu.VMEM((2 * S, D), F32), pltpu.VMEM((2 * S, D), F32),
                  pltpu.SemaphoreType.DMA((16, 2)), pltpu.SemaphoreType.DMA((3, 4)),
                  pltpu.SemaphoreType.DMA((5,)))

    def phase2(o3):
        NG = H // GH

        def softmax(sc, allowed):
            sc = jnp.where(allowed, sc * c_exp, -1e9)
            e = jnp.exp2(sc - jnp.max(sc, -1, keepdims=True))
            return (e * (1.0 / jnp.sum(e, -1, keepdims=True))).astype(BF16)

        def step(s, mem, si, keep):
            allowed = mask_ref[32 * si:32 * si + 32, 0:48] > 0.5
            allowed3 = mask_ref[64:80, 0:80] > 0.5
            xs0 = xs[s >> 1, 32 * si:32 * si + 16, :].astype(F32)
            xs1 = xs[s >> 1, 32 * si + 16:32 * si + 24, :].astype(F32)
            hb = jnp.concatenate([mem, xs1, xs0], 0).astype(BF16)
            jr = pl.ds(pl.multiple_of((s >> 1) * 8, 8), 8)
            o3v = o3.at[pl.ds(pl.multiple_of((s >> 1) * 16, 16), 16), :]
            st = {}

            def do(op, g):
                if g < 0 or g >= NG or (op[-1] == '3' and si == 0):
                    return
                if op in 'qkv':
                    m = 'qkv'.index(op)
                    t = _nn(hb, _b(w3[m, :, g * GH * DH:(g + 1) * GH * DH]))
                for hh in range(GH):
                    h = g * GH + hh
                    hs = slice(h * DH, (h + 1) * DH)
                    ls = slice(hh * DH, (hh + 1) * DH)
                    if op == 'q':
                        st['q', h] = t[:, ls].astype(BF16)
                    elif op in 'kv':
                        two = [_pe(t[0:8, ls], t[8:16, ls]), _pe(t[16:24, ls], t[24:32, ls])]
                        st[op, h] = jnp.concatenate(two + [qkv3[m, jr, hs]], 0)
                        if si == 0:
                            keep[op, h] = two
                        else:
                            st[op + '3', h] = jnp.concatenate(keep.pop((op, h)) + two + [qkv3[m, jr, hs]], 0)
                    elif op == 'qk':
                        st['s', h] = _nt(st.pop(('q', h)), _b(st.pop(('k', h))))
                    elif op == 'sm':
                        st['p', h] = softmax(st.pop(('s', h)), allowed)
                    elif op == 'pv':
                        st['o', h] = _nn(st.pop(('p', h)), _b(st.pop(('v', h))))
                    elif op == 'qk3':
                        st['s3', h] = _nt(_b(qkv3[0, jr, hs]), _b(st.pop(('k3', h))))
                    elif op == 'sm3':
                        st['p3', h] = softmax(st.pop(('s3', h)), allowed3)
                    else:
                        o3v[:, hs] = _nn(st.pop(('p3', h)), _b(st.pop(('v3', h))))
            def fill(cb):
                c = s >> 2
                cols = pl.ds(pl.multiple_of(cb * 256, 256), 256)
                wrows = pl.ds(pl.multiple_of(c * CW, CW), CW)
                y = _nn(inv_ref[...], _b(yb[pl.ds(pl.multiple_of(c * C, C), C), cols]))
                dd = sd_ref[:, cols].astype(F32)
                kvw, qw = kv[wrows, cols], bq[wrows, cols]
                out = []
                for i in range(C // 16):
                    wr = slice(8 * i, 8 * i + 8)
                    ye = y[16 * i:16 * i + 8] + _lo(kvw[wr]) * dd
                    yo = y[16 * i + 8:16 * i + 16] + _hi(kvw[wr]) * dd
                    out.append(_pe(ye * _lo(qw[wr]), yo * _hi(qw[wr])))
                obb[pl.ds(c * (C // SEG), C // SEG), :, cols] = jnp.concatenate(out, 0).reshape(C // SEG, SEG // 2, 256)

            def fills(pos):
                for fsi, fpos, k in FILL:
                    if fsi == si and fpos == pos:
                        fill((s & 2) + k)
            r = None
            done = 0
            order = ORDER
            for g in range(NG + max(d for _, d in order)):
                fills(100 + g)
                for op, d in order:
                    do(op, g - d)
                for p, gmin in PARTS:
                    if g >= gmin and done < p and all(('o', h) in st for h in range(done, p)):
                        fills(p)
                        part = _nn(jnp.concatenate([st.pop(('o', h)) for h in range(done, p)], 1).astype(BF16),
                                   _b(wo[done * DH // 2:p * DH // 2, :]))
                        r = part if r is None else r + part
                        done = p
            fills(99)
            rb = r.astype(BF16)
            ob[s, 0:16, :] = rb[16:32]
            ob[s, 16:24, :] = rb[8:16]

            if si == 1:
                @pl.when((s & 3) == 3)
                def _():
                    b_cp(s >> 2).start()
            return rb[0:8].astype(F32)
        def steps(t, mem):
            keep = {}
            for i in range(2):
                mem = step(t * 2 + i, mem, i, keep)
            return mem
        jax.lax.fori_loop(0, NSEG // 2, steps, mem0_ref[...].astype(F32))

        a_cp = pltpu.make_async_copy(ob.at[:, pl.ds(0, 24), :], out_h.at[:, pl.ds(0, 24), pl.ds(0, DM)],
                                     osem.at[0])
        a_cp.start()

        FS = FINM // 8

        def f_cp(n):
            return pltpu.make_async_copy(ob.at[pl.ds(n * FS, FS), pl.ds(24, 8), :],
                                         out_h.at[pl.ds(n * FS, FS), pl.ds(24, 8), pl.ds(0, DM)], osem.at[2])

        def fin(n, _):
            rows = pl.ds(pl.multiple_of(n * FINM, FINM), FINM)
            lhs = o3[rows, :].astype(BF16)
            for cb in range(DM // FINW):
                cols = slice(cb * FINW, (cb + 1) * FINW)
                w = pltpu.bitcast(_nn(lhs, _b(wo[:, cols])).astype(BF16), U32)
                for i in range(FINM // 16):
                    wi = w[i * 8:(i + 1) * 8]
                    for half, val in ((0, _lo(wi)), (1, _hi(wi))):
                        ob[n * FS + 2 * i + half, 24:32, cols] = val.astype(BF16)
            f_cp(n).start()
            return 0
        jax.lax.fori_loop(0, 512 // FINM, fin, 0)
        a_cp.wait()
        for c in range(NC):
            b_cp(c).wait()
        for n in range(512 // FINM):
            f_cp(n).wait()

    pl.run_scoped(phase2, pltpu.VMEM((NSEG * 8, HD), F32))


@functools.partial(jax.jit, static_argnames=("A_seg_len",))
def pallas_concat_heads__memory_aug_recurrent_mem_tr__ssm_conv_h3__prompt_kernel(
        A_x, A_mem0, A_Wq, A_Wk, A_Wv, A_Wo, A_seg_len, B_q, B_k, B_v, B_shift_k, B_ssm_k, B_ssm_D):
    assert int(A_seg_len) == SEG
    vm = pl.BlockSpec(memory_space=pltpu.VMEM)
    hbm = pl.BlockSpec(memory_space=pl.ANY)
    out = pl.pallas_call(
        _kernel,
        in_specs=[hbm] * 15,
        out_specs=hbm,
        out_shape=jax.ShapeDtypeStruct((NSEG, SEG, DM + D), BF16),
        scratch_shapes=[pltpu.VMEM((3, 512, HD), U32), pltpu.VMEM((HD // 2, DM), U32),
                        pltpu.VMEM((NSEG // 2, 2 * SEG, DM), BF16), pltpu.VMEM((3, 256, HD), U32),
                        pltpu.VMEM((NSEG, SEG, DM), BF16), pltpu.VMEM((NSEG, SEG // 2, D), U32),
                        pltpu.VMEM((S // 2, D), U32), pltpu.VMEM((S // 2, D), U32), pltpu.VMEM((S, D), U32),
                        pltpu.SemaphoreType.DMA((3,)),
                        pltpu.VMEM((M, DM), BF16), pltpu.VMEM((4, D), BF16), pltpu.VMEM((1, D), BF16),
                        pltpu.VMEM((2 * C, C), BF16), pltpu.VMEM((C, 2 * C), BF16), pltpu.VMEM((80, 128), F32),
                        pltpu.SemaphoreType.DMA((6,))],
        compiler_params=pltpu.CompilerParams(vmem_limit_bytes=126 * 1024 * 1024),
    )(A_mem0[0], *[w.reshape(DM // 2, 2, H, DH) for w in (A_Wq, A_Wk, A_Wv)], A_Wo.reshape(HD, DM),
      A_x.reshape(NSEG // 2, 2 * SEG, DM), B_q[0], B_k[0], B_v[0],
      B_shift_k.T, B_ssm_k, B_ssm_D.reshape(1, D),
      jnp.asarray(_FWD).astype(BF16), jnp.asarray(_INV).astype(BF16), jnp.asarray(_MASKS))
    return out.reshape(1, S, DM + D)
```

```python
import functools
import numpy as np
import jax
import jax.numpy as jnp
import jax.experimental.pallas as pl
import jax.experimental.pallas.tpu as pltpu

S, DM, H, DH, M, D = 2048, 1024, 32, 128, 8, 1024
HD = H * DH
SEG = 32
NSEG = S // SEG
C = 128
NC = S // C
CW = C // 2
GH = 2
ORDER = (('qk', 1), ('pv', 2), ('k', 0), ('pv3', 3), ('q', 0), ('v', 0), ('sm3', 2), ('qk3', 1), ('sm', 1))
PARTS = ((16, 0), (22, 16), (30, 17), (32, 0))
FILL = ((0, 100, 0), (1, 100, 1))
FINM, FINW = 64, 1024
OB = 4
NPRE = 2
BSCHED = ((0,), (1, 2))
BSCHED2 = ((3,), (), (), ())
USCHED = ((), (2, 3), (4,), ())
F32, BF16, U32 = jnp.float32, jnp.bfloat16, jnp.uint32
LOG2E = 1.4426950408889634


def _dft_consts():
    th = 2 * np.pi * (np.arange(C)[:, None] + 0.5) / (2 * C)
    n = np.arange(2 * C)[None, :]
    cos, sin = np.cos(th * n), np.sin(th * n)
    fwd = np.concatenate([cos[:, :C], -sin[:, :C]], 0)
    inv = np.concatenate([cos, -sin], 0).T / C
    perm = np.arange(2 * C).reshape(2, C).T.reshape(-1)
    inv = inv[:, perm]
    g = inv[:C]
    rows = np.arange(C).reshape(C // 16, 8, 2).transpose(0, 2, 1).reshape(-1)
    g = g[rows]
    return fwd.astype(np.float32), g.astype(np.float32)


def _attn_masks():
    nat = np.array([-1] * 8 + list(range(16, 24)) + list(range(16)))
    c = np.arange(16)
    inter = c // 2 + 8 * (c % 2)
    klab = np.concatenate([nat[:16][inter], nat[16:][inter], 24 + c // 2])
    out = np.zeros((80, 128), np.float32)
    for par in range(2):
        valid = np.concatenate([np.ones(32, bool), c % 2 == par])
        ok = (nat[:, None] < 0) | (klab[None, :] < 0) | (klab[None, :] <= nat[:, None])
        out[32 * par:32 * par + 32, :48] = ok & valid[None, :]
    for r in range(16):
        par, i = r % 2, r // 2
        out[64 + r, 32 * par:32 * par + 32] = 1
        out[64 + r, 64:80] = (c % 2 == par) & (c // 2 <= i)
    return out


_FWD, _INV = _dft_consts()
_MASKS = _attn_masks()


def _nn(a, b):
    return jnp.dot(a, b, preferred_element_type=F32)


def _nt(a, b):
    return jax.lax.dot_general(a, b, (((1,), (1,)), ((), ())), preferred_element_type=F32)


def _b(x):
    return pltpu.bitcast(x, BF16)


def _pe(lo, hi):
    rnd = lambda t: pltpu.bitcast(t.astype(BF16).astype(F32), U32)
    return (rnd(lo) >> 16) | rnd(hi)


def _lo(w):
    return pltpu.bitcast(w << 16, F32)


def _hi(w):
    return pltpu.bitcast(w & jnp.uint32(0xffff0000), F32)


def _kernel(mem0_h, wq_h, wk_h, wv_h, wo_h, x_h, bq_h, bk_h, bv_h, sk_h, ssmk_h, sd_h,
            fwd_h, inv_h, mask_h, out_h,
            w3, wo, xs, qkv3, ob, obb, bq, kv, yb, osem,
            mem0_ref, sk_ref, sd_ref, fwd_ref, inv_ref, mask_ref, csem):
    c_exp = DH ** -0.5 * LOG2E
    small = [pltpu.make_async_copy(src, dst, csem.at[i]) for i, (src, dst) in enumerate(
        ((sk_h, sk_ref), (fwd_h, fwd_ref), (mem0_h, mem0_ref), (sd_h, sd_ref), (inv_h, inv_ref), (mask_h, mask_ref)))]
    w_h = [r.bitcast(U32) for r in (wq_h, wk_h, wv_h)]

    def b_cp(c):
        segs = pl.ds(c * (C // SEG), C // SEG)
        return pltpu.make_async_copy(obb.at[segs], out_h.bitcast(U32).at[segs, :, pl.ds(DM, D)], osem.at[1])

    def phase1(slab, x3, bk, sk, xf, kf, wsem, bsem, dsem):
        def slab_cp(m, hp, par):
            return pltpu.make_async_copy(w_h[m].at[:, par, hp, :], slab.at[hp, par], wsem.at[hp, par])
        x32 = x_h.bitcast(U32)
        x3_cps = [pltpu.make_async_copy(x32.at[:, pl.ds(12 + 16 * p, 4), :], x3.at[:, pl.ds(4 * p, 4), :],
                                        dsem.at[3 + p]) for p in range(2)]
        wo_cp = pltpu.make_async_copy(wo_h.bitcast(U32), wo, dsem.at[0])
        x_cp = pltpu.make_async_copy(x_h, xs, dsem.at[1])
        bq_cp = pltpu.make_async_copy(bq_h.bitcast(U32), bq, dsem.at[2])
        QB = NC // 4

        bk32, bv32 = bk_h.bitcast(U32), bv_h.bitcast(U32)

        def bin_cps(p):
            rows = pl.ds(p * QB * C, QB * C)
            wr = pl.ds(p * QB * CW, QB * CW)
            return [pltpu.make_async_copy(bk32.at[wr], bk.at[pl.ds(8 + p * QB * CW, QB * CW)], bsem.at[0, p]),
                    pltpu.make_async_copy(bv32.at[wr], kv.at[wr], bsem.at[1, p]),
                    pltpu.make_async_copy(ssmk_h.at[:, rows], sk.at[:, rows], bsem.at[2, p])]

        def unit_cps(m, qi):
            return [slab_cp(m, qi * 4 + hh, par) for hh in range(4) for par in range(2)]

        def start(cps):
            for cp in cps:
                cp.start()

        start(x3_cps)
        start(unit_cps(0, 0))
        start(small)
        bk[0:8, :] = jnp.zeros((8, D), U32)
        CB = 512

        def bfwd(p):
            fwd = fwd_ref[...]
            for c in range(p * QB, (p + 1) * QB):
                rows, wrows, spec = pl.ds(c * C, C), pl.ds(c * CW, CW), pl.ds(c * 2 * C, 2 * C)
                for cb in range(D // CB):
                    cols = slice(cb * CB, (cb + 1) * CB)
                    kf[spec, cols] = _nt(fwd, sk[cols, rows])
                    t0, t1, t2, t3 = [sk_ref[d:d + 1, cols].astype(F32) for d in range(4)]
                    blk = bk[pl.ds(c * CW, CW + 8), cols]
                    w0, w1, w2 = blk[8:], pltpu.roll(blk, 1, 0)[8:], pltpu.roll(blk, 2, 0)[8:]
                    e0, o0, e1, o1, o2 = _lo(w0), _hi(w0), _lo(w1), _hi(w1), _hi(w2)
                    v = kv[wrows, cols]
                    kvw = _pe((e0 * t0 + o1 * t1 + e1 * t2 + o2 * t3) * _lo(v),
                              (o0 * t0 + e0 * t1 + o1 * t2 + e1 * t3) * _hi(v))
                    kv[wrows, cols] = kvw
                    xf[spec, cols] = _nn(fwd, _b(kvw))

        def products(u):
            fr = pl.multiple_of((u >> 3) * 8, 8)
            col = pl.ds(pl.multiple_of((u & 7) * 128, 128), 128)
            xv = xf.at[pl.ds(fr, 2 * S - C + 8), col]
            kw = kf.at[pl.ds(fr, 2 * S - C + 8), col]
            yv = yb.at[pl.ds(fr, S - C + 8), col]
            sign = jax.lax.broadcasted_iota(U32, (8, 128), 0) << 31

            def flip(t):
                return pltpu.bitcast(pltpu.bitcast(t, U32) ^ sign, F32)
            prev = None
            for i0 in range(0, NC, OB):
                acc = [None] * OB
                xs_ = {}
                for j in range(i0 + OB):
                    kr, ki = kw[j * 2 * C:j * 2 * C + 8, :], kw[j * 2 * C + C:j * 2 * C + C + 8, :]
                    for o in range(OB):
                        n = i0 + o - j
                        if n < 0:
                            continue
                        if n not in xs_:
                            xs_[n] = (xv[n * 2 * C:n * 2 * C + 8, :], xv[n * 2 * C + C:n * 2 * C + C + 8, :])
                        xr, xi = xs_[n]
                        tr, ti = xr * kr - xi * ki, xr * ki + xi * kr
                        acc[o] = (tr, ti) if acc[o] is None else (acc[o][0] + tr, acc[o][1] + ti)
                        if n == 0:
                            ar, ai = acc[o]
                            zr, zi = (ar, ai) if prev is None else (ar - flip(prev[1]), ai + flip(prev[0]))
                            yv[(i0 + o) * C:(i0 + o) * C + 8, :] = _pe(zr, zi)
                            prev = (ar, ai)
                        yield
                    xs_.pop(i0 + OB - 1 - j, None)

        NST = -(-128 // (12 - NPRE))

        def unit(un, _, with_products):
            m, qi = un >> 2, un & 3
            wm = w3.at[m]
            for mm in range(3 if with_products else 1):
                @pl.when(m == mm)
                def _():
                    for cp in unit_cps(mm, qi):
                        cp.wait()
            if with_products:
                nx = un + 3
                for mm in range(1, 3):
                    @pl.when((nx >> 2) == mm)
                    def _():
                        start(unit_cps(mm, nx & 3))

                @pl.when(un == 5)
                def _():
                    bq_cp.start()

                @pl.when(un == 8)
                def _():
                    wo_cp.start()
                    x_cp.start()
            else:
                for u0 in range(NPRE):
                    @pl.when(un == u0)
                    def _():
                        if u0 + 1 < NPRE:
                            start(unit_cps(0, u0 + 1))
                        for pp in BSCHED[u0]:
                            start(bin_cps(pp))
            sl = slab.at[pl.ds(qi * 4, 4)]
            wv = wm.at[:, pl.ds(pl.multiple_of(qi * 1024, 1024), 1024)]

            for i in range(64):
                r = slice(i * 8, i * 8 + 8)
                for hh in range(4):
                    a, b = sl[hh, 0, r, :], sl[hh, 1, r, :]
                    wv[r, hh * 256:hh * 256 + 128] = (a & 0xffff) | (b << 16)
                    wv[r, hh * 256 + 128:hh * 256 + 256] = (a >> 16) | (b & jnp.uint32(0xffff0000))

            def strips():
                for t in range(NST if with_products else 0):
                    yield from products(jnp.minimum((un - NPRE) * NST + t, 127))
            work = strips()
            per_dot = -(-NST * (NC * (NC + 1) // 2) // 64)
            qo = qkv3.at[m].at[:, pl.ds(pl.multiple_of(qi * 1024, 1024), 1024)]
            for mb in range(8):
                for n in range(8):
                    cols = slice(n * 128, (n + 1) * 128)
                    r = _nn(_b(x3[mb * 4:(mb + 1) * 4].reshape(32, DM)), _b(wv[:, cols]))
                    for j in range(4):
                        qo[mb * 32 + 8 * j:mb * 32 + 8 * j + 8, cols] = _pe(r[16 * j:16 * j + 8],
                                                                            r[16 * j + 8:16 * j + 16])
                    for _ in range(per_dot):
                        next(work, None)
            for _ in work:
                pass
            return 0

        for cp in x3_cps:
            cp.wait()
        jax.lax.fori_loop(0, NPRE, functools.partial(unit, with_products=False), 0)
        for cp in small:
            cp.wait()
        for p in range(4):
            for cp in bin_cps(p):
                cp.wait()
            for pp in BSCHED2[p]:
                start(bin_cps(pp))
            for uu in USCHED[p]:
                start(unit_cps(uu >> 2, uu & 3))
            bfwd(p)
        jax.lax.fori_loop(NPRE, 12, functools.partial(unit, with_products=True), 0)

        bq_cp.wait()
        wo_cp.wait()
        x_cp.wait()

    pl.run_scoped(phase1, pltpu.VMEM((16, 2, 512, 128), U32), pltpu.VMEM((NSEG // 2, 8, DM), U32),
                  pltpu.VMEM((S // 2 + 8, D), U32), pltpu.VMEM((D, S), BF16),
                  pltpu.VMEM((2 * S, D), F32), pltpu.VMEM((2 * S, D), F32),
                  pltpu.SemaphoreType.DMA((16, 2)), pltpu.SemaphoreType.DMA((3, 4)),
                  pltpu.SemaphoreType.DMA((5,)))

    def phase2(o3):
        NG = H // GH

        def softmax(sc, allowed):
            sc = jnp.where(allowed, sc * c_exp, -1e9)
            e = jnp.exp2(sc - jnp.max(sc, -1, keepdims=True))
            return (e * (1.0 / jnp.sum(e, -1, keepdims=True))).astype(BF16)

        def step(s, mem, si, keep):
            allowed = mask_ref[32 * si:32 * si + 32, 0:48] > 0.5
            allowed3 = mask_ref[64:80, 0:80] > 0.5
            xs0 = xs[s >> 1, 32 * si:32 * si + 16, :].astype(F32)
            xs1 = xs[s >> 1, 32 * si + 16:32 * si + 24, :].astype(F32)
            hb = jnp.concatenate([mem, xs1, xs0], 0).astype(BF16)
            jr = pl.ds(pl.multiple_of((s >> 1) * 8, 8), 8)
            o3v = o3.at[pl.ds(pl.multiple_of((s >> 1) * 16, 16), 16), :]
            st = {}

            def do(op, g):
                if g < 0 or g >= NG or (op[-1] == '3' and si == 0):
                    return
                if op in 'qkv':
                    m = 'qkv'.index(op)
                    t = _nn(hb, _b(w3[m, :, g * GH * DH:(g + 1) * GH * DH]))
                for hh in range(GH):
                    h = g * GH + hh
                    hs = slice(h * DH, (h + 1) * DH)
                    ls = slice(hh * DH, (hh + 1) * DH)
                    if op == 'q':
                        st['q', h] = t[:, ls].astype(BF16)
                    elif op in 'kv':
                        two = [_pe(t[0:8, ls], t[8:16, ls]), _pe(t[16:24, ls], t[24:32, ls])]
                        st[op, h] = jnp.concatenate(two + [qkv3[m, jr, hs]], 0)
                        if si == 0:
                            keep[op, h] = two
                        else:
                            st[op + '3', h] = jnp.concatenate(keep.pop((op, h)) + two + [qkv3[m, jr, hs]], 0)
                    elif op == 'qk':
                        st['s', h] = _nt(st.pop(('q', h)), _b(st.pop(('k', h))))
                    elif op == 'sm':
                        st['p', h] = softmax(st.pop(('s', h)), allowed)
                    elif op == 'pv':
                        st['o', h] = _nn(st.pop(('p', h)), _b(st.pop(('v', h))))
                    elif op == 'qk3':
                        st['s3', h] = _nt(_b(qkv3[0, jr, hs]), _b(st.pop(('k3', h))))
                    elif op == 'sm3':
                        st['p3', h] = softmax(st.pop(('s3', h)), allowed3)
                    else:
                        o3v[:, hs] = _nn(st.pop(('p3', h)), _b(st.pop(('v3', h))))
            def fill(cb):
                c = s >> 2
                cols = pl.ds(pl.multiple_of(cb * 256, 256), 256)
                wrows = pl.ds(pl.multiple_of(c * CW, CW), CW)
                y = _nn(inv_ref[...], _b(yb[pl.ds(pl.multiple_of(c * C, C), C), cols]))
                dd = sd_ref[:, cols].astype(F32)
                kvw, qw = kv[wrows, cols], bq[wrows, cols]
                out = []
                for i in range(C // 16):
                    wr = slice(8 * i, 8 * i + 8)
                    ye = y[16 * i:16 * i + 8] + _lo(kvw[wr]) * dd
                    yo = y[16 * i + 8:16 * i + 16] + _hi(kvw[wr]) * dd
                    out.append(_pe(ye * _lo(qw[wr]), yo * _hi(qw[wr])))
                obb[pl.ds(c * (C // SEG), C // SEG), :, cols] = jnp.concatenate(out, 0).reshape(C // SEG, SEG // 2, 256)

            def fills(pos):
                for fsi, fpos, k in FILL:
                    if fsi == si and fpos == pos:
                        fill((s & 2) + k)
            r = None
            done = 0
            order = ORDER
            for g in range(NG + max(d for _, d in order)):
                fills(100 + g)
                for op, d in order:
                    do(op, g - d)
                for p, gmin in PARTS:
                    if g >= gmin and done < p and all(('o', h) in st for h in range(done, p)):
                        fills(p)
                        part = _nn(jnp.concatenate([st.pop(('o', h)) for h in range(done, p)], 1).astype(BF16),
                                   _b(wo[done * DH // 2:p * DH // 2, :]))
                        r = part if r is None else r + part
                        done = p
            fills(99)
            rb = r.astype(BF16)
            ob[s, 0:16, :] = rb[16:32]
            ob[s, 16:24, :] = rb[8:16]

            return rb[0:8].astype(F32)
        def steps(t, mem):
            @pl.when(jnp.logical_and(t > 0, (t & 1) == 0))
            def _():
                b_cp((t >> 1) - 1).start()
            keep = {}
            for i in range(2):
                mem = step(t * 2 + i, mem, i, keep)
            return mem
        jax.lax.fori_loop(0, NSEG // 2, steps, mem0_ref[...].astype(F32))

        a_cp = pltpu.make_async_copy(ob.at[:, pl.ds(0, 24), :], out_h.at[:, pl.ds(0, 24), pl.ds(0, DM)],
                                     osem.at[0])
        b_cp(NC - 1).start()
        a_cp.start()

        FS = FINM // 8

        def f_cp(n):
            return pltpu.make_async_copy(ob.at[pl.ds(n * FS, FS), pl.ds(24, 8), :],
                                         out_h.at[pl.ds(n * FS, FS), pl.ds(24, 8), pl.ds(0, DM)], osem.at[2])

        def fin(n, _):
            rows = pl.ds(pl.multiple_of(n * FINM, FINM), FINM)
            lhs = o3[rows, :].astype(BF16)
            for cb in range(DM // FINW):
                cols = slice(cb * FINW, (cb + 1) * FINW)
                w = pltpu.bitcast(_nn(lhs, _b(wo[:, cols])).astype(BF16), U32)
                for i in range(FINM // 16):
                    wi = w[i * 8:(i + 1) * 8]
                    for half, val in ((0, _lo(wi)), (1, _hi(wi))):
                        ob[n * FS + 2 * i + half, 24:32, cols] = val.astype(BF16)
            f_cp(n).start()
            return 0
        jax.lax.fori_loop(0, 512 // FINM, fin, 0)
        a_cp.wait()
        for c in range(NC):
            b_cp(c).wait()
        for n in range(512 // FINM):
            f_cp(n).wait()

    pl.run_scoped(phase2, pltpu.VMEM((NSEG * 8, HD), F32))


@functools.partial(jax.jit, static_argnames=("A_seg_len",))
def pallas_concat_heads__memory_aug_recurrent_mem_tr__ssm_conv_h3__prompt_kernel(
        A_x, A_mem0, A_Wq, A_Wk, A_Wv, A_Wo, A_seg_len, B_q, B_k, B_v, B_shift_k, B_ssm_k, B_ssm_D):
    assert int(A_seg_len) == SEG
    vm = pl.BlockSpec(memory_space=pltpu.VMEM)
    hbm = pl.BlockSpec(memory_space=pl.ANY)
    out = pl.pallas_call(
        _kernel,
        in_specs=[hbm] * 15,
        out_specs=hbm,
        out_shape=jax.ShapeDtypeStruct((NSEG, SEG, DM + D), BF16),
        scratch_shapes=[pltpu.VMEM((3, 512, HD), U32), pltpu.VMEM((HD // 2, DM), U32),
                        pltpu.VMEM((NSEG // 2, 2 * SEG, DM), BF16), pltpu.VMEM((3, 256, HD), U32),
                        pltpu.VMEM((NSEG, SEG, DM), BF16), pltpu.VMEM((NSEG, SEG // 2, D), U32),
                        pltpu.VMEM((S // 2, D), U32), pltpu.VMEM((S // 2, D), U32), pltpu.VMEM((S, D), U32),
                        pltpu.SemaphoreType.DMA((3,)),
                        pltpu.VMEM((M, DM), BF16), pltpu.VMEM((4, D), BF16), pltpu.VMEM((1, D), BF16),
                        pltpu.VMEM((2 * C, C), BF16), pltpu.VMEM((C, 2 * C), BF16), pltpu.VMEM((80, 128), F32),
                        pltpu.SemaphoreType.DMA((6,))],
        compiler_params=pltpu.CompilerParams(vmem_limit_bytes=126 * 1024 * 1024),
    )(A_mem0[0], *[w.reshape(DM // 2, 2, H, DH) for w in (A_Wq, A_Wk, A_Wv)], A_Wo.reshape(HD, DM),
      A_x.reshape(NSEG // 2, 2 * SEG, DM), B_q[0], B_k[0], B_v[0],
      B_shift_k.T, B_ssm_k, B_ssm_D.reshape(1, D),
      jnp.asarray(_FWD).astype(BF16), jnp.asarray(_INV).astype(BF16), jnp.asarray(_MASKS))
    return out.reshape(1, S, DM + D)
```
